```python
import os as _os
_os.environ.setdefault("JAX_PLATFORMS", "cpu")
import jax
import jax.numpy as jnp

def _softmax(x, axis=-1):
    return jax.nn.softmax(x, axis=axis)
def _gelu(x):
    return jax.nn.gelu(x, approximate=True)
def _silu(x):
    return jax.nn.silu(x)
def _sigmoid(x):
    return jax.nn.sigmoid(x)
def _layernorm(x, axis=-1, eps=1e-5):
    m = jnp.mean(x, axis=axis, keepdims=True)
    v = jnp.var(x, axis=axis, keepdims=True)
    return (x - m) / jnp.sqrt(v + eps)
def _scatter_add(tgt, idx, src, axis=0):
    return tgt.at[idx].add(src)
def _segment_sum(src, seg, n):
    return jax.ops.segment_sum(src, seg, n)
class _Rng:
    def __init__(self, key):
        self._k = key
    def _next(self):
        self._k, sub = jax.random.split(self._k)
        return sub
    def normal(self, shape):
        return jax.random.normal(self._next(), shape, dtype=jnp.bfloat16)
    def randint(self, lo, hi, shape):
        return jax.random.randint(self._next(), shape, lo, hi, dtype=jnp.int32)
    def uniform(self, shape, lo=0.0, hi=1.0):
        return jax.random.uniform(self._next(), shape, jnp.bfloat16, lo, hi)
    def permutation(self, n):
        return jax.random.permutation(self._next(), n)


kernel_name = 'gated_mix__sliding_block__sliding_local_dilated__prompt'

def setup_inputs():
    _rng = _Rng(jax.random.key(int.from_bytes(__import__("os").urandom(4), "little")))
    _w = (lambda a: (lambda t: t.astype(jnp.bfloat16) if jnp.issubdtype(t.dtype, jnp.floating) else t)(jnp.asarray(a)))
    def _A_setup():
        B, S, D = 1, 2048, 640
        return {
            "x": _w((lambda *s: _rng.normal(s) * 0.05)(B, S, D)),
            "wqkv": _w((lambda *s: _rng.normal(s) * 0.8)(D, 3 * D)),
            "wo": _w((lambda *s: _rng.normal(s) * 0.05)(D, D)),
        }
    _A_in = _A_setup()

    def _B_setup():
        B, S, D = 1, 2048, 640
        return {
            "x": _w((lambda *s: _rng.normal(s) * 0.05)(B, S, D)),
            "wqkv": _w((lambda *s: _rng.normal(s) * 0.8)(D, 3 * D)),
            "wo": _w((lambda *s: _rng.normal(s) * 0.05)(D, D)),
        }
    _B_in = _B_setup()

    return {
        "A_x": _A_in["x"],
        "A_wqkv": _A_in["wqkv"],
        "A_wo": _A_in["wo"],
        "B_x": _B_in["x"],
        "B_wqkv": _B_in["wqkv"],
        "B_wo": _B_in["wo"],
        "gate_w": _w((lambda *s: _rng.normal(s) * 0.05)(640) * 16.0),
    }

def reference(A_x, A_wqkv, A_wo, B_x, B_wqkv, B_wo, gate_w):
    def _A_ref(x, wqkv, wo):
        B, S, D = x.shape
        H = 32; Dh = D // H; W = 256
        qkv = (lambda x, *d: x.transpose(*d))((x @ wqkv).reshape(B, S, 3, H, Dh), 2, 0, 3, 1, 4)
        q, k, v = qkv[0], qkv[1], qkv[2]
        scores = jnp.einsum("bhqd,bhkd->bhqk", q, k) * (Dh ** -0.5)
        idx = jnp.arange(S)
        mask = (idx[:, None] - idx[None, :] >= 0) & (idx[:, None] - idx[None, :] < W)
        scores = jnp.where(mask[None, None], scores, -1e9)
        p = _softmax(scores, axis=-1)
        o = jnp.einsum("bhqk,bhkd->bhqd", p, v)
        return (lambda x, *d: x.transpose(*d))(o, 0, 2, 1, 3).reshape(B, S, D) @ wo

    def _B_ref(x, wqkv, wo):
        B, S, D = x.shape
        H = 32; Dh = D // H
        W, dil = 8, 2
        qkv = (lambda x, *d: x.transpose(*d))((x @ wqkv).reshape(B, S, 3, H, Dh), 2, 0, 3, 1, 4)
        q, k, v = qkv[0], qkv[1], qkv[2]
        scale = Dh ** -0.5
        pos = jnp.arange(S)
        off = jnp.arange(W) * dil
        idx = pos[:, None] - off[None, :]
        mask = idx >= 0
        idx_c = jnp.where(mask, idx, 0).reshape(-1)
        kg = k[:, :, idx_c, :].reshape(B, H, S, W, Dh)
        vg = v[:, :, idx_c, :].reshape(B, H, S, W, Dh)
        logits = jnp.einsum("bhsd,bhswd->bhsw", q, kg) * scale
        logits = jnp.where(mask[None, None, :, :], logits, -1e9)
        attn = _softmax(logits, axis=-1)
        o = jnp.einsum("bhsw,bhswd->bhsd", attn, vg)
        return (lambda x, *d: x.transpose(*d))(o, 0, 2, 1, 3).reshape(B, S, D) @ wo

    x = A_x
    g = _sigmoid((x * gate_w).sum(-1, keepdims=True))
    a = _A_ref(x, A_wqkv, A_wo)
    b = _B_ref(x, B_wqkv, B_wo)
    return g * a + (1 - g) * b
```

```python
import functools

import jax
import jax.numpy as jnp
import numpy as np
import jax.experimental.pallas as pl
import jax.experimental.pallas.tpu as pltpu

S = 2048
D = 640
H = 32
DH = 20
R = 256
QC = 64
NCH = R // QC
NPAIR = H // 2
WA = 256
HB = 16
NEG = -1e30
LOG2E = 1.4426950408889634
QSCALE = float(DH ** -0.5) * LOG2E


def _pair_tile(p):
    c0 = 40 * p
    t0, off = divmod(c0, 128)
    if off + 40 <= 128:
        return (t0, t0, 0), off
    return (t0, t0 + 1, off), off


_TILES = []
_PAIR = []
for _p in range(NPAIR):
    _t, _o = _pair_tile(_p)
    if _t not in _TILES:
        _TILES.append(_t)
    _PAIR.append((_TILES.index(_t), _o))
NT = len(_TILES)


def _build_tiles(y):
    rows = y.shape[0]
    lane = jax.lax.broadcasted_iota(jnp.int32, (rows, 128), 1)
    out = []
    for (a, b, split) in _TILES:
        ta = y[:, a * 128:(a + 1) * 128]
        if a == b:
            out.append(ta)
        else:
            tb = y[:, b * 128:(b + 1) * 128]
            out.append(jnp.where(lane >= split, ta, tb))
    return out


def _nt_dot(a, b):
    return jax.lax.dot_general(a, b, (((1,), (1,)), ((), ())),
                               preferred_element_type=jnp.float32)


def _dot(a, b):
    return jnp.dot(a, b, preferred_element_type=jnp.float32)


def kernel(x_ref, wa_ref, woa_ref, wb_ref, wob_ref, gw_ref, o_ref,
           qa_ref, ka_ref, vta_ref, qb_ref, kb_ref, vb_ref, vtb_ref, ot_ref):
    t = pl.program_id(0)
    bf = jnp.bfloat16

    @pl.when(t == 0)
    def _():
        ka_ref[:, 0:WA, :] = jnp.zeros((NT, WA, 128), bf)
        vta_ref[:, 0:WA] = jnp.zeros((D, WA), bf)
        kb_ref[:, 0:HB, :] = jnp.zeros((NT, HB, 128), bf)
        vb_ref[0:HB, :] = jnp.zeros((HB, D), bf)
        vb_ref[HB + R:HB + R + 48, :] = jnp.zeros((48, D), bf)

    @pl.when(t > 0)
    def _():
        ka_ref[:, 0:WA, :] = ka_ref[:, R:R + WA, :]
        vta_ref[:, 0:WA] = vta_ref[:, R:R + WA]
        kb_ref[:, 0:HB, :] = kb_ref[:, R:R + HB, :]
        vb_ref[0:HB, :] = vb_ref[R:R + HB, :]

    x = x_ref[...]

    def proj(w_ref, q_ref, k_ref, koff):
        q = (_dot(x, w_ref[:, 0:D]) * QSCALE).astype(bf)
        for i, tl in enumerate(_build_tiles(q)):
            q_ref[i] = tl
        k = _dot(x, w_ref[:, D:2 * D]).astype(bf)
        for i, tl in enumerate(_build_tiles(k)):
            k_ref[i, koff:koff + R, :] = tl
        v = _dot(x, w_ref[:, 2 * D:3 * D]).astype(bf)
        return v

    va = proj(wa_ref, qa_ref, ka_ref, WA)
    vta_ref[:, WA:WA + R] = va.T
    vb = proj(wb_ref, qb_ref, kb_ref, HB)
    vb_ref[HB:HB + R, :] = vb
    for i in range(NCH):
        vtb_ref[i] = vb_ref[i * QC:i * QC + 128, :].T

    lane128 = jax.lax.broadcasted_iota(jnp.int32, (QC, 128), 1)
    row64 = jax.lax.broadcasted_iota(jnp.int32, (QC, 128), 0)
    jq = lane128 & (QC - 1)
    lower = row64 <= jq
    rb = jax.lax.broadcasted_iota(jnp.int32, (QC + HB, 128), 0)
    jb = jax.lax.broadcasted_iota(jnp.int32, (QC + HB, 128), 1) & (QC - 1)
    db = jb + HB - rb
    band_b = (db >= 0) & (db < 16) & ((db & 1) == 0)
    row48 = jax.lax.broadcasted_iota(jnp.int32, (48, 128), 0)
    lane48 = jax.lax.broadcasted_iota(jnp.int32, (48, 128), 1)
    zeros64 = jnp.zeros((QC, 128), bf)
    zeros48 = jnp.zeros((48, 128), bf)

    def masked_q(q_ref, tix, off, i):
        qt = q_ref[tix, i * QC:(i + 1) * QC, :]
        rel = (lane128 - off) & 127
        z = jnp.zeros_like(qt)
        return jnp.concatenate(
            [jnp.where(rel < DH, qt, z), jnp.where((rel >= DH) & (rel < 2 * DH), qt, z)], axis=0)

    def unit_a(p, i):
        tix, off = _PAIR[p]
        qm = masked_q(qa_ref, tix, off, i)
        kk = ka_ref[tix, i * QC:i * QC + WA + QC, :]
        s = _nt_dot(kk, qm)
        key0 = t * R + i * QC - WA
        rk = jax.lax.broadcasted_iota(jnp.int32, s.shape, 0)
        s = jnp.where(rk + key0 >= 0, s, NEG)
        mid = s[QC:WA]
        mrg = jnp.where(lower, s[WA:WA + QC], s[0:QC])
        m = jnp.maximum(jnp.max(mid, axis=0, keepdims=True), jnp.max(mrg, axis=0, keepdims=True))
        pm = jnp.exp2(mid - m)
        pg = jnp.exp2(mrg - m)
        l = jnp.sum(pm, axis=0, keepdims=True) + jnp.sum(pg, axis=0, keepdims=True)
        pgb = pg.astype(bf)
        first = jnp.where(lower, zeros64, pgb)
        last = jnp.where(lower, pgb, zeros64)
        parts = [first, pm.astype(bf), last]
        parts = ([zeros64] + parts) if (i % 2) else (parts + [zeros64])
        pt = jnp.concatenate(parts, axis=0)
        r0 = 40 * p - 8 * (p % 2)
        c0 = (i // 2) * 128
        vt = vta_ref[r0:r0 + 48, c0:c0 + 384]
        return _dot(vt, pt) * (1.0 / l)

    def unit_b(p, i):
        tix, off = _PAIR[p]
        qm = masked_q(qb_ref, tix, off, i)
        kk = kb_ref[tix, i * QC:i * QC + HB + QC, :]
        s = _nt_dot(kk, qm)
        key0 = t * R + i * QC - HB
        s = jnp.where(band_b & (rb + key0 >= 0), s, NEG)
        m = jnp.max(s, axis=0, keepdims=True)
        pr = jnp.exp2(s - m)
        l = jnp.sum(pr, axis=0, keepdims=True)
        pt = jnp.concatenate([pr.astype(bf), zeros48], axis=0)
        r0 = 40 * p - 8 * (p % 2)
        vt = vtb_ref[i, r0:r0 + 48, :]
        return _dot(vt, pt) * (1.0 / l)

    def attend(unit, wo_ref):
        for p in range(NPAIR):
            for mm in range(NCH // 2):
                r_e = unit(p, 2 * mm)
                r_o = unit(p, 2 * mm + 1)
                sh = 8 * (p % 2)
                h0 = (row48 - sh) < DH
                re_r = pltpu.roll(r_e, 64, 1)
                ro_r = pltpu.roll(r_o, 64, 1)
                tt = jnp.where(lane48 < 64, jnp.where(h0, r_e, re_r), jnp.where(h0, ro_r, r_o))
                ot_ref[40 * p:40 * p + 40, mm * 128:(mm + 1) * 128] = tt[sh:sh + 40]
        o = ot_ref[...].astype(bf).T
        return _dot(o, wo_ref[...])

    a = attend(unit_a, woa_ref)
    b = attend(unit_b, wob_ref)
    gl = jnp.sum(x.astype(jnp.float32) * gw_ref[...].astype(jnp.float32), axis=1, keepdims=True)
    g = jax.nn.sigmoid(gl)
    o_ref[...] = (g * a + (1.0 - g) * b).astype(o_ref.dtype)


@jax.jit
def pallas_gated_mix__sliding_block__sliding_local_dilated__prompt_kernel(
    A_x: jax.Array,
    A_wqkv: jax.Array,
    A_wo: jax.Array,
    B_x: jax.Array,
    B_wqkv: jax.Array,
    B_wo: jax.Array,
    gate_w: jax.Array,
):
    del B_x
    bf = jnp.bfloat16
    x = A_x.reshape(S, D)
    gw = gate_w.reshape(1, D)
    const = lambda shape: pl.BlockSpec(shape, lambda t: (0,) * len(shape))
    out = pl.pallas_call(
        kernel,
        grid=(S // R,),
        in_specs=[
            pl.BlockSpec((R, D), lambda t: (t, 0)),
            const((D, 3 * D)), const((D, D)), const((D, 3 * D)), const((D, D)), const((1, D)),
        ],
        out_specs=pl.BlockSpec((R, D), lambda t: (t, 0)),
        out_shape=jax.ShapeDtypeStruct((S, D), bf),
        scratch_shapes=[
            pltpu.VMEM((NT, R, 128), bf),
            pltpu.VMEM((NT, WA + R, 128), bf),
            pltpu.VMEM((D, WA + R), bf),
            pltpu.VMEM((NT, R, 128), bf),
            pltpu.VMEM((NT, HB + R, 128), bf),
            pltpu.VMEM((HB + R + 48, D), bf),
            pltpu.VMEM((NCH, D, 128), bf),
            pltpu.VMEM((D, R), jnp.float32),
        ],
        compiler_params=pltpu.CompilerParams(
            dimension_semantics=("arbitrary",),
            vmem_limit_bytes=100 * 1024 * 1024,
        ),
        name="gated_mix_attn",
    )(x, A_wqkv, A_wo, B_wqkv, B_wo, gw)
    return out.reshape(1, S, D)
```

```python
import jax
import jax.numpy as jnp
import numpy as np
import jax.experimental.pallas as pl
import jax.experimental.pallas.tpu as pltpu

S = 2048
D = 640
H = 32
DH = 20
R = 256
QC = 64
NCH = R // QC
NPAIR = H // 2
WA = 256
HB = 16
NEG = -1e30
LOG2E = 1.4426950408889634
QSCALE = float(DH ** -0.5) * LOG2E
BF = jnp.bfloat16


def _pair_tile(p):
    c0 = 40 * p
    t0, off = divmod(c0, 128)
    if off + 40 <= 128:
        return (t0, t0, 0), off
    return (t0, t0 + 1, off), off


_TILES = []
_PAIR = []
for _p in range(NPAIR):
    _t, _o = _pair_tile(_p)
    if _t not in _TILES:
        _TILES.append(_t)
    _PAIR.append((_TILES.index(_t), _o))
NT = len(_TILES)


def _u32(x):
    return pltpu.bitcast(x, jnp.uint32)


def _bf(x):
    return pltpu.bitcast(x, BF)


def _build_tiles(y):
    rows = y.shape[0]
    lane = jax.lax.broadcasted_iota(jnp.int32, (rows // 2, 128), 1)
    out = []
    for (a, b, split) in _TILES:
        ta = y[:, a * 128:(a + 1) * 128]
        if a == b:
            out.append(ta)
        else:
            tb = y[:, b * 128:(b + 1) * 128]
            out.append(_bf(jnp.where(lane >= split, _u32(ta), _u32(tb))))
    return out


def _nt_dot(a, b):
    return jax.lax.dot_general(a, b, (((1,), (1,)), ((), ())),
                               preferred_element_type=jnp.float32)


def _dot(a, b):
    return jnp.dot(a, b, preferred_element_type=jnp.float32)


def kernel(x_ref, wa_ref, woa_ref, wb_ref, wob_ref, gw_ref, o_ref,
           qa_ref, ka_ref, vta_ref, qb_ref, kb_ref, vb_ref, vtb_ref, ot_ref,
           s_ref, p_ref, l_ref):
    t = pl.program_id(0)
    x = x_ref[...]
    not_first = t > 0

    ka_ref[:, 0:WA, :] = _bf(jnp.where(not_first, _u32(ka_ref[:, R:R + WA, :]), jnp.uint32(0)))
    vta_ref[:, 0:WA] = _bf(jnp.where(not_first, _u32(vta_ref[:, R:R + WA]), jnp.uint32(0)))
    kb_ref[:, 0:HB, :] = _bf(jnp.where(not_first, _u32(kb_ref[:, R:R + HB, :]), jnp.uint32(0)))
    vb_ref[0:HB, :] = _bf(jnp.where(not_first, _u32(vb_ref[R:R + HB, :]), jnp.uint32(0)))
    vb_ref[HB + R:HB + R + 48, :] = jnp.zeros((48, D), BF)

    def proj(w_ref, q_ref, k_ref, koff):
        q = (_dot(x, w_ref[:, 0:D]) * QSCALE).astype(BF)
        for i, tl in enumerate(_build_tiles(q)):
            q_ref[i] = tl
        k = _dot(x, w_ref[:, D:2 * D]).astype(BF)
        for i, tl in enumerate(_build_tiles(k)):
            k_ref[i, koff:koff + R, :] = tl
        return _dot(x, w_ref[:, 2 * D:3 * D]).astype(BF)

    va = proj(wa_ref, qa_ref, ka_ref, WA)
    vta_ref[:, WA:WA + R] = va.T
    vb = proj(wb_ref, qb_ref, kb_ref, HB)
    vb_ref[HB:HB + R, :] = vb
    for i in range(NCH):
        vtb_ref[i] = vb_ref[i * QC:i * QC + 128, :].T

    lane128 = jax.lax.broadcasted_iota(jnp.int32, (QC, 128), 1)
    row64 = jax.lax.broadcasted_iota(jnp.int32, (QC, 128), 0)
    lower = row64 <= (lane128 & (QC - 1))
    lane32 = jax.lax.broadcasted_iota(jnp.int32, (QC // 2, 128), 1)
    rb = jax.lax.broadcasted_iota(jnp.int32, (QC + HB, 128), 0)
    jb = jax.lax.broadcasted_iota(jnp.int32, (QC + HB, 128), 1) & (QC - 1)
    db = jb + HB - rb
    band_b = (db >= 0) & (db < 16) & ((db & 1) == 0)
    band_b0 = band_b & ((rb >= HB) | not_first)
    row48 = jax.lax.broadcasted_iota(jnp.int32, (48, 128), 0)
    lane48 = jax.lax.broadcasted_iota(jnp.int32, (48, 128), 1)
    left = lane48 < 64

    def masked_q(q_ref, p, i):
        tix, off = _PAIR[p]
        qt = _u32(q_ref[tix, i * QC:(i + 1) * QC, :])
        rel = (lane32 - off) & 127
        ones = jnp.uint32(0xFFFFFFFF)
        m0 = jnp.where(rel < DH, ones, jnp.uint32(0))
        m1 = jnp.where((rel >= DH) & (rel < 2 * DH), ones, jnp.uint32(0))
        return _bf(jnp.concatenate([qt & m0, qt & m1], axis=0))

    def qk_a(sl, u, p, i):
        kk = ka_ref[_PAIR[p][0], i * QC:i * QC + WA + QC, :]
        s_ref[sl, u] = _nt_dot(kk, masked_q(qa_ref, p, i))

    def sm_a(sl, u, p, i):
        def chunk(c):
            v = s_ref[sl, u, c * QC:(c + 1) * QC, :]
            if c < NCH - i:
                v = jnp.where(not_first, v, NEG)
            return v
        mrg = jnp.where(lower, s_ref[sl, u, WA:WA + QC, :], chunk(0))
        mid = [chunk(c) for c in range(1, 4)]
        m = jnp.max(mrg, axis=0, keepdims=True)
        for v in mid:
            m = jnp.maximum(m, jnp.max(v, axis=0, keepdims=True))
        pg = jnp.exp2(mrg - m)
        l = jnp.sum(pg, axis=0, keepdims=True)
        o = QC * (i % 2)
        p_ref[sl, u, o:o + QC, :] = jnp.where(lower, 0.0, pg).astype(BF)
        p_ref[sl, u, o + WA:o + WA + QC, :] = jnp.where(lower, pg, 0.0).astype(BF)
        for c, v in enumerate(mid):
            pm = jnp.exp2(v - m)
            l = l + jnp.sum(pm, axis=0, keepdims=True)
            p_ref[sl, u, o + (c + 1) * QC:o + (c + 2) * QC, :] = pm.astype(BF)
        z = (WA + QC) if i % 2 == 0 else 0
        p_ref[sl, u, z:z + QC, :] = jnp.zeros((QC, 128), BF)
        l_ref[sl, u] = jnp.broadcast_to(1.0 / l, (8, 128))

    def pv_a(sl, u, p, i):
        r0 = 40 * p - 8 * (p % 2)
        c0 = (i // 2) * 128
        return _dot(vta_ref[r0:r0 + 48, c0:c0 + 384], p_ref[sl, u]) * l_ref[sl, u][0:1]

    def qk_b(sl, u, p, i):
        kk = kb_ref[_PAIR[p][0], i * QC:i * QC + HB + QC, :]
        s_ref[sl, u, 0:QC + HB, :] = _nt_dot(kk, masked_q(qb_ref, p, i))

    def sm_b(sl, u, p, i):
        s = jnp.where(band_b0 if i == 0 else band_b, s_ref[sl, u, 0:QC + HB, :], NEG)
        m = jnp.max(s, axis=0, keepdims=True)
        pr = jnp.exp2(s - m)
        l = jnp.sum(pr, axis=0, keepdims=True)
        p_ref[sl, u, 0:QC + HB, :] = pr.astype(BF)
        p_ref[sl, u, QC + HB:128, :] = jnp.zeros((48, 128), BF)
        l_ref[sl, u] = jnp.broadcast_to(1.0 / l, (8, 128))

    def pv_b(sl, u, p, i):
        r0 = 40 * p - 8 * (p % 2)
        return _dot(vtb_ref[i, r0:r0 + 48, :], p_ref[sl, u, 0:128, :]) * l_ref[sl, u][0:1]

    def put(p, mm, r_e, r_o):
        sh = 8 * (p % 2)
        h0 = (row48 - sh) < DH
        tt = jnp.where(left, jnp.where(h0, r_e, pltpu.roll(r_e, 64, 1)),
                       jnp.where(h0, pltpu.roll(r_o, 64, 1), r_o))
        ot_ref[40 * p:40 * p + 40, mm * 128:(mm + 1) * 128] = tt[sh:sh + 40]

    def attend(qk, sm, pv, wo_ref):
        for n in range(NPAIR + 2):
            res = {}
            for u in range(NCH):
                if n < NPAIR:
                    qk(n % 2, u, n, u)
                if 1 <= n <= NPAIR:
                    sm((n - 1) % 2, u, n - 1, u)
                if n >= 2:
                    res[u] = pv((n - 2) % 2, u, n - 2, u)
                    if u % 2:
                        put(n - 2, u // 2, res[u - 1], res[u])
        o = ot_ref[...].astype(BF).T
        return _dot(o, wo_ref[...])

    a = attend(qk_a, sm_a, pv_a, woa_ref)
    b = attend(qk_b, sm_b, pv_b, wob_ref)
    gl = jnp.sum(x.astype(jnp.float32) * gw_ref[...].astype(jnp.float32), axis=1, keepdims=True)
    g = jax.nn.sigmoid(gl)
    o_ref[...] = (g * a + (1.0 - g) * b).astype(o_ref.dtype)


@jax.jit
def pallas_gated_mix__sliding_block__sliding_local_dilated__prompt_kernel(
    A_x: jax.Array,
    A_wqkv: jax.Array,
    A_wo: jax.Array,
    B_x: jax.Array,
    B_wqkv: jax.Array,
    B_wo: jax.Array,
    gate_w: jax.Array,
):
    del B_x
    x = A_x.reshape(S, D)
    gw = gate_w.reshape(1, D)
    const = lambda shape: pl.BlockSpec(shape, lambda t: (0,) * len(shape))
    out = pl.pallas_call(
        kernel,
        grid=(S // R,),
        in_specs=[
            pl.BlockSpec((R, D), lambda t: (t, 0)),
            const((D, 3 * D)), const((D, D)), const((D, 3 * D)), const((D, D)), const((1, D)),
        ],
        out_specs=pl.BlockSpec((R, D), lambda t: (t, 0)),
        out_shape=jax.ShapeDtypeStruct((S, D), BF),
        scratch_shapes=[
            pltpu.VMEM((NT, R, 128), BF),
            pltpu.VMEM((NT, WA + R, 128), BF),
            pltpu.VMEM((D, WA + R), BF),
            pltpu.VMEM((NT, R, 128), BF),
            pltpu.VMEM((NT, HB + R, 128), BF),
            pltpu.VMEM((HB + R + 48, D), BF),
            pltpu.VMEM((NCH, D, 128), BF),
            pltpu.VMEM((D, R), jnp.float32),
            pltpu.VMEM((2, NCH, WA + QC, 128), jnp.float32),
            pltpu.VMEM((2, NCH, 384, 128), BF),
            pltpu.VMEM((2, NCH, 8, 128), jnp.float32),
        ],
        compiler_params=pltpu.CompilerParams(
            dimension_semantics=("arbitrary",),
            vmem_limit_bytes=100 * 1024 * 1024,
        ),
        name="gated_mix_attn",
    )(x, A_wqkv, A_wo, B_wqkv, B_wo, gw)
    return out.reshape(1, S, D)
```

```python
import jax
import jax.numpy as jnp
import numpy as np
import jax.experimental.pallas as pl
import jax.experimental.pallas.tpu as pltpu

S = 2048
D = 640
H = 32
DH = 20
R = 256
QC = 64
NCH = R // QC
NPAIR = H // 2
WA = 256
HB = 16
NEG = -1e30
LOG2E = 1.4426950408889634
QSCALE = float(DH ** -0.5) * LOG2E
BF = jnp.bfloat16
U32 = jnp.uint32


def _pair_tile(p):
    c0 = 40 * p
    t0, off = divmod(c0, 128)
    if off + 40 <= 128:
        return (t0, t0, 0), off
    return (t0, t0 + 1, off), off


_TILES = []
_PAIR = []
for _p in range(NPAIR):
    _t, _o = _pair_tile(_p)
    if _t not in _TILES:
        _TILES.append(_t)
    _PAIR.append((_TILES.index(_t), _o))
NT = len(_TILES)


def _u32(x):
    return pltpu.bitcast(x, jnp.uint32)


def _bf(x):
    return pltpu.bitcast(x, BF)


def _build_tiles(y):
    rows = y.shape[0]
    lane = jax.lax.broadcasted_iota(jnp.int32, (rows // 2, 128), 1)
    out = []
    for (a, b, split) in _TILES:
        ta = y[:, a * 128:(a + 1) * 128]
        if a == b:
            out.append(_u32(ta))
        else:
            tb = y[:, b * 128:(b + 1) * 128]
            out.append(jnp.where(lane >= split, _u32(ta), _u32(tb)))
    return out


def _nt_dot(a, b):
    return jax.lax.dot_general(a, b, (((1,), (1,)), ((), ())),
                               preferred_element_type=jnp.float32)


def _dot(a, b):
    return jnp.dot(a, b, preferred_element_type=jnp.float32)


def kernel(x_ref, wa_ref, woa_ref, wb_ref, wob_ref, gw_ref, o_ref,
           qa_ref, ka_ref, vta_ref, qb_ref, kb_ref, vb_ref, vtb_ref, ot_ref,
           s_ref, p_ref, l_ref):
    t = pl.program_id(0)
    x = x_ref[...]
    not_first = t > 0

    z32 = jnp.uint32(0)
    ka_ref[:, 0:WA // 2, :] = jnp.where(not_first, ka_ref[:, R // 2:(R + WA) // 2, :], z32)
    vta_ref[:, 0:WA] = jnp.where(not_first, vta_ref[:, R:R + WA], z32)
    kb_ref[:, 0:HB // 2, :] = jnp.where(not_first, kb_ref[:, R // 2:(R + HB) // 2, :], z32)
    vb_ref[0:HB // 2, :] = jnp.where(not_first, vb_ref[R // 2:(R + HB) // 2, :], z32)
    vb_ref[(HB + R) // 2:(HB + R + 48) // 2, :] = jnp.zeros((24, D), jnp.uint32)

    def proj(w_ref, q_ref, k_ref, koff):
        q = (_dot(x, w_ref[:, 0:D]) * QSCALE).astype(BF)
        for i, tl in enumerate(_build_tiles(q)):
            q_ref[i] = tl
        k = _dot(x, w_ref[:, D:2 * D]).astype(BF)
        for i, tl in enumerate(_build_tiles(k)):
            k_ref[i, koff // 2:(koff + R) // 2, :] = tl
        return _dot(x, w_ref[:, 2 * D:3 * D]).astype(BF)

    va = proj(wa_ref, qa_ref, ka_ref, WA)
    vta_ref[:, WA:WA + R] = _u32(va.T)
    vb = proj(wb_ref, qb_ref, kb_ref, HB)
    vb_ref[HB // 2:(HB + R) // 2, :] = _u32(vb)
    for i in range(NCH):
        vtb_ref[i] = _u32(_bf(vb_ref[i * QC // 2:i * QC // 2 + 64, :]).T)

    lane128 = jax.lax.broadcasted_iota(jnp.int32, (QC, 128), 1)
    row64 = jax.lax.broadcasted_iota(jnp.int32, (QC, 128), 0)
    lower = row64 <= (lane128 & (QC - 1))
    lane32 = jax.lax.broadcasted_iota(jnp.int32, (QC // 2, 128), 1)
    rb = jax.lax.broadcasted_iota(jnp.int32, (QC + HB, 128), 0)
    jb = jax.lax.broadcasted_iota(jnp.int32, (QC + HB, 128), 1) & (QC - 1)
    db = jb + HB - rb
    band_b = (db >= 0) & (db < 16) & ((db & 1) == 0)
    band_b0 = band_b & ((rb >= HB) | not_first)
    row48 = jax.lax.broadcasted_iota(jnp.int32, (48, 128), 0)
    lane48 = jax.lax.broadcasted_iota(jnp.int32, (48, 128), 1)
    left = lane48 < 64

    def masked_q(q_ref, p, i):
        tix, off = _PAIR[p]
        qt = q_ref[tix, i * QC // 2:(i + 1) * QC // 2, :]
        rel = (lane32 - off) & 127
        ones = jnp.uint32(0xFFFFFFFF)
        m0 = jnp.where(rel < DH, ones, jnp.uint32(0))
        m1 = jnp.where((rel >= DH) & (rel < 2 * DH), ones, jnp.uint32(0))
        return _bf(jnp.concatenate([qt & m0, qt & m1], axis=0))

    def qk_a(sl, u, p, i):
        kk = _bf(ka_ref[_PAIR[p][0], i * QC // 2:(i * QC + WA + QC) // 2, :])
        s_ref[sl, u] = _nt_dot(kk, masked_q(qa_ref, p, i))

    def sm_a(sl, u, p, i):
        def chunk(c):
            v = s_ref[sl, u, c * QC:(c + 1) * QC, :]
            if c < NCH - i:
                v = jnp.where(not_first, v, NEG)
            return v
        mrg = jnp.where(lower, s_ref[sl, u, WA:WA + QC, :], chunk(0))
        mid = [chunk(c) for c in range(1, 4)]
        m = jnp.max(mrg, axis=0, keepdims=True)
        for v in mid:
            m = jnp.maximum(m, jnp.max(v, axis=0, keepdims=True))
        pg = jnp.exp2(mrg - m)
        l = jnp.sum(pg, axis=0, keepdims=True)
        o = QC * (i % 2)
        p_ref[sl, u, o // 2:(o + QC) // 2, :] = _u32(jnp.where(lower, 0.0, pg).astype(BF))
        p_ref[sl, u, (o + WA) // 2:(o + WA + QC) // 2, :] = _u32(jnp.where(lower, pg, 0.0).astype(BF))
        for c, v in enumerate(mid):
            pm = jnp.exp2(v - m)
            l = l + jnp.sum(pm, axis=0, keepdims=True)
            p_ref[sl, u, (o + (c + 1) * QC) // 2:(o + (c + 2) * QC) // 2, :] = _u32(pm.astype(BF))
        z = (WA + QC) if i % 2 == 0 else 0
        p_ref[sl, u, z // 2:(z + QC) // 2, :] = jnp.zeros((QC // 2, 128), jnp.uint32)
        l_ref[sl, u] = jnp.broadcast_to(1.0 / l, (8, 128))

    def pv_a(sl, u, p, i):
        r0 = 40 * p - 8 * (p % 2)
        c0 = (i // 2) * 128
        return _dot(_bf(vta_ref[r0 // 2:r0 // 2 + 24, c0:c0 + 384]), _bf(p_ref[sl, u])) * l_ref[sl, u][0:1]

    def qk_b(sl, u, p, i):
        kk = _bf(kb_ref[_PAIR[p][0], i * QC // 2:(i * QC + HB + QC) // 2, :])
        s_ref[sl, u, 0:QC + HB, :] = _nt_dot(kk, masked_q(qb_ref, p, i))

    def sm_b(sl, u, p, i):
        s = jnp.where(band_b0 if i == 0 else band_b, s_ref[sl, u, 0:QC + HB, :], NEG)
        m = jnp.max(s, axis=0, keepdims=True)
        pr = jnp.exp2(s - m)
        l = jnp.sum(pr, axis=0, keepdims=True)
        p_ref[sl, u, 0:(QC + HB) // 2, :] = _u32(pr.astype(BF))
        p_ref[sl, u, (QC + HB) // 2:64, :] = jnp.zeros((24, 128), jnp.uint32)
        l_ref[sl, u] = jnp.broadcast_to(1.0 / l, (8, 128))

    def pv_b(sl, u, p, i):
        r0 = 40 * p - 8 * (p % 2)
        return _dot(_bf(vtb_ref[i, r0 // 2:r0 // 2 + 24, :]), _bf(p_ref[sl, u, 0:64, :])) * l_ref[sl, u][0:1]

    def put(p, mm, r_e, r_o):
        sh = 8 * (p % 2)
        h0 = (row48 - sh) < DH
        tt = jnp.where(left, jnp.where(h0, r_e, pltpu.roll(r_e, 64, 1)),
                       jnp.where(h0, pltpu.roll(r_o, 64, 1), r_o))
        ot_ref[40 * p:40 * p + 40, mm * 128:(mm + 1) * 128] = tt[sh:sh + 40]

    def attend(qk, sm, pv, wo_ref):
        for n in range(NPAIR + 2):
            res = {}
            for u in range(NCH):
                if n < NPAIR:
                    qk(n % 2, u, n, u)
                if 1 <= n <= NPAIR:
                    sm((n - 1) % 2, u, n - 1, u)
                if n >= 2:
                    res[u] = pv((n - 2) % 2, u, n - 2, u)
                    if u % 2:
                        put(n - 2, u // 2, res[u - 1], res[u])
        o = ot_ref[...].astype(BF).T
        return _dot(o, wo_ref[...])

    a = attend(qk_a, sm_a, pv_a, woa_ref)
    b = attend(qk_b, sm_b, pv_b, wob_ref)
    gl = jnp.sum(x.astype(jnp.float32) * gw_ref[...].astype(jnp.float32), axis=1, keepdims=True)
    g = jax.nn.sigmoid(gl)
    o_ref[...] = (g * a + (1.0 - g) * b).astype(o_ref.dtype)


@jax.jit
def pallas_gated_mix__sliding_block__sliding_local_dilated__prompt_kernel(
    A_x: jax.Array,
    A_wqkv: jax.Array,
    A_wo: jax.Array,
    B_x: jax.Array,
    B_wqkv: jax.Array,
    B_wo: jax.Array,
    gate_w: jax.Array,
):
    del B_x
    x = A_x.reshape(S, D)
    gw = gate_w.reshape(1, D)
    const = lambda shape: pl.BlockSpec(shape, lambda t: (0,) * len(shape))
    out = pl.pallas_call(
        kernel,
        grid=(S // R,),
        in_specs=[
            pl.BlockSpec((R, D), lambda t: (t, 0)),
            const((D, 3 * D)), const((D, D)), const((D, 3 * D)), const((D, D)), const((1, D)),
        ],
        out_specs=pl.BlockSpec((R, D), lambda t: (t, 0)),
        out_shape=jax.ShapeDtypeStruct((S, D), BF),
        scratch_shapes=[
            pltpu.VMEM((NT, R // 2, 128), U32),
            pltpu.VMEM((NT, (WA + R) // 2, 128), U32),
            pltpu.VMEM((D // 2, WA + R), U32),
            pltpu.VMEM((NT, R // 2, 128), U32),
            pltpu.VMEM((NT, (HB + R) // 2, 128), U32),
            pltpu.VMEM(((HB + R + 48) // 2, D), U32),
            pltpu.VMEM((NCH, D // 2, 128), U32),
            pltpu.VMEM((D, R), jnp.float32),
            pltpu.VMEM((2, NCH, WA + QC, 128), jnp.float32),
            pltpu.VMEM((2, NCH, 192, 128), U32),
            pltpu.VMEM((2, NCH, 8, 128), jnp.float32),
        ],
        compiler_params=pltpu.CompilerParams(
            dimension_semantics=("arbitrary",),
            vmem_limit_bytes=100 * 1024 * 1024,
        ),
        name="gated_mix_attn",
    )(x, A_wqkv, A_wo, B_wqkv, B_wo, gw)
    return out.reshape(1, S, D)
```

```python
import jax
import jax.numpy as jnp
import numpy as np
import jax.experimental.pallas as pl
import jax.experimental.pallas.tpu as pltpu

S = 2048
D = 640
H = 32
DH = 20
R = 256
QC = 64
NCH = R // QC
NPAIR = H // 2
WA = 256
HB = 16
NEG = -1e30
LOG2E = 1.4426950408889634
QSCALE = float(DH ** -0.5) * LOG2E
BF = jnp.bfloat16
U32 = jnp.uint32


def _pair_tile(p):
    c0 = 40 * p
    t0, off = divmod(c0, 128)
    if off + 40 <= 128:
        return (t0, t0, 0), off
    return (t0, t0 + 1, off), off


_TILES = []
_PAIR = []
for _p in range(NPAIR):
    _t, _o = _pair_tile(_p)
    if _t not in _TILES:
        _TILES.append(_t)
    _PAIR.append((_TILES.index(_t), _o))
NT = len(_TILES)


def _u32(x):
    return pltpu.bitcast(x, jnp.uint32)


def _bf(x):
    return pltpu.bitcast(x, BF)


def _build_tiles(y):
    rows = y.shape[0]
    lane = jax.lax.broadcasted_iota(jnp.int32, (rows // 2, 128), 1)
    out = []
    for (a, b, split) in _TILES:
        ta = y[:, a * 128:(a + 1) * 128]
        if a == b:
            out.append(_u32(ta))
        else:
            tb = y[:, b * 128:(b + 1) * 128]
            out.append(jnp.where(lane >= split, _u32(ta), _u32(tb)))
    return out


def _nt_dot(a, b):
    return jax.lax.dot_general(a, b, (((1,), (1,)), ((), ())),
                               preferred_element_type=jnp.float32)


def _dot(a, b):
    return jnp.dot(a, b, preferred_element_type=jnp.float32)


def kernel(x_ref, wa_ref, woa_ref, wb_ref, wob_ref, gw_ref, o_ref,
           qa_ref, ka_ref, vta_ref, qb_ref, kb_ref, vb_ref, vtb_ref, ot_ref,
           s_ref, p_ref, l_ref):
    t = pl.program_id(0)
    x = x_ref[...]
    not_first = t > 0
    pb_ref = p_ref.bitcast(BF)

    z32 = jnp.uint32(0)
    ka_ref[:, 0:WA // 2, :] = jnp.where(not_first, ka_ref[:, R // 2:(R + WA) // 2, :], z32)
    vta_ref[:, 0:WA] = jnp.where(not_first, vta_ref[:, R:R + WA], z32)
    kb_ref[:, 0:HB // 2, :] = jnp.where(not_first, kb_ref[:, R // 2:(R + HB) // 2, :], z32)
    vb_ref[0:HB // 2, :] = jnp.where(not_first, vb_ref[R // 2:(R + HB) // 2, :], z32)
    vb_ref[(HB + R) // 2:(HB + R + 48) // 2, :] = jnp.zeros((24, D), jnp.uint32)

    def proj(w_ref, q_ref, k_ref, koff):
        q = (_dot(x, w_ref[:, 0:D]) * QSCALE).astype(BF)
        for i, tl in enumerate(_build_tiles(q)):
            q_ref[i] = tl
        k = _dot(x, w_ref[:, D:2 * D]).astype(BF)
        for i, tl in enumerate(_build_tiles(k)):
            k_ref[i, koff // 2:(koff + R) // 2, :] = tl
        return _dot(x, w_ref[:, 2 * D:3 * D]).astype(BF)

    va = proj(wa_ref, qa_ref, ka_ref, WA)
    vta_ref[:, WA:WA + R] = _u32(va.T)
    vb = proj(wb_ref, qb_ref, kb_ref, HB)
    vb_ref[HB // 2:(HB + R) // 2, :] = _u32(vb)
    for i in range(NCH):
        vtb_ref[i] = _u32(_bf(vb_ref[i * QC // 2:i * QC // 2 + 64, :]).T)

    lane128 = jax.lax.broadcasted_iota(jnp.int32, (QC, 128), 1)
    row64 = jax.lax.broadcasted_iota(jnp.int32, (QC, 128), 0)
    lower = row64 <= (lane128 & (QC - 1))
    lane32 = jax.lax.broadcasted_iota(jnp.int32, (QC // 2, 128), 1)
    rb = jax.lax.broadcasted_iota(jnp.int32, (QC + HB, 128), 0)
    jb = jax.lax.broadcasted_iota(jnp.int32, (QC + HB, 128), 1) & (QC - 1)
    db = jb + HB - rb
    band_b = (db >= 0) & (db < 16) & ((db & 1) == 0)
    band_b0 = band_b & ((rb >= HB) | not_first)
    row48 = jax.lax.broadcasted_iota(jnp.int32, (48, 128), 0)
    lane48 = jax.lax.broadcasted_iota(jnp.int32, (48, 128), 1)
    left = lane48 < 64

    def masked_q(q_ref, p, i):
        tix, off = _PAIR[p]
        qt = q_ref[tix, i * QC // 2:(i + 1) * QC // 2, :]
        rel = (lane32 - off) & 127
        ones = jnp.uint32(0xFFFFFFFF)
        m0 = jnp.where(rel < DH, ones, jnp.uint32(0))
        m1 = jnp.where((rel >= DH) & (rel < 2 * DH), ones, jnp.uint32(0))
        return _bf(jnp.concatenate([qt & m0, qt & m1], axis=0))

    def qk_a(sl, u, p, i):
        kk = _bf(ka_ref[_PAIR[p][0], i * QC // 2:(i * QC + WA + QC) // 2, :])
        s_ref[sl, u] = _nt_dot(kk, masked_q(qa_ref, p, i))

    def sm_a(sl, u, p, i):
        def chunk(c):
            v = s_ref[sl, u, c * QC:(c + 1) * QC, :]
            if c < NCH - i:
                v = jnp.where(not_first, v, NEG)
            return v
        mrg = jnp.where(lower, s_ref[sl, u, WA:WA + QC, :], chunk(0))
        mid = [chunk(c) for c in range(1, 4)]
        m = jnp.max(mrg, axis=0, keepdims=True)
        for v in mid:
            m = jnp.maximum(m, jnp.max(v, axis=0, keepdims=True))
        pg = jnp.exp2(mrg - m)
        l = jnp.sum(pg, axis=0, keepdims=True)
        o = QC * (i % 2)
        pb_ref[sl, u, o:o + QC, :] = jnp.where(lower, 0.0, pg).astype(BF)
        pb_ref[sl, u, o + WA:o + WA + QC, :] = jnp.where(lower, pg, 0.0).astype(BF)
        for c, v in enumerate(mid):
            pm = jnp.exp2(v - m)
            l = l + jnp.sum(pm, axis=0, keepdims=True)
            pb_ref[sl, u, o + (c + 1) * QC:o + (c + 2) * QC, :] = pm.astype(BF)
        z = (WA + QC) if i % 2 == 0 else 0
        p_ref[sl, u, z // 2:(z + QC) // 2, :] = jnp.zeros((QC // 2, 128), jnp.uint32)
        l_ref[sl, u] = jnp.broadcast_to(1.0 / l, (8, 128))

    def pv_a(sl, u, p, i):
        r0 = 40 * p - 8 * (p % 2)
        c0 = (i // 2) * 128
        return _dot(_bf(vta_ref[r0 // 2:r0 // 2 + 24, c0:c0 + 384]), _bf(p_ref[sl, u])) * l_ref[sl, u][0:1]

    def qk_b(sl, u, p, i):
        kk = _bf(kb_ref[_PAIR[p][0], i * QC // 2:(i * QC + HB + QC) // 2, :])
        s_ref[sl, u, 0:QC + HB, :] = _nt_dot(kk, masked_q(qb_ref, p, i))

    def sm_b(sl, u, p, i):
        s = jnp.where(band_b0 if i == 0 else band_b, s_ref[sl, u, 0:QC + HB, :], NEG)
        m = jnp.max(s, axis=0, keepdims=True)
        pr = jnp.exp2(s - m)
        l = jnp.sum(pr, axis=0, keepdims=True)
        pb_ref[sl, u, 0:QC + HB, :] = pr.astype(BF)
        p_ref[sl, u, (QC + HB) // 2:64, :] = jnp.zeros((24, 128), jnp.uint32)
        l_ref[sl, u] = jnp.broadcast_to(1.0 / l, (8, 128))

    def pv_b(sl, u, p, i):
        r0 = 40 * p - 8 * (p % 2)
        return _dot(_bf(vtb_ref[i, r0 // 2:r0 // 2 + 24, :]), _bf(p_ref[sl, u, 0:64, :])) * l_ref[sl, u][0:1]

    def put(p, mm, r_e, r_o):
        sh = 8 * (p % 2)
        h0 = (row48 - sh) < DH
        tt = jnp.where(left, jnp.where(h0, r_e, pltpu.roll(r_e, 64, 1)),
                       jnp.where(h0, pltpu.roll(r_o, 64, 1), r_o))
        ot_ref[40 * p:40 * p + 40, mm * 128:(mm + 1) * 128] = tt[sh:sh + 40]

    def attend(qk, sm, pv, wo_ref):
        for n in range(NPAIR + 2):
            res = {}
            for u in range(NCH):
                if n < NPAIR:
                    qk(n % 2, u, n, u)
                if 1 <= n <= NPAIR:
                    sm((n - 1) % 2, u, n - 1, u)
                if n >= 2:
                    res[u] = pv((n - 2) % 2, u, n - 2, u)
                    if u % 2:
                        put(n - 2, u // 2, res[u - 1], res[u])
        o = ot_ref[...].astype(BF).T
        return _dot(o, wo_ref[...])

    a = attend(qk_a, sm_a, pv_a, woa_ref)
    b = attend(qk_b, sm_b, pv_b, wob_ref)
    gl = jnp.sum(x.astype(jnp.float32) * gw_ref[...].astype(jnp.float32), axis=1, keepdims=True)
    g = jax.nn.sigmoid(gl)
    o_ref[...] = (g * a + (1.0 - g) * b).astype(o_ref.dtype)


@jax.jit
def pallas_gated_mix__sliding_block__sliding_local_dilated__prompt_kernel(
    A_x: jax.Array,
    A_wqkv: jax.Array,
    A_wo: jax.Array,
    B_x: jax.Array,
    B_wqkv: jax.Array,
    B_wo: jax.Array,
    gate_w: jax.Array,
):
    del B_x
    x = A_x.reshape(S, D)
    gw = gate_w.reshape(1, D)
    const = lambda shape: pl.BlockSpec(shape, lambda t: (0,) * len(shape))
    out = pl.pallas_call(
        kernel,
        grid=(S // R,),
        in_specs=[
            pl.BlockSpec((R, D), lambda t: (t, 0)),
            const((D, 3 * D)), const((D, D)), const((D, 3 * D)), const((D, D)), const((1, D)),
        ],
        out_specs=pl.BlockSpec((R, D), lambda t: (t, 0)),
        out_shape=jax.ShapeDtypeStruct((S, D), BF),
        scratch_shapes=[
            pltpu.VMEM((NT, R // 2, 128), U32),
            pltpu.VMEM((NT, (WA + R) // 2, 128), U32),
            pltpu.VMEM((D // 2, WA + R), U32),
            pltpu.VMEM((NT, R // 2, 128), U32),
            pltpu.VMEM((NT, (HB + R) // 2, 128), U32),
            pltpu.VMEM(((HB + R + 48) // 2, D), U32),
            pltpu.VMEM((NCH, D // 2, 128), U32),
            pltpu.VMEM((D, R), jnp.float32),
            pltpu.VMEM((2, NCH, WA + QC, 128), jnp.float32),
            pltpu.VMEM((2, NCH, 192, 128), U32),
            pltpu.VMEM((2, NCH, 8, 128), jnp.float32),
        ],
        compiler_params=pltpu.CompilerParams(
            dimension_semantics=("arbitrary",),
            vmem_limit_bytes=100 * 1024 * 1024,
        ),
        name="gated_mix_attn",
    )(x, A_wqkv, A_wo, B_wqkv, B_wo, gw)
    return out.reshape(1, S, D)
```

```python
import jax
import jax.numpy as jnp
import numpy as np
import jax.experimental.pallas as pl
import jax.experimental.pallas.tpu as pltpu

S = 2048
D = 640
H = 32
DH = 20
R = 256
QC = 64
NCH = R // QC
NPAIR = H // 2
WA = 256
HB = 16
NEG = -1e30
LOG2E = 1.4426950408889634
QSCALE = float(DH ** -0.5) * LOG2E
BF = jnp.bfloat16
U32 = jnp.uint32


def _pair_tile(p):
    c0 = 40 * p
    t0, off = divmod(c0, 128)
    if off + 40 <= 128:
        return (t0, t0, 0), off
    return (t0, t0 + 1, off), off


_TILES = []
_PAIR = []
for _p in range(NPAIR):
    _t, _o = _pair_tile(_p)
    if _t not in _TILES:
        _TILES.append(_t)
    _PAIR.append((_TILES.index(_t), _o))
NT = len(_TILES)


def _u32(x):
    return pltpu.bitcast(x, jnp.uint32)


def _bf(x):
    return pltpu.bitcast(x, BF)


def _build_tiles(y):
    rows = y.shape[0]
    lane = jax.lax.broadcasted_iota(jnp.int32, (rows, 128), 1)
    out = []
    for (a, b, split) in _TILES:
        ta = y[:, a * 128:(a + 1) * 128]
        if a != b:
            ta = jnp.where(lane >= split, ta, y[:, b * 128:(b + 1) * 128])
        out.append(ta.astype(BF))
    return out


def _nt_dot(a, b):
    return jax.lax.dot_general(a, b, (((1,), (1,)), ((), ())),
                               preferred_element_type=jnp.float32)


def _dot(a, b):
    return jnp.dot(a, b, preferred_element_type=jnp.float32)


def kernel(x_ref, wa_ref, woa_ref, wb_ref, wob_ref, gw_ref, o_ref,
           qa_ref, ka_ref, vta_ref, qb_ref, kb_ref, vb_ref, vtb_ref, ot_ref,
           s_ref, p_ref, l_ref):
    t = pl.program_id(0)
    x = x_ref[...]
    not_first = t > 0
    row0 = pl.multiple_of(t * R, R)

    @pl.when(t == 0)
    def _():
        ka_ref[:, 0:WA, :] = jnp.zeros((NT, WA, 128), BF)
        for j in range(WA // 128):
            vta_ref[j] = jnp.zeros((D, 128), BF)
        kb_ref[:, 0:HB, :] = jnp.zeros((NT, HB, 128), BF)
        vb_ref[0:HB, :] = jnp.zeros((HB, D), BF)
        vb_ref[HB + S:HB + S + 48, :] = jnp.zeros((48, D), BF)

    def proj(w_ref, q_ref, k_ref, koff):
        q = _dot(x, w_ref[:, 0:D]) * QSCALE
        for i, tl in enumerate(_build_tiles(q)):
            q_ref[i] = tl
        k = _dot(x, w_ref[:, D:2 * D])
        for i, tl in enumerate(_build_tiles(k)):
            k_ref[i, pl.ds(row0 + koff, R), :] = tl
        return _dot(x, w_ref[:, 2 * D:3 * D]).astype(BF)

    va = proj(wa_ref, qa_ref, ka_ref, WA)
    for j in range(R // 128):
        vta_ref[t * (R // 128) + WA // 128 + j] = va[j * 128:(j + 1) * 128, :].T
    vb = proj(wb_ref, qb_ref, kb_ref, HB)
    vb_ref[pl.ds(row0 + HB, R), :] = vb
    for i in range(NCH):
        vtb_ref[i] = vb_ref[pl.ds(row0 + i * QC, 128), :].T

    lane128 = jax.lax.broadcasted_iota(jnp.int32, (QC, 128), 1)
    row64 = jax.lax.broadcasted_iota(jnp.int32, (QC, 128), 0)
    lower = row64 <= (lane128 & (QC - 1))
    lane32 = jax.lax.broadcasted_iota(jnp.int32, (QC // 2, 128), 1)
    rb = jax.lax.broadcasted_iota(jnp.int32, (QC + HB, 128), 0)
    jb = jax.lax.broadcasted_iota(jnp.int32, (QC + HB, 128), 1) & (QC - 1)
    db = jb + HB - rb
    band_b = (db >= 0) & (db < 16) & ((db & 1) == 0)
    band_b0 = band_b & ((rb >= HB) | not_first)
    row48 = jax.lax.broadcasted_iota(jnp.int32, (48, 128), 0)
    lane48 = jax.lax.broadcasted_iota(jnp.int32, (48, 128), 1)
    left = lane48 < 64

    def masked_q(q_ref, p, i):
        tix, off = _PAIR[p]
        qt = _u32(q_ref[tix, i * QC:(i + 1) * QC, :])
        rel = (lane32 - off) & 127
        ones = jnp.uint32(0xFFFFFFFF)
        m0 = jnp.where(rel < DH, ones, jnp.uint32(0))
        m1 = jnp.where((rel >= DH) & (rel < 2 * DH), ones, jnp.uint32(0))
        return _bf(jnp.concatenate([qt & m0, qt & m1], axis=0))

    def qk_a(sl, u, p, i):
        kk = ka_ref[_PAIR[p][0], pl.ds(row0 + i * QC, WA + QC), :]
        s_ref[sl, u] = _nt_dot(kk, masked_q(qa_ref, p, i))

    def sm_a(sl, u, p, i):
        def chunk(c):
            v = s_ref[sl, u, c * QC:(c + 1) * QC, :]
            if c < NCH - i:
                v = jnp.where(not_first, v, NEG)
            return v
        mrg = jnp.where(lower, s_ref[sl, u, WA:WA + QC, :], chunk(0))
        mid = [chunk(c) for c in range(1, 4)]
        m = jnp.max(mrg, axis=0, keepdims=True)
        for v in mid:
            m = jnp.maximum(m, jnp.max(v, axis=0, keepdims=True))
        pg = jnp.exp2(mrg - m)
        l = jnp.sum(pg, axis=0, keepdims=True)
        o = QC * (i % 2)
        p_ref[sl, u, o:o + QC, :] = jnp.where(lower, 0.0, pg).astype(BF)
        p_ref[sl, u, o + WA:o + WA + QC, :] = jnp.where(lower, pg, 0.0).astype(BF)
        for c, v in enumerate(mid):
            pm = jnp.exp2(v - m)
            l = l + jnp.sum(pm, axis=0, keepdims=True)
            p_ref[sl, u, o + (c + 1) * QC:o + (c + 2) * QC, :] = pm.astype(BF)
        z = (WA + QC) if i % 2 == 0 else 0
        p_ref[sl, u, z:z + QC, :] = jnp.zeros((QC, 128), BF)
        l_ref[sl, u] = jnp.broadcast_to(1.0 / l, (8, 128))

    def pv_a(sl, u, p, i):
        r0 = 40 * p - 8 * (p % 2)
        c0 = t * (R // 128) + i // 2
        acc = None
        for j in range(3):
            y = _dot(vta_ref[c0 + j, r0:r0 + 48, :], p_ref[sl, u, j * 128:(j + 1) * 128, :])
            acc = y if acc is None else acc + y
        return acc * l_ref[sl, u][0:1]

    def qk_b(sl, u, p, i):
        kk = kb_ref[_PAIR[p][0], pl.ds(row0 + i * QC, HB + QC), :]
        s_ref[sl, u, 0:QC + HB, :] = _nt_dot(kk, masked_q(qb_ref, p, i))

    def sm_b(sl, u, p, i):
        s = jnp.where(band_b0 if i == 0 else band_b, s_ref[sl, u, 0:QC + HB, :], NEG)
        m = jnp.max(s, axis=0, keepdims=True)
        pr = jnp.exp2(s - m)
        l = jnp.sum(pr, axis=0, keepdims=True)
        p_ref[sl, u, 0:QC + HB, :] = pr.astype(BF)
        p_ref[sl, u, QC + HB:128, :] = jnp.zeros((48, 128), BF)
        l_ref[sl, u] = jnp.broadcast_to(1.0 / l, (8, 128))

    def pv_b(sl, u, p, i):
        r0 = 40 * p - 8 * (p % 2)
        return _dot(vtb_ref[i, r0:r0 + 48, :], p_ref[sl, u, 0:128, :]) * l_ref[sl, u][0:1]

    def put(p, mm, r_e, r_o):
        sh = 8 * (p % 2)
        h0 = (row48 - sh) < DH
        tt = jnp.where(left, jnp.where(h0, r_e, pltpu.roll(r_e, 64, 1)),
                       jnp.where(h0, pltpu.roll(r_o, 64, 1), r_o))
        ot_ref[40 * p:40 * p + 40, mm * 128:(mm + 1) * 128] = tt[sh:sh + 40]

    def attend(qk, sm, pv, wo_ref):
        for n in range(NPAIR + 2):
            res = {}
            for u in range(NCH):
                if n < NPAIR:
                    qk(n % 2, u, n, u)
                if 1 <= n <= NPAIR:
                    sm((n - 1) % 2, u, n - 1, u)
                if n >= 2:
                    res[u] = pv((n - 2) % 2, u, n - 2, u)
                    if u % 2:
                        put(n - 2, u // 2, res[u - 1], res[u])
        o = ot_ref[...].astype(BF).T
        return _dot(o, wo_ref[...])

    a = attend(qk_a, sm_a, pv_a, woa_ref)
    b = attend(qk_b, sm_b, pv_b, wob_ref)
    gl = jnp.sum(x.astype(jnp.float32) * gw_ref[...].astype(jnp.float32), axis=1, keepdims=True)
    g = jax.nn.sigmoid(gl)
    o_ref[...] = (g * a + (1.0 - g) * b).astype(o_ref.dtype)


@jax.jit
def pallas_gated_mix__sliding_block__sliding_local_dilated__prompt_kernel(
    A_x: jax.Array,
    A_wqkv: jax.Array,
    A_wo: jax.Array,
    B_x: jax.Array,
    B_wqkv: jax.Array,
    B_wo: jax.Array,
    gate_w: jax.Array,
):
    del B_x
    x = A_x.reshape(S, D)
    gw = gate_w.reshape(1, D)
    const = lambda shape: pl.BlockSpec(shape, lambda t: (0,) * len(shape))
    out = pl.pallas_call(
        kernel,
        grid=(S // R,),
        in_specs=[
            pl.BlockSpec((R, D), lambda t: (t, 0)),
            const((D, 3 * D)), const((D, D)), const((D, 3 * D)), const((D, D)), const((1, D)),
        ],
        out_specs=pl.BlockSpec((R, D), lambda t: (t, 0)),
        out_shape=jax.ShapeDtypeStruct((S, D), BF),
        scratch_shapes=[
            pltpu.VMEM((NT, R, 128), BF),
            pltpu.VMEM((NT, WA + S, 128), BF),
            pltpu.VMEM(((WA + S) // 128, D, 128), BF),
            pltpu.VMEM((NT, R, 128), BF),
            pltpu.VMEM((NT, HB + S, 128), BF),
            pltpu.VMEM((HB + S + 48, D), BF),
            pltpu.VMEM((NCH, D, 128), BF),
            pltpu.VMEM((D, R), jnp.float32),
            pltpu.VMEM((2, NCH, WA + QC, 128), jnp.float32),
            pltpu.VMEM((2, NCH, 384, 128), BF),
            pltpu.VMEM((2, NCH, 8, 128), jnp.float32),
        ],
        compiler_params=pltpu.CompilerParams(
            dimension_semantics=("arbitrary",),
            vmem_limit_bytes=100 * 1024 * 1024,
        ),
        name="gated_mix_attn",
    )(x, A_wqkv, A_wo, B_wqkv, B_wo, gw)
    return out.reshape(1, S, D)
```

```python
import jax
import jax.numpy as jnp
import numpy as np
import jax.experimental.pallas as pl
import jax.experimental.pallas.tpu as pltpu

S = 2048
D = 640
H = 32
DH = 20
NLT = D // 128
R = 256
QC = 64
NCH = R // QC
NPAIR = H // 2
WA = 256
HB = 16
RB = 16
NEG = -1e30
LOG2E = 1.4426950408889634
QSCALE = float(DH ** -0.5) * LOG2E
BF = jnp.bfloat16
F32 = jnp.float32


def _pair_tile(p):
    c0 = 40 * p
    t0, off = divmod(c0, 128)
    if off + 40 <= 128:
        return (t0, t0, 0), off
    return (t0, t0 + 1, off), off


_TILES = []
_PAIR = []
for _p in range(NPAIR):
    _t, _o = _pair_tile(_p)
    if _t not in _TILES:
        _TILES.append(_t)
    _PAIR.append((_TILES.index(_t), _o))
NT = len(_TILES)


def _u32(x):
    return pltpu.bitcast(x, jnp.uint32)


def _bf(x):
    return pltpu.bitcast(x, BF)


def _build_tiles(y):
    rows = y.shape[0]
    lane = jax.lax.broadcasted_iota(jnp.int32, (rows, 128), 1)
    out = []
    for (a, b, split) in _TILES:
        ta = y[:, a * 128:(a + 1) * 128]
        if a != b:
            ta = jnp.where(lane >= split, ta, y[:, b * 128:(b + 1) * 128])
        out.append(ta.astype(BF))
    return out


def _nt_dot(a, b):
    return jax.lax.dot_general(a, b, (((1,), (1,)), ((), ())), preferred_element_type=F32)


def _dot(a, b):
    return jnp.dot(a, b, preferred_element_type=F32)


def kernel(x_ref, wa_ref, woa_ref, wb_ref, wob_ref, gw_ref, o_ref,
           qa_ref, ka_ref, vta_ref, ot_ref, s_ref, p_ref, l_ref,
           wbt_ref, wobp_ref, tmp_ref, qb_ref, kb_ref, vb_ref, ob_ref):
    t = pl.program_id(0)
    x = x_ref[...]
    not_first = t > 0
    row0 = pl.multiple_of(t * R, R)

    @pl.when(t == 0)
    def _():
        ka_ref[:, 0:WA, :] = jnp.zeros((NT, WA, 128), BF)
        for j in range(WA // 128):
            vta_ref[j] = jnp.zeros((D, 128), BF)
        kb_ref[:, 0:HB, :] = jnp.zeros((NLT, HB, 128), F32)
        vb_ref[:, 0:HB, :] = jnp.zeros((NLT, HB, 128), F32)
        for sec in range(3):
            for ct in range(NLT):
                for nt in range(NLT):
                    w = wb_ref[ct * 128:(ct + 1) * 128, sec * D + nt * 128:sec * D + (nt + 1) * 128]
                    tmp_ref[ct, nt * 128:(nt + 1) * 128, :] = w.astype(F32).T
            for ct in range(NLT):
                for d in range(DH):
                    wbt_ref[sec, d * H:(d + 1) * H, ct * 128:(ct + 1) * 128] = (
                        tmp_ref[ct, pl.ds(d, H, stride=DH), :].astype(BF))
        for nt in range(NLT):
            tmp_ref[nt] = wob_ref[:, nt * 128:(nt + 1) * 128].astype(F32)
        for nt in range(NLT):
            for d in range(DH):
                wobp_ref[d * H:(d + 1) * H, nt * 128:(nt + 1) * 128] = (
                    tmp_ref[nt, pl.ds(d, H, stride=DH), :].astype(BF))

    qb = _nt_dot(x, wbt_ref[0]) * QSCALE
    kb = _nt_dot(x, wbt_ref[1])
    vb = _nt_dot(x, wbt_ref[2])
    for c in range(NLT):
        qb_ref[c] = qb[:, c * 128:(c + 1) * 128]
        kb_ref[c, pl.ds(row0 + HB, R), :] = kb[:, c * 128:(c + 1) * 128]
        vb_ref[c, pl.ds(row0 + HB, R), :] = vb[:, c * 128:(c + 1) * 128]

    rowb = jax.lax.broadcasted_iota(jnp.int32, (RB, 128), 0)

    def attn_b(ci):
        r = ci * RB
        q = [qb_ref[c, r:r + RB, :] for c in range(NLT)]
        sc = []
        for j in range(8):
            acc = None
            for c in range(NLT):
                y = q[c] * kb_ref[c, pl.ds(row0 + (r + HB - 2 * j), RB), :]
                acc = y if acc is None else acc + y
            acc = acc + pltpu.roll(acc, 64, 1)
            acc = acc + pltpu.roll(acc, 32, 1)
            if r < 2 * j:
                acc = jnp.where(not_first | (rowb >= 2 * j - r), acc, NEG)
            sc.append(acc)
        m = sc[0]
        for y in sc[1:]:
            m = jnp.maximum(m, y)
        e = [jnp.exp2(y - m) for y in sc]
        l = e[0]
        for y in e[1:]:
            l = l + y
        inv = 1.0 / l
        for c in range(NLT):
            acc = None
            for j in range(8):
                y = e[j] * vb_ref[c, pl.ds(row0 + (r + HB - 2 * j), RB), :]
                acc = y if acc is None else acc + y
            ob_ref[r:r + RB, c * 128:(c + 1) * 128] = (acc * inv).astype(BF)

    nb = R // RB
    q = _dot(x, wa_ref[:, 0:D]) * QSCALE
    for i, tl in enumerate(_build_tiles(q)):
        qa_ref[i] = tl
    for ci in range(0, nb // 3):
        attn_b(ci)
    k = _dot(x, wa_ref[:, D:2 * D])
    for i, tl in enumerate(_build_tiles(k)):
        ka_ref[i, pl.ds(row0 + WA, R), :] = tl
    for ci in range(nb // 3, 2 * nb // 3):
        attn_b(ci)
    va = _dot(x, wa_ref[:, 2 * D:3 * D]).astype(BF)
    for j in range(R // 128):
        vta_ref[t * (R // 128) + WA // 128 + j] = va[j * 128:(j + 1) * 128, :].T
    for ci in range(2 * nb // 3, nb):
        attn_b(ci)

    lane128 = jax.lax.broadcasted_iota(jnp.int32, (QC, 128), 1)
    row64 = jax.lax.broadcasted_iota(jnp.int32, (QC, 128), 0)
    lower = row64 <= (lane128 & (QC - 1))
    lane32 = jax.lax.broadcasted_iota(jnp.int32, (QC // 2, 128), 1)
    row48 = jax.lax.broadcasted_iota(jnp.int32, (48, 128), 0)
    lane48 = jax.lax.broadcasted_iota(jnp.int32, (48, 128), 1)
    left = lane48 < 64

    def masked_q(p, i):
        tix, off = _PAIR[p]
        qt = _u32(qa_ref[tix, i * QC:(i + 1) * QC, :])
        rel = (lane32 - off) & 127
        ones = jnp.uint32(0xFFFFFFFF)
        m0 = jnp.where(rel < DH, ones, jnp.uint32(0))
        m1 = jnp.where((rel >= DH) & (rel < 2 * DH), ones, jnp.uint32(0))
        return _bf(jnp.concatenate([qt & m0, qt & m1], axis=0))

    def qk_a(sl, u, p, i):
        kk = ka_ref[_PAIR[p][0], pl.ds(row0 + i * QC, WA + QC), :]
        s_ref[sl, u] = _nt_dot(kk, masked_q(p, i))

    def sm_a(sl, u, p, i):
        def chunk(c):
            v = s_ref[sl, u, c * QC:(c + 1) * QC, :]
            if c < NCH - i:
                v = jnp.where(not_first, v, NEG)
            return v
        mrg = jnp.where(lower, s_ref[sl, u, WA:WA + QC, :], chunk(0))
        mid = [chunk(c) for c in range(1, 4)]
        m = jnp.max(mrg, axis=0, keepdims=True)
        for v in mid:
            m = jnp.maximum(m, jnp.max(v, axis=0, keepdims=True))
        pg = jnp.exp2(mrg - m)
        l = jnp.sum(pg, axis=0, keepdims=True)
        o = QC * (i % 2)
        p_ref[sl, u, o:o + QC, :] = jnp.where(lower, 0.0, pg).astype(BF)
        p_ref[sl, u, o + WA:o + WA + QC, :] = jnp.where(lower, pg, 0.0).astype(BF)
        for c, v in enumerate(mid):
            pm = jnp.exp2(v - m)
            l = l + jnp.sum(pm, axis=0, keepdims=True)
            p_ref[sl, u, o + (c + 1) * QC:o + (c + 2) * QC, :] = pm.astype(BF)
        z = (WA + QC) if i % 2 == 0 else 0
        p_ref[sl, u, z:z + QC, :] = jnp.zeros((QC, 128), BF)
        l_ref[sl, u] = jnp.broadcast_to(1.0 / l, (8, 128))

    def pv_a(sl, u, p, i):
        r0 = 40 * p - 8 * (p % 2)
        c0 = t * (R // 128) + i // 2
        acc = None
        for j in range(3):
            y = _dot(vta_ref[c0 + j, r0:r0 + 48, :], p_ref[sl, u, j * 128:(j + 1) * 128, :])
            acc = y if acc is None else acc + y
        return acc * l_ref[sl, u][0:1]

    def put(p, mm, r_e, r_o):
        sh = 8 * (p % 2)
        h0 = (row48 - sh) < DH
        tt = jnp.where(left, jnp.where(h0, r_e, pltpu.roll(r_e, 64, 1)),
                       jnp.where(h0, pltpu.roll(r_o, 64, 1), r_o))
        ot_ref[40 * p:40 * p + 40, mm * 128:(mm + 1) * 128] = tt[sh:sh + 40]

    for n in range(NPAIR + 2):
        res = {}
        for u in range(NCH):
            if n < NPAIR:
                qk_a(n % 2, u, n, u)
            if 1 <= n <= NPAIR:
                sm_a((n - 1) % 2, u, n - 1, u)
            if n >= 2:
                res[u] = pv_a((n - 2) % 2, u, n - 2, u)
                if u % 2:
                    put(n - 2, u // 2, res[u - 1], res[u])

    b = _dot(ob_ref[...], wobp_ref[...])
    a = _dot(ot_ref[...].astype(BF).T, woa_ref[...])
    gl = jnp.sum(x.astype(F32) * gw_ref[...].astype(F32), axis=1, keepdims=True)
    g = jax.nn.sigmoid(gl)
    o_ref[...] = (g * a + (1.0 - g) * b).astype(o_ref.dtype)


@jax.jit
def pallas_gated_mix__sliding_block__sliding_local_dilated__prompt_kernel(
    A_x: jax.Array,
    A_wqkv: jax.Array,
    A_wo: jax.Array,
    B_x: jax.Array,
    B_wqkv: jax.Array,
    B_wo: jax.Array,
    gate_w: jax.Array,
):
    del B_x
    x = A_x.reshape(S, D)
    gw = gate_w.reshape(1, D)
    const = lambda shape: pl.BlockSpec(shape, lambda t: (0,) * len(shape))
    out = pl.pallas_call(
        kernel,
        grid=(S // R,),
        in_specs=[
            pl.BlockSpec((R, D), lambda t: (t, 0)),
            const((D, 3 * D)), const((D, D)), const((D, 3 * D)), const((D, D)), const((1, D)),
        ],
        out_specs=pl.BlockSpec((R, D), lambda t: (t, 0)),
        out_shape=jax.ShapeDtypeStruct((S, D), BF),
        scratch_shapes=[
            pltpu.VMEM((NT, R, 128), BF),
            pltpu.VMEM((NT, WA + S, 128), BF),
            pltpu.VMEM(((WA + S) // 128, D, 128), BF),
            pltpu.VMEM((D, R), F32),
            pltpu.VMEM((2, NCH, WA + QC, 128), F32),
            pltpu.VMEM((2, NCH, 384, 128), BF),
            pltpu.VMEM((2, NCH, 8, 128), F32),
            pltpu.VMEM((3, D, D), BF),
            pltpu.VMEM((D, D), BF),
            pltpu.VMEM((NLT, D, 128), F32),
            pltpu.VMEM((NLT, R, 128), F32),
            pltpu.VMEM((NLT, HB + S, 128), F32),
            pltpu.VMEM((NLT, HB + S, 128), F32),
            pltpu.VMEM((R, D), BF),
        ],
        compiler_params=pltpu.CompilerParams(
            dimension_semantics=("arbitrary",),
            vmem_limit_bytes=100 * 1024 * 1024,
        ),
        name="gated_mix_attn",
    )(x, A_wqkv, A_wo, B_wqkv, B_wo, gw)
    return out.reshape(1, S, D)
```

```python
import jax
import jax.numpy as jnp
import numpy as np
import jax.experimental.pallas as pl
import jax.experimental.pallas.tpu as pltpu

S = 2048
D = 640
H = 32
DH = 20
NLT = D // 128
R = 256
QC = 64
NCH = R // QC
NPAIR = H // 2
WA = 256
HB = 16
RB = 16
NEG = -1e30
LOG2E = 1.4426950408889634
QSCALE = float(DH ** -0.5) * LOG2E
BF = jnp.bfloat16
F32 = jnp.float32


def _pair_tile(p):
    c0 = 40 * p
    t0, off = divmod(c0, 128)
    if off + 40 <= 128:
        return (t0, t0, 0), off
    return (t0, t0 + 1, off), off


_TILES = []
_PAIR = []
for _p in range(NPAIR):
    _t, _o = _pair_tile(_p)
    if _t not in _TILES:
        _TILES.append(_t)
    _PAIR.append((_TILES.index(_t), _o))
NT = len(_TILES)


def _u32(x):
    return pltpu.bitcast(x, jnp.uint32)


def _bf(x):
    return pltpu.bitcast(x, BF)


def _build_tiles(y):
    rows = y.shape[0]
    lane = jax.lax.broadcasted_iota(jnp.int32, (rows, 128), 1)
    out = []
    for (a, b, split) in _TILES:
        ta = y[:, a * 128:(a + 1) * 128]
        if a != b:
            ta = jnp.where(lane >= split, ta, y[:, b * 128:(b + 1) * 128])
        out.append(ta.astype(BF))
    return out


def _nt_dot(a, b):
    return jax.lax.dot_general(a, b, (((1,), (1,)), ((), ())), preferred_element_type=F32)


def _dot(a, b):
    return jnp.dot(a, b, preferred_element_type=F32)


def kernel(x_ref, wa_ref, woa_ref, wb_ref, wob_ref, gw_ref, o_ref,
           qa_ref, ka_ref, vta_ref, ot_ref, s_ref, p_ref, l_ref,
           wbt_ref, wobp_ref, tmp_ref, qb_ref, kb_ref, vb_ref, ob_ref, acc_ref):
    t = pl.program_id(0)
    x = x_ref[...]
    not_first = t > 0
    row0 = pl.multiple_of(t * R, R)

    @pl.when(t == 0)
    def _():
        ka_ref[:, 0:WA, :] = jnp.zeros((NT, WA, 128), BF)
        for j in range(WA // 128):
            vta_ref[j] = jnp.zeros((D, 128), BF)
        kb_ref[:, 0:HB, :] = jnp.zeros((NLT, HB, 128), F32)
        vb_ref[:, 0:HB, :] = jnp.zeros((NLT, HB, 128), F32)
        for sec in range(3):
            for ct in range(NLT):
                for nt in range(NLT):
                    w = wb_ref[ct * 128:(ct + 1) * 128, sec * D + nt * 128:sec * D + (nt + 1) * 128]
                    tmp_ref[ct, nt * 128:(nt + 1) * 128, :] = w.astype(F32).T
            for ct in range(NLT):
                for d in range(DH):
                    wbt_ref[sec, d * H:(d + 1) * H, ct * 128:(ct + 1) * 128] = (
                        tmp_ref[ct, pl.ds(d, H, stride=DH), :].astype(BF))
        for nt in range(NLT):
            tmp_ref[nt] = wob_ref[:, nt * 128:(nt + 1) * 128].astype(F32)
        for nt in range(NLT):
            for d in range(DH):
                wobp_ref[d * H:(d + 1) * H, nt * 128:(nt + 1) * 128] = (
                    tmp_ref[nt, pl.ds(d, H, stride=DH), :].astype(BF))

    qb = _nt_dot(x, wbt_ref[0]) * QSCALE
    kb = _nt_dot(x, wbt_ref[1])
    vb = _nt_dot(x, wbt_ref[2])
    for c in range(NLT):
        qb_ref[c] = qb[:, c * 128:(c + 1) * 128]
        kb_ref[c, pl.ds(row0 + HB, R), :] = kb[:, c * 128:(c + 1) * 128]
        vb_ref[c, pl.ds(row0 + HB, R), :] = vb[:, c * 128:(c + 1) * 128]

    rowb = jax.lax.broadcasted_iota(jnp.int32, (RB, 128), 0)

    def attn_b(ci):
        r = ci * RB
        q = [qb_ref[c, r:r + RB, :] for c in range(NLT)]
        sc = []
        for j in range(8):
            acc = None
            for c in range(NLT):
                y = q[c] * kb_ref[c, pl.ds(row0 + (r + HB - 2 * j), RB), :]
                acc = y if acc is None else acc + y
            acc = acc + pltpu.roll(acc, 64, 1)
            acc = acc + pltpu.roll(acc, 32, 1)
            if r < 2 * j:
                acc = jnp.where(not_first | (rowb >= 2 * j - r), acc, NEG)
            sc.append(acc)
        m = sc[0]
        for y in sc[1:]:
            m = jnp.maximum(m, y)
        e = [jnp.exp2(y - m) for y in sc]
        l = e[0]
        for y in e[1:]:
            l = l + y
        inv = 1.0 / l
        for c in range(NLT):
            acc = None
            for j in range(8):
                y = e[j] * vb_ref[c, pl.ds(row0 + (r + HB - 2 * j), RB), :]
                acc = y if acc is None else acc + y
            ob_ref[r:r + RB, c * 128:(c + 1) * 128] = (acc * inv).astype(BF)

    nb = R // RB
    q = _dot(x, wa_ref[:, 0:D]) * QSCALE
    for i, tl in enumerate(_build_tiles(q)):
        qa_ref[i] = tl
    for ci in range(0, nb // 3):
        attn_b(ci)
    k = _dot(x, wa_ref[:, D:2 * D])
    for i, tl in enumerate(_build_tiles(k)):
        ka_ref[i, pl.ds(row0 + WA, R), :] = tl
    for ci in range(nb // 3, 2 * nb // 3):
        attn_b(ci)
    va = _dot(x, wa_ref[:, 2 * D:3 * D]).astype(BF)
    for j in range(R // 128):
        vta_ref[t * (R // 128) + WA // 128 + j] = va[j * 128:(j + 1) * 128, :].T
    for ci in range(2 * nb // 3, nb):
        attn_b(ci)

    gl = jnp.sum(x.astype(F32) * gw_ref[...].astype(F32), axis=1, keepdims=True)
    g = jax.nn.sigmoid(gl)
    acc_ref[...] = (1.0 - g) * _dot(ob_ref[...], wobp_ref[...])

    lane128 = jax.lax.broadcasted_iota(jnp.int32, (QC, 128), 1)
    row64 = jax.lax.broadcasted_iota(jnp.int32, (QC, 128), 0)
    lower = row64 <= (lane128 & (QC - 1))
    lane32 = jax.lax.broadcasted_iota(jnp.int32, (QC // 2, 128), 1)
    row48 = jax.lax.broadcasted_iota(jnp.int32, (48, 128), 0)
    lane48 = jax.lax.broadcasted_iota(jnp.int32, (48, 128), 1)
    left = lane48 < 64

    def masked_q(p, i):
        tix, off = _PAIR[p]
        qt = _u32(qa_ref[tix, i * QC:(i + 1) * QC, :])
        rel = (lane32 - off) & 127
        ones = jnp.uint32(0xFFFFFFFF)
        m0 = jnp.where(rel < DH, ones, jnp.uint32(0))
        m1 = jnp.where((rel >= DH) & (rel < 2 * DH), ones, jnp.uint32(0))
        return _bf(jnp.concatenate([qt & m0, qt & m1], axis=0))

    def qk_a(sl, u, p, i):
        kk = ka_ref[_PAIR[p][0], pl.ds(row0 + i * QC, WA + QC), :]
        s_ref[sl, u] = _nt_dot(kk, masked_q(p, i))

    def sm_a(sl, u, p, i):
        def chunk(c):
            v = s_ref[sl, u, c * QC:(c + 1) * QC, :]
            if c < NCH - i:
                v = jnp.where(not_first, v, NEG)
            return v
        mrg = jnp.where(lower, s_ref[sl, u, WA:WA + QC, :], chunk(0))
        mid = [chunk(c) for c in range(1, 4)]
        m = jnp.max(mrg, axis=0, keepdims=True)
        for v in mid:
            m = jnp.maximum(m, jnp.max(v, axis=0, keepdims=True))
        pg = jnp.exp2(mrg - m)
        l = jnp.sum(pg, axis=0, keepdims=True)
        o = QC * (i % 2)
        p_ref[sl, u, o:o + QC, :] = jnp.where(lower, 0.0, pg).astype(BF)
        p_ref[sl, u, o + WA:o + WA + QC, :] = jnp.where(lower, pg, 0.0).astype(BF)
        for c, v in enumerate(mid):
            pm = jnp.exp2(v - m)
            l = l + jnp.sum(pm, axis=0, keepdims=True)
            p_ref[sl, u, o + (c + 1) * QC:o + (c + 2) * QC, :] = pm.astype(BF)
        z = (WA + QC) if i % 2 == 0 else 0
        p_ref[sl, u, z:z + QC, :] = jnp.zeros((QC, 128), BF)
        l_ref[sl, u] = jnp.broadcast_to(1.0 / l, (8, 128))

    def pv_a(sl, u, p, i):
        r0 = 40 * p - 8 * (p % 2)
        c0 = t * (R // 128) + i // 2
        acc = None
        for j in range(3):
            y = _dot(vta_ref[c0 + j, r0:r0 + 48, :], p_ref[sl, u, j * 128:(j + 1) * 128, :])
            acc = y if acc is None else acc + y
        return acc * l_ref[sl, u][0:1]

    def put(p, mm, r_e, r_o):
        sh = 8 * (p % 2)
        h0 = (row48 - sh) < DH
        tt = jnp.where(left, jnp.where(h0, r_e, pltpu.roll(r_e, 64, 1)),
                       jnp.where(h0, pltpu.roll(r_o, 64, 1), r_o))
        ot_ref[40 * p:40 * p + 40, mm * 128:(mm + 1) * 128] = tt[sh:sh + 40]

    for n in range(NPAIR + 2):
        res = {}
        for u in range(NCH):
            if n < NPAIR:
                qk_a(n % 2, u, n, u)
            if 1 <= n <= NPAIR:
                sm_a((n - 1) % 2, u, n - 1, u)
            if n >= 2:
                res[u] = pv_a((n - 2) % 2, u, n - 2, u)
                if u % 2:
                    put(n - 2, u // 2, res[u - 1], res[u])

    a = _dot(ot_ref[...].astype(BF).T, woa_ref[...])
    o_ref[...] = (g * a + acc_ref[...]).astype(o_ref.dtype)


@jax.jit
def pallas_gated_mix__sliding_block__sliding_local_dilated__prompt_kernel(
    A_x: jax.Array,
    A_wqkv: jax.Array,
    A_wo: jax.Array,
    B_x: jax.Array,
    B_wqkv: jax.Array,
    B_wo: jax.Array,
    gate_w: jax.Array,
):
    del B_x
    x = A_x.reshape(S, D)
    gw = gate_w.reshape(1, D)
    const = lambda shape: pl.BlockSpec(shape, lambda t: (0,) * len(shape))
    out = pl.pallas_call(
        kernel,
        grid=(S // R,),
        in_specs=[
            pl.BlockSpec((R, D), lambda t: (t, 0)),
            const((D, 3 * D)), const((D, D)), const((D, 3 * D)), const((D, D)), const((1, D)),
        ],
        out_specs=pl.BlockSpec((R, D), lambda t: (t, 0)),
        out_shape=jax.ShapeDtypeStruct((S, D), BF),
        scratch_shapes=[
            pltpu.VMEM((NT, R, 128), BF),
            pltpu.VMEM((NT, WA + S, 128), BF),
            pltpu.VMEM(((WA + S) // 128, D, 128), BF),
            pltpu.VMEM((D, R), F32),
            pltpu.VMEM((2, NCH, WA + QC, 128), F32),
            pltpu.VMEM((2, NCH, 384, 128), BF),
            pltpu.VMEM((2, NCH, 8, 128), F32),
            pltpu.VMEM((3, D, D), BF),
            pltpu.VMEM((D, D), BF),
            pltpu.VMEM((NLT, D, 128), F32),
            pltpu.VMEM((NLT, R, 128), F32),
            pltpu.VMEM((NLT, HB + S, 128), F32),
            pltpu.VMEM((NLT, HB + S, 128), F32),
            pltpu.VMEM((R, D), BF),
            pltpu.VMEM((R, D), F32),
        ],
        compiler_params=pltpu.CompilerParams(
            dimension_semantics=("arbitrary",),
            vmem_limit_bytes=100 * 1024 * 1024,
        ),
        name="gated_mix_attn",
    )(x, A_wqkv, A_wo, B_wqkv, B_wo, gw)
    return out.reshape(1, S, D)
```

```python
import jax
import jax.numpy as jnp
import numpy as np
import jax.experimental.pallas as pl
import jax.experimental.pallas.tpu as pltpu

S = 2048
D = 640
H = 32
DH = 20
NLT = D // 128
R = 256
QC = 64
NCH = R // QC
NPAIR = H // 2
WA = 256
HB = 16
RB = 16
NEG = -1e30
LOG2E = 1.4426950408889634
QSCALE = float(DH ** -0.5) * LOG2E
BF = jnp.bfloat16
F32 = jnp.float32


def _pair_tile(p):
    c0 = 40 * p
    t0, off = divmod(c0, 128)
    if off + 40 <= 128:
        return (t0, t0, 0), off
    return (t0, t0 + 1, off), off


_TILES = []
_PAIR = []
for _p in range(NPAIR):
    _t, _o = _pair_tile(_p)
    if _t not in _TILES:
        _TILES.append(_t)
    _PAIR.append((_TILES.index(_t), _o))
NT = len(_TILES)


def _u32(x):
    return pltpu.bitcast(x, jnp.uint32)


def _bf(x):
    return pltpu.bitcast(x, BF)


def _build_tiles(y):
    rows = y.shape[0]
    lane = jax.lax.broadcasted_iota(jnp.int32, (rows, 128), 1)
    out = []
    for (a, b, split) in _TILES:
        ta = y[:, a * 128:(a + 1) * 128]
        if a != b:
            ta = jnp.where(lane >= split, ta, y[:, b * 128:(b + 1) * 128])
        out.append(ta.astype(BF))
    return out


def _nt_dot(a, b):
    return jax.lax.dot_general(a, b, (((1,), (1,)), ((), ())), preferred_element_type=F32)


def _dot(a, b):
    return jnp.dot(a, b, preferred_element_type=F32)


def kernel(x_ref, wa_ref, woa_ref, wb_ref, wob_ref, gw_ref, o_ref,
           qa_ref, ka_ref, vta_ref, ot_ref, s_ref, p_ref, l_ref,
           wbt_ref, wobp_ref, tmp_ref, qb_ref, kb_ref, vb_ref, ob_ref, acc_ref):
    t = pl.program_id(0)
    x = x_ref[...]
    not_first = t > 0
    row0 = pl.multiple_of(t * R, R)

    @pl.when(t == 0)
    def _():
        ka_ref[:, 0:WA, :] = jnp.zeros((NT, WA, 128), BF)
        for j in range(WA // 128):
            vta_ref[j] = jnp.zeros((D, 128), BF)
        kb_ref[:, 0:HB, :] = jnp.zeros((NLT, HB, 128), F32)
        vb_ref[:, 0:HB, :] = jnp.zeros((NLT, HB, 128), F32)
        for sec in range(3):
            for ct in range(NLT):
                for nt in range(NLT):
                    w = wb_ref[ct * 128:(ct + 1) * 128, sec * D + nt * 128:sec * D + (nt + 1) * 128]
                    tmp_ref[ct, nt * 128:(nt + 1) * 128, :] = w.astype(F32).T
            for ct in range(NLT):
                for d in range(DH):
                    wbt_ref[sec, d * H:(d + 1) * H, ct * 128:(ct + 1) * 128] = (
                        tmp_ref[ct, pl.ds(d, H, stride=DH), :].astype(BF))
        for nt in range(NLT):
            tmp_ref[nt] = wob_ref[:, nt * 128:(nt + 1) * 128].astype(F32)
        for nt in range(NLT):
            for d in range(DH):
                wobp_ref[d * H:(d + 1) * H, nt * 128:(nt + 1) * 128] = (
                    tmp_ref[nt, pl.ds(d, H, stride=DH), :].astype(BF))

    @pl.when(t >= 0)
    def _():
        qb = _nt_dot(x, wbt_ref[0]) * QSCALE
        kb = _nt_dot(x, wbt_ref[1])
        vb = _nt_dot(x, wbt_ref[2])
        for c in range(NLT):
            qb_ref[c] = qb[:, c * 128:(c + 1) * 128]
            kb_ref[c, pl.ds(row0 + HB, R), :] = kb[:, c * 128:(c + 1) * 128]
            vb_ref[c, pl.ds(row0 + HB, R), :] = vb[:, c * 128:(c + 1) * 128]

    rowb = jax.lax.broadcasted_iota(jnp.int32, (RB, 128), 0)

    def attn_b(ci):
        r = ci * RB
        q = [qb_ref[c, r:r + RB, :] for c in range(NLT)]
        sc = []
        for j in range(8):
            acc = None
            for c in range(NLT):
                y = q[c] * kb_ref[c, pl.ds(row0 + (r + HB - 2 * j), RB), :]
                acc = y if acc is None else acc + y
            acc = acc + pltpu.roll(acc, 64, 1)
            acc = acc + pltpu.roll(acc, 32, 1)
            if r < 2 * j:
                acc = jnp.where(not_first | (rowb >= 2 * j - r), acc, NEG)
            sc.append(acc)
        m = sc[0]
        for y in sc[1:]:
            m = jnp.maximum(m, y)
        e = [jnp.exp2(y - m) for y in sc]
        l = e[0]
        for y in e[1:]:
            l = l + y
        inv = 1.0 / l
        for c in range(NLT):
            acc = None
            for j in range(8):
                y = e[j] * vb_ref[c, pl.ds(row0 + (r + HB - 2 * j), RB), :]
                acc = y if acc is None else acc + y
            ob_ref[r:r + RB, c * 128:(c + 1) * 128] = (acc * inv).astype(BF)

    nb = R // RB
    q = _dot(x, wa_ref[:, 0:D]) * QSCALE
    for i, tl in enumerate(_build_tiles(q)):
        qa_ref[i] = tl
    for ci in range(0, nb // 3):
        attn_b(ci)
    k = _dot(x, wa_ref[:, D:2 * D])
    for i, tl in enumerate(_build_tiles(k)):
        ka_ref[i, pl.ds(row0 + WA, R), :] = tl
    for ci in range(nb // 3, 2 * nb // 3):
        attn_b(ci)
    va = _dot(x, wa_ref[:, 2 * D:3 * D]).astype(BF)
    for j in range(R // 128):
        vta_ref[t * (R // 128) + WA // 128 + j] = va[j * 128:(j + 1) * 128, :].T
    for ci in range(2 * nb // 3, nb):
        attn_b(ci)

    gl = jnp.sum(x.astype(F32) * gw_ref[...].astype(F32), axis=1, keepdims=True)
    g = jax.nn.sigmoid(gl)
    acc_ref[...] = (1.0 - g) * _dot(ob_ref[...], wobp_ref[...])

    lane128 = jax.lax.broadcasted_iota(jnp.int32, (QC, 128), 1)
    row64 = jax.lax.broadcasted_iota(jnp.int32, (QC, 128), 0)
    lower = row64 <= (lane128 & (QC - 1))
    lane32 = jax.lax.broadcasted_iota(jnp.int32, (QC // 2, 128), 1)
    row48 = jax.lax.broadcasted_iota(jnp.int32, (48, 128), 0)
    lane48 = jax.lax.broadcasted_iota(jnp.int32, (48, 128), 1)
    left = lane48 < 64

    def masked_q(p, i):
        tix, off = _PAIR[p]
        qt = _u32(qa_ref[tix, i * QC:(i + 1) * QC, :])
        rel = (lane32 - off) & 127
        ones = jnp.uint32(0xFFFFFFFF)
        m0 = jnp.where(rel < DH, ones, jnp.uint32(0))
        m1 = jnp.where((rel >= DH) & (rel < 2 * DH), ones, jnp.uint32(0))
        return _bf(jnp.concatenate([qt & m0, qt & m1], axis=0))

    def qk_a(sl, u, p, i):
        kk = ka_ref[_PAIR[p][0], pl.ds(row0 + i * QC, WA + QC), :]
        s_ref[sl, u] = _nt_dot(kk, masked_q(p, i))

    def sm_a(sl, u, p, i):
        def chunk(c):
            v = s_ref[sl, u, c * QC:(c + 1) * QC, :]
            if c < NCH - i:
                v = jnp.where(not_first, v, NEG)
            return v
        mrg = jnp.where(lower, s_ref[sl, u, WA:WA + QC, :], chunk(0))
        mid = [chunk(c) for c in range(1, 4)]
        m = jnp.max(mrg, axis=0, keepdims=True)
        for v in mid:
            m = jnp.maximum(m, jnp.max(v, axis=0, keepdims=True))
        pg = jnp.exp2(mrg - m)
        l = jnp.sum(pg, axis=0, keepdims=True)
        o = QC * (i % 2)
        p_ref[sl, u, o:o + QC, :] = jnp.where(lower, 0.0, pg).astype(BF)
        p_ref[sl, u, o + WA:o + WA + QC, :] = jnp.where(lower, pg, 0.0).astype(BF)
        for c, v in enumerate(mid):
            pm = jnp.exp2(v - m)
            l = l + jnp.sum(pm, axis=0, keepdims=True)
            p_ref[sl, u, o + (c + 1) * QC:o + (c + 2) * QC, :] = pm.astype(BF)
        z = (WA + QC) if i % 2 == 0 else 0
        p_ref[sl, u, z:z + QC, :] = jnp.zeros((QC, 128), BF)
        l_ref[sl, u] = jnp.broadcast_to(1.0 / l, (8, 128))

    def pv_a(sl, u, p, i):
        r0 = 40 * p - 8 * (p % 2)
        c0 = t * (R // 128) + i // 2
        acc = None
        for j in range(3):
            y = _dot(vta_ref[c0 + j, r0:r0 + 48, :], p_ref[sl, u, j * 128:(j + 1) * 128, :])
            acc = y if acc is None else acc + y
        return acc * l_ref[sl, u][0:1]

    def put(p, mm, r_e, r_o):
        sh = 8 * (p % 2)
        h0 = (row48 - sh) < DH
        tt = jnp.where(left, jnp.where(h0, r_e, pltpu.roll(r_e, 64, 1)),
                       jnp.where(h0, pltpu.roll(r_o, 64, 1), r_o))
        ot_ref[40 * p:40 * p + 40, mm * 128:(mm + 1) * 128] = tt[sh:sh + 40]

    for n in range(NPAIR + 2):
        res = {}
        for u in range(NCH):
            if n < NPAIR:
                qk_a(n % 2, u, n, u)
            if 1 <= n <= NPAIR:
                sm_a((n - 1) % 2, u, n - 1, u)
            if n >= 2:
                res[u] = pv_a((n - 2) % 2, u, n - 2, u)
                if u % 2:
                    put(n - 2, u // 2, res[u - 1], res[u])

    a = _dot(ot_ref[...].astype(BF).T, woa_ref[...])
    o_ref[...] = (g * a + acc_ref[...]).astype(o_ref.dtype)


@jax.jit
def pallas_gated_mix__sliding_block__sliding_local_dilated__prompt_kernel(
    A_x: jax.Array,
    A_wqkv: jax.Array,
    A_wo: jax.Array,
    B_x: jax.Array,
    B_wqkv: jax.Array,
    B_wo: jax.Array,
    gate_w: jax.Array,
):
    del B_x
    x = A_x.reshape(S, D)
    gw = gate_w.reshape(1, D)
    const = lambda shape: pl.BlockSpec(shape, lambda t: (0,) * len(shape))
    out = pl.pallas_call(
        kernel,
        grid=(S // R,),
        in_specs=[
            pl.BlockSpec((R, D), lambda t: (t, 0)),
            const((D, 3 * D)), const((D, D)), const((D, 3 * D)), const((D, D)), const((1, D)),
        ],
        out_specs=pl.BlockSpec((R, D), lambda t: (t, 0)),
        out_shape=jax.ShapeDtypeStruct((S, D), BF),
        scratch_shapes=[
            pltpu.VMEM((NT, R, 128), BF),
            pltpu.VMEM((NT, WA + S, 128), BF),
            pltpu.VMEM(((WA + S) // 128, D, 128), BF),
            pltpu.VMEM((D, R), F32),
            pltpu.VMEM((2, NCH, WA + QC, 128), F32),
            pltpu.VMEM((2, NCH, 384, 128), BF),
            pltpu.VMEM((2, NCH, 8, 128), F32),
            pltpu.VMEM((3, D, D), BF),
            pltpu.VMEM((D, D), BF),
            pltpu.VMEM((NLT, D, 128), F32),
            pltpu.VMEM((NLT, R, 128), F32),
            pltpu.VMEM((NLT, HB + S, 128), F32),
            pltpu.VMEM((NLT, HB + S, 128), F32),
            pltpu.VMEM((R, D), BF),
            pltpu.VMEM((R, D), F32),
        ],
        compiler_params=pltpu.CompilerParams(
            dimension_semantics=("arbitrary",),
            vmem_limit_bytes=100 * 1024 * 1024,
        ),
        name="gated_mix_attn",
    )(x, A_wqkv, A_wo, B_wqkv, B_wo, gw)
    return out.reshape(1, S, D)
```

```python
import jax
import jax.numpy as jnp
import numpy as np
import jax.experimental.pallas as pl
import jax.experimental.pallas.tpu as pltpu

S = 2048
D = 640
H = 32
DH = 20
NLT = D // 128
R = 256
QC = 64
NCH = R // QC
NPAIR = H // 2
WA = 256
HB = 16
RB = 16
LINK = 1
NEG = -1e30
LOG2E = 1.4426950408889634
QSCALE = float(DH ** -0.5) * LOG2E
BF = jnp.bfloat16
F32 = jnp.float32


def _pair_tile(p):
    c0 = 40 * p
    t0, off = divmod(c0, 128)
    if off + 40 <= 128:
        return (t0, t0, 0), off
    return (t0, t0 + 1, off), off


_TILES = []
_PAIR = []
for _p in range(NPAIR):
    _t, _o = _pair_tile(_p)
    if _t not in _TILES:
        _TILES.append(_t)
    _PAIR.append((_TILES.index(_t), _o))
NT = len(_TILES)


def _u32(x):
    return pltpu.bitcast(x, jnp.uint32)


def _bf(x):
    return pltpu.bitcast(x, BF)


def _build_tiles(y):
    rows = y.shape[0]
    lane = jax.lax.broadcasted_iota(jnp.int32, (rows, 128), 1)
    out = []
    for (a, b, split) in _TILES:
        ta = y[:, a * 128:(a + 1) * 128]
        if a != b:
            ta = jnp.where(lane >= split, ta, y[:, b * 128:(b + 1) * 128])
        out.append(ta.astype(BF))
    return out


def _nt_dot(a, b):
    return jax.lax.dot_general(a, b, (((1,), (1,)), ((), ())), preferred_element_type=F32)


def _dot(a, b):
    return jnp.dot(a, b, preferred_element_type=F32)


def kernel(x_ref, wa_ref, woa_ref, wb_ref, wob_ref, gw_ref, o_ref,
           qa_ref, ka_ref, vta_ref, ot_ref, s_ref, p_ref, l_ref,
           wbt_ref, wobp_ref, tmp_ref, qb_ref, kb_ref, vb_ref, ob_ref, acc_ref):
    t = pl.program_id(0)
    x = x_ref[...]
    not_first = t > 0
    row0 = pl.multiple_of(t * R, R)

    @pl.when(t == 0)
    def _():
        ka_ref[:, 0:WA, :] = jnp.zeros((NT, WA, 128), BF)
        for j in range(WA // 128):
            vta_ref[j] = jnp.zeros((D, 128), BF)
        kb_ref[:, 0:HB, :] = jnp.zeros((NLT, HB, 128), F32)
        vb_ref[:, 0:HB, :] = jnp.zeros((NLT, HB, 128), F32)
        for sec in range(3):
            for ct in range(NLT):
                for nt in range(NLT):
                    w = wb_ref[ct * 128:(ct + 1) * 128, sec * D + nt * 128:sec * D + (nt + 1) * 128]
                    tmp_ref[ct, nt * 128:(nt + 1) * 128, :] = w.astype(F32).T
            for ct in range(NLT):
                for d in range(DH):
                    wbt_ref[sec, d * H:(d + 1) * H, ct * 128:(ct + 1) * 128] = (
                        tmp_ref[ct, pl.ds(d, H, stride=DH), :].astype(BF))
        for nt in range(NLT):
            tmp_ref[nt] = wob_ref[:, nt * 128:(nt + 1) * 128].astype(F32)
        for nt in range(NLT):
            for d in range(DH):
                wobp_ref[d * H:(d + 1) * H, nt * 128:(nt + 1) * 128] = (
                    tmp_ref[nt, pl.ds(d, H, stride=DH), :].astype(BF))

    @pl.when(t >= 0)
    def _():
        qb = _nt_dot(x, wbt_ref[0]) * QSCALE
        kb = _nt_dot(x, wbt_ref[1])
        vb = _nt_dot(x, wbt_ref[2])
        for c in range(NLT):
            qb_ref[c] = qb[:, c * 128:(c + 1) * 128]
            kb_ref[c, pl.ds(row0 + HB, R), :] = kb[:, c * 128:(c + 1) * 128]
            vb_ref[c, pl.ds(row0 + HB, R), :] = vb[:, c * 128:(c + 1) * 128]

    rowb = jax.lax.broadcasted_iota(jnp.int32, (RB, 128), 0)

    never = t < 0
    chain = [None, None]

    def attn_b(ci):
        r = ci * RB
        q = [qb_ref[c, r:r + RB, :] for c in range(NLT)]
        if chain[ci % LINK] is not None:
            q[0] = jnp.where(never, chain[ci % LINK], q[0])
            q[NLT - 1] = jnp.where(never, chain[ci % LINK], q[NLT - 1])
        sc = []
        for j in range(8):
            acc = None
            for c in range(NLT):
                y = q[c] * kb_ref[c, pl.ds(row0 + (r + HB - 2 * j), RB), :]
                acc = y if acc is None else acc + y
            acc = acc + pltpu.roll(acc, 64, 1)
            acc = acc + pltpu.roll(acc, 32, 1)
            if r < 2 * j:
                acc = jnp.where(not_first | (rowb >= 2 * j - r), acc, NEG)
            sc.append(acc)
        m = sc[0]
        for y in sc[1:]:
            m = jnp.maximum(m, y)
        e = [jnp.exp2(y - m) for y in sc]
        l = e[0]
        for y in e[1:]:
            l = l + y
        inv = 1.0 / l
        for c in range(NLT):
            acc = None
            for j in range(8):
                y = e[j] * vb_ref[c, pl.ds(row0 + (r + HB - 2 * j), RB), :]
                acc = y if acc is None else acc + y
            ob_ref[r:r + RB, c * 128:(c + 1) * 128] = (acc * inv).astype(BF)
        chain[ci % LINK] = acc

    nb = R // RB
    q = _dot(x, wa_ref[:, 0:D]) * QSCALE
    for i, tl in enumerate(_build_tiles(q)):
        qa_ref[i] = tl
    for ci in range(0, nb // 3):
        attn_b(ci)
    k = _dot(x, wa_ref[:, D:2 * D])
    for i, tl in enumerate(_build_tiles(k)):
        ka_ref[i, pl.ds(row0 + WA, R), :] = tl
    for ci in range(nb // 3, 2 * nb // 3):
        attn_b(ci)
    va = _dot(x, wa_ref[:, 2 * D:3 * D]).astype(BF)
    for j in range(R // 128):
        vta_ref[t * (R // 128) + WA // 128 + j] = va[j * 128:(j + 1) * 128, :].T
    for ci in range(2 * nb // 3, nb):
        attn_b(ci)

    gl = jnp.sum(x.astype(F32) * gw_ref[...].astype(F32), axis=1, keepdims=True)
    g = jax.nn.sigmoid(gl)
    acc_ref[...] = (1.0 - g) * _dot(ob_ref[...], wobp_ref[...])

    lane128 = jax.lax.broadcasted_iota(jnp.int32, (QC, 128), 1)
    row64 = jax.lax.broadcasted_iota(jnp.int32, (QC, 128), 0)
    lower = row64 <= (lane128 & (QC - 1))
    lane32 = jax.lax.broadcasted_iota(jnp.int32, (QC // 2, 128), 1)
    row48 = jax.lax.broadcasted_iota(jnp.int32, (48, 128), 0)
    lane48 = jax.lax.broadcasted_iota(jnp.int32, (48, 128), 1)
    left = lane48 < 64

    def masked_q(p, i):
        tix, off = _PAIR[p]
        qt = _u32(qa_ref[tix, i * QC:(i + 1) * QC, :])
        rel = (lane32 - off) & 127
        ones = jnp.uint32(0xFFFFFFFF)
        m0 = jnp.where(rel < DH, ones, jnp.uint32(0))
        m1 = jnp.where((rel >= DH) & (rel < 2 * DH), ones, jnp.uint32(0))
        return _bf(jnp.concatenate([qt & m0, qt & m1], axis=0))

    def qk_a(sl, u, p, i):
        kk = ka_ref[_PAIR[p][0], pl.ds(row0 + i * QC, WA + QC), :]
        s_ref[sl, u] = _nt_dot(kk, masked_q(p, i))

    def sm_a(sl, u, p, i):
        def chunk(c):
            v = s_ref[sl, u, c * QC:(c + 1) * QC, :]
            if c < NCH - i:
                v = jnp.where(not_first, v, NEG)
            return v
        mrg = jnp.where(lower, s_ref[sl, u, WA:WA + QC, :], chunk(0))
        mid = [chunk(c) for c in range(1, 4)]
        m = jnp.max(mrg, axis=0, keepdims=True)
        for v in mid:
            m = jnp.maximum(m, jnp.max(v, axis=0, keepdims=True))
        pg = jnp.exp2(mrg - m)
        l = jnp.sum(pg, axis=0, keepdims=True)
        o = QC * (i % 2)
        p_ref[sl, u, o:o + QC, :] = jnp.where(lower, 0.0, pg).astype(BF)
        p_ref[sl, u, o + WA:o + WA + QC, :] = jnp.where(lower, pg, 0.0).astype(BF)
        for c, v in enumerate(mid):
            pm = jnp.exp2(v - m)
            l = l + jnp.sum(pm, axis=0, keepdims=True)
            p_ref[sl, u, o + (c + 1) * QC:o + (c + 2) * QC, :] = pm.astype(BF)
        z = (WA + QC) if i % 2 == 0 else 0
        p_ref[sl, u, z:z + QC, :] = jnp.zeros((QC, 128), BF)
        l_ref[sl, u] = jnp.broadcast_to(1.0 / l, (8, 128))

    def pv_a(sl, u, p, i):
        r0 = 40 * p - 8 * (p % 2)
        c0 = t * (R // 128) + i // 2
        acc = None
        for j in range(3):
            y = _dot(vta_ref[c0 + j, r0:r0 + 48, :], p_ref[sl, u, j * 128:(j + 1) * 128, :])
            acc = y if acc is None else acc + y
        return acc * l_ref[sl, u][0:1]

    def put(p, mm, r_e, r_o):
        sh = 8 * (p % 2)
        h0 = (row48 - sh) < DH
        tt = jnp.where(left, jnp.where(h0, r_e, pltpu.roll(r_e, 64, 1)),
                       jnp.where(h0, pltpu.roll(r_o, 64, 1), r_o))
        ot_ref[40 * p:40 * p + 40, mm * 128:(mm + 1) * 128] = tt[sh:sh + 40]

    for n in range(NPAIR + 2):
        res = {}
        for u in range(NCH):
            if n < NPAIR:
                qk_a(n % 2, u, n, u)
            if 1 <= n <= NPAIR:
                sm_a((n - 1) % 2, u, n - 1, u)
            if n >= 2:
                res[u] = pv_a((n - 2) % 2, u, n - 2, u)
                if u % 2:
                    put(n - 2, u // 2, res[u - 1], res[u])

    a = _dot(ot_ref[...].astype(BF).T, woa_ref[...])
    o_ref[...] = (g * a + acc_ref[...]).astype(o_ref.dtype)


@jax.jit
def pallas_gated_mix__sliding_block__sliding_local_dilated__prompt_kernel(
    A_x: jax.Array,
    A_wqkv: jax.Array,
    A_wo: jax.Array,
    B_x: jax.Array,
    B_wqkv: jax.Array,
    B_wo: jax.Array,
    gate_w: jax.Array,
):
    del B_x
    x = A_x.reshape(S, D)
    gw = gate_w.reshape(1, D)
    const = lambda shape: pl.BlockSpec(shape, lambda t: (0,) * len(shape))
    out = pl.pallas_call(
        kernel,
        grid=(S // R,),
        in_specs=[
            pl.BlockSpec((R, D), lambda t: (t, 0)),
            const((D, 3 * D)), const((D, D)), const((D, 3 * D)), const((D, D)), const((1, D)),
        ],
        out_specs=pl.BlockSpec((R, D), lambda t: (t, 0)),
        out_shape=jax.ShapeDtypeStruct((S, D), BF),
        scratch_shapes=[
            pltpu.VMEM((NT, R, 128), BF),
            pltpu.VMEM((NT, WA + S, 128), BF),
            pltpu.VMEM(((WA + S) // 128, D, 128), BF),
            pltpu.VMEM((D, R), F32),
            pltpu.VMEM((2, NCH, WA + QC, 128), F32),
            pltpu.VMEM((2, NCH, 384, 128), BF),
            pltpu.VMEM((2, NCH, 8, 128), F32),
            pltpu.VMEM((3, D, D), BF),
            pltpu.VMEM((D, D), BF),
            pltpu.VMEM((NLT, D, 128), F32),
            pltpu.VMEM((NLT, R, 128), F32),
            pltpu.VMEM((NLT, HB + S, 128), F32),
            pltpu.VMEM((NLT, HB + S, 128), F32),
            pltpu.VMEM((R, D), BF),
            pltpu.VMEM((R, D), F32),
        ],
        compiler_params=pltpu.CompilerParams(
            dimension_semantics=("arbitrary",),
            vmem_limit_bytes=100 * 1024 * 1024,
        ),
        name="gated_mix_attn",
    )(x, A_wqkv, A_wo, B_wqkv, B_wo, gw)
    return out.reshape(1, S, D)
```

```python
import jax
import jax.numpy as jnp
import numpy as np
import jax.experimental.pallas as pl
import jax.experimental.pallas.tpu as pltpu

S = 2048
D = 640
H = 32
DH = 20
NLT = D // 128
R = 256
QC = 64
NCH = R // QC
NPAIR = H // 2
WA = 256
HB = 16
RB = 16
LINK = 1
NEG = -1e30
LOG2E = 1.4426950408889634
QSCALE = float(DH ** -0.5) * LOG2E
BF = jnp.bfloat16
F32 = jnp.float32


def _pair_tile(p):
    c0 = 40 * p
    t0, off = divmod(c0, 128)
    if off + 40 <= 128:
        return (t0, t0, 0), off
    return (t0, t0 + 1, off), off


_TILES = []
_PAIR = []
for _p in range(NPAIR):
    _t, _o = _pair_tile(_p)
    if _t not in _TILES:
        _TILES.append(_t)
    _PAIR.append((_TILES.index(_t), _o))
NT = len(_TILES)


def _u32(x):
    return pltpu.bitcast(x, jnp.uint32)


def _bf(x):
    return pltpu.bitcast(x, BF)


def _build_tiles(y):
    rows = y.shape[0]
    lane = jax.lax.broadcasted_iota(jnp.int32, (rows, 128), 1)
    out = []
    for (a, b, split) in _TILES:
        ta = y[:, a * 128:(a + 1) * 128]
        if a != b:
            ta = jnp.where(lane >= split, ta, y[:, b * 128:(b + 1) * 128])
        out.append(ta.astype(BF))
    return out


def _nt_dot(a, b):
    return jax.lax.dot_general(a, b, (((1,), (1,)), ((), ())), preferred_element_type=F32)


def _dot(a, b):
    return jnp.dot(a, b, preferred_element_type=F32)


def kernel(x_ref, wa_hbm, woa_hbm, wb_hbm, wob_hbm, gw_ref, o_ref,
           wa_ref, woa_ref, wb_ref, wob_ref, sems,
           qa_ref, ka_ref, vta_ref, ot_ref, oa_ref, s_ref, p_ref, l_ref,
           wbt_ref, wobp_ref, tmp_ref, qb_ref, kb_ref, vb_ref, ob_ref, acc_ref):
    t = pl.program_id(0)
    x = x_ref[...]
    not_first = t > 0
    row0 = pl.multiple_of(t * R, R)

    def sec(ref, i):
        return ref.at[:, pl.ds(i * D, D)]

    copies = [pltpu.make_async_copy(sec(wb_hbm, i), wb_ref.at[i], sems.at[i]) for i in range(3)]
    copies += [pltpu.make_async_copy(sec(wa_hbm, i), wa_ref.at[i], sems.at[3 + i]) for i in range(3)]
    copies += [pltpu.make_async_copy(wob_hbm, wob_ref, sems.at[6]),
               pltpu.make_async_copy(woa_hbm, woa_ref, sems.at[7])]

    @pl.when(t == 0)
    def _():
        for cp in copies:
            cp.start()
        ka_ref[:, 0:WA, :] = jnp.zeros((NT, WA, 128), BF)
        for j in range(WA // 128):
            vta_ref[j] = jnp.zeros((D, 128), BF)
        kb_ref[:, 0:HB, :] = jnp.zeros((NLT, HB, 128), F32)
        vb_ref[:, 0:HB, :] = jnp.zeros((NLT, HB, 128), F32)

    def permute_rows(dst_ref):
        for c in range(NLT):
            for d in range(DH):
                dst_ref[c, d * H:(d + 1) * H, :] = tmp_ref[c, pl.ds(d, H, stride=DH), :].astype(BF)

    for i, dst in enumerate((qb_ref, kb_ref, vb_ref)):
        @pl.when(t == 0)
        def _():
            copies[i].wait()
            for c in range(NLT):
                for n in range(NLT):
                    w = wb_ref[i, c * 128:(c + 1) * 128, n * 128:(n + 1) * 128]
                    tmp_ref[c, n * 128:(n + 1) * 128, :] = w.astype(F32).T
            permute_rows(wbt_ref.at[i])

        y = None
        for c in range(NLT):
            z = _nt_dot(x[:, c * 128:(c + 1) * 128], wbt_ref[i, c])
            y = z if y is None else y + z
        for c in range(NLT):
            if i == 0:
                dst[c] = y[:, c * 128:(c + 1) * 128] * QSCALE
            else:
                dst[c, pl.ds(row0 + HB, R), :] = y[:, c * 128:(c + 1) * 128]

    @pl.when(t == 0)
    def _():
        for cp in copies[3:7]:
            cp.wait()
        for c in range(NLT):
            tmp_ref[c] = wob_ref[:, c * 128:(c + 1) * 128].astype(F32)
        permute_rows(wobp_ref)

    rowb = jax.lax.broadcasted_iota(jnp.int32, (RB, 128), 0)

    never = t < 0
    chain = [None, None]

    def attn_b(ci):
        r = ci * RB
        q = [qb_ref[c, r:r + RB, :] for c in range(NLT)]
        if chain[ci % LINK] is not None:
            q[0] = jnp.where(never, chain[ci % LINK], q[0])
            q[NLT - 1] = jnp.where(never, chain[ci % LINK], q[NLT - 1])
        sc = []
        for j in range(8):
            acc = None
            for c in range(NLT):
                y = q[c] * kb_ref[c, pl.ds(row0 + (r + HB - 2 * j), RB), :]
                acc = y if acc is None else acc + y
            acc = acc + pltpu.roll(acc, 64, 1)
            acc = acc + pltpu.roll(acc, 32, 1)
            if r < 2 * j:
                acc = jnp.where(not_first | (rowb >= 2 * j - r), acc, NEG)
            sc.append(acc)
        m = sc[0]
        for y in sc[1:]:
            m = jnp.maximum(m, y)
        e = [jnp.exp2(y - m) for y in sc]
        l = e[0]
        for y in e[1:]:
            l = l + y
        inv = 1.0 / l
        for c in range(NLT):
            acc = None
            for j in range(8):
                y = e[j] * vb_ref[c, pl.ds(row0 + (r + HB - 2 * j), RB), :]
                acc = y if acc is None else acc + y
            ob_ref[r:r + RB, c * 128:(c + 1) * 128] = (acc * inv).astype(BF)
        chain[ci % LINK] = acc

    nb = R // RB
    q = _dot(x, wa_ref[0]) * QSCALE
    for i, tl in enumerate(_build_tiles(q)):
        qa_ref[i] = tl
    for ci in range(0, nb // 3):
        attn_b(ci)
    k = _dot(x, wa_ref[1])
    for i, tl in enumerate(_build_tiles(k)):
        ka_ref[i, pl.ds(row0 + WA, R), :] = tl
    for ci in range(nb // 3, 2 * nb // 3):
        attn_b(ci)
    va = _dot(x, wa_ref[2]).astype(BF)
    for j in range(R // 128):
        vta_ref[t * (R // 128) + WA // 128 + j] = va[j * 128:(j + 1) * 128, :].T
    for ci in range(2 * nb // 3, nb):
        attn_b(ci)

    gl = jnp.sum(x.astype(F32) * gw_ref[...].astype(F32), axis=1, keepdims=True)
    g = jax.nn.sigmoid(gl)
    for c in range(NLT):
        acc_ref[:, c * 128:(c + 1) * 128] = (1.0 - g) * _dot(ob_ref[...], wobp_ref[c])

    lane128 = jax.lax.broadcasted_iota(jnp.int32, (QC, 128), 1)
    row64 = jax.lax.broadcasted_iota(jnp.int32, (QC, 128), 0)
    lower = row64 <= (lane128 & (QC - 1))
    lane32 = jax.lax.broadcasted_iota(jnp.int32, (QC // 2, 128), 1)
    row48 = jax.lax.broadcasted_iota(jnp.int32, (48, 128), 0)
    lane48 = jax.lax.broadcasted_iota(jnp.int32, (48, 128), 1)
    left = lane48 < 64

    def masked_q(p, i):
        tix, off = _PAIR[p]
        qt = _u32(qa_ref[tix, i * QC:(i + 1) * QC, :])
        rel = (lane32 - off) & 127
        ones = jnp.uint32(0xFFFFFFFF)
        m0 = jnp.where(rel < DH, ones, jnp.uint32(0))
        m1 = jnp.where((rel >= DH) & (rel < 2 * DH), ones, jnp.uint32(0))
        return _bf(jnp.concatenate([qt & m0, qt & m1], axis=0))

    def qk_a(sl, u, p, i):
        kk = ka_ref[_PAIR[p][0], pl.ds(row0 + i * QC, WA + QC), :]
        s_ref[sl, u] = _nt_dot(kk, masked_q(p, i))

    def sm_a(sl, u, p, i):
        def chunk(c):
            v = s_ref[sl, u, c * QC:(c + 1) * QC, :]
            if c < NCH - i:
                v = jnp.where(not_first, v, NEG)
            return v
        mrg = jnp.where(lower, s_ref[sl, u, WA:WA + QC, :], chunk(0))
        mid = [chunk(c) for c in range(1, 4)]
        m = jnp.max(mrg, axis=0, keepdims=True)
        for v in mid:
            m = jnp.maximum(m, jnp.max(v, axis=0, keepdims=True))
        pg = jnp.exp2(mrg - m)
        l = jnp.sum(pg, axis=0, keepdims=True)
        o = QC * (i % 2)
        p_ref[sl, u, o:o + QC, :] = jnp.where(lower, 0.0, pg).astype(BF)
        p_ref[sl, u, o + WA:o + WA + QC, :] = jnp.where(lower, pg, 0.0).astype(BF)
        for c, v in enumerate(mid):
            pm = jnp.exp2(v - m)
            l = l + jnp.sum(pm, axis=0, keepdims=True)
            p_ref[sl, u, o + (c + 1) * QC:o + (c + 2) * QC, :] = pm.astype(BF)
        z = (WA + QC) if i % 2 == 0 else 0
        p_ref[sl, u, z:z + QC, :] = jnp.zeros((QC, 128), BF)
        l_ref[sl, u] = jnp.broadcast_to(1.0 / l, (8, 128))

    def pv_a(sl, u, p, i):
        r0 = 40 * p - 8 * (p % 2)
        c0 = t * (R // 128) + i // 2
        acc = None
        for j in range(3):
            y = _dot(vta_ref[c0 + j, r0:r0 + 48, :], p_ref[sl, u, j * 128:(j + 1) * 128, :])
            acc = y if acc is None else acc + y
        return acc * l_ref[sl, u][0:1]

    def put(p, mm, r_e, r_o):
        sh = 8 * (p % 2)
        h0 = (row48 - sh) < DH
        tt = jnp.where(left, jnp.where(h0, r_e, pltpu.roll(r_e, 64, 1)),
                       jnp.where(h0, pltpu.roll(r_o, 64, 1), r_o))
        ot_ref[40 * p:40 * p + 40, mm * 128:(mm + 1) * 128] = tt[sh:sh + 40]
        for c in range(NLT):
            if 40 * p < (c + 1) * 128 <= 40 * p + 40:
                oa_ref[mm * 128:(mm + 1) * 128, c * 128:(c + 1) * 128] = (
                    ot_ref[c * 128:(c + 1) * 128, mm * 128:(mm + 1) * 128].astype(BF).T)

    for n in range(NPAIR + 2):
        res = {}
        for u in range(NCH):
            if n < NPAIR:
                qk_a(n % 2, u, n, u)
            if 1 <= n <= NPAIR:
                sm_a((n - 1) % 2, u, n - 1, u)
            if n >= 2:
                res[u] = pv_a((n - 2) % 2, u, n - 2, u)
                if u % 2:
                    put(n - 2, u // 2, res[u - 1], res[u])

    @pl.when(t == 0)
    def _():
        copies[7].wait()

    a = _dot(oa_ref[...], woa_ref[...])
    o_ref[...] = (g * a + acc_ref[...]).astype(o_ref.dtype)


@jax.jit
def pallas_gated_mix__sliding_block__sliding_local_dilated__prompt_kernel(
    A_x: jax.Array,
    A_wqkv: jax.Array,
    A_wo: jax.Array,
    B_x: jax.Array,
    B_wqkv: jax.Array,
    B_wo: jax.Array,
    gate_w: jax.Array,
):
    del B_x
    x = A_x.reshape(S, D)
    gw = gate_w.reshape(1, D)
    hbm = pl.BlockSpec(memory_space=pl.ANY)
    out = pl.pallas_call(
        kernel,
        grid=(S // R,),
        in_specs=[
            pl.BlockSpec((R, D), lambda t: (t, 0)),
            hbm, hbm, hbm, hbm, pl.BlockSpec((1, D), lambda t: (0, 0)),
        ],
        out_specs=pl.BlockSpec((R, D), lambda t: (t, 0)),
        out_shape=jax.ShapeDtypeStruct((S, D), BF),
        scratch_shapes=[
            pltpu.VMEM((3, D, D), BF),
            pltpu.VMEM((D, D), BF),
            pltpu.VMEM((3, D, D), BF),
            pltpu.VMEM((D, D), BF),
            pltpu.SemaphoreType.DMA((8,)),
            pltpu.VMEM((NT, R, 128), BF),
            pltpu.VMEM((NT, WA + S, 128), BF),
            pltpu.VMEM(((WA + S) // 128, D, 128), BF),
            pltpu.VMEM((D, R), F32),
            pltpu.VMEM((R, D), BF),
            pltpu.VMEM((2, NCH, WA + QC, 128), F32),
            pltpu.VMEM((2, NCH, 384, 128), BF),
            pltpu.VMEM((2, NCH, 8, 128), F32),
            pltpu.VMEM((3, NLT, D, 128), BF),
            pltpu.VMEM((NLT, D, 128), BF),
            pltpu.VMEM((NLT, D, 128), F32),
            pltpu.VMEM((NLT, R, 128), F32),
            pltpu.VMEM((NLT, HB + S, 128), F32),
            pltpu.VMEM((NLT, HB + S, 128), F32),
            pltpu.VMEM((R, D), BF),
            pltpu.VMEM((R, D), F32),
        ],
        compiler_params=pltpu.CompilerParams(
            dimension_semantics=("arbitrary",),
            vmem_limit_bytes=100 * 1024 * 1024,
        ),
        name="gated_mix_attn",
    )(x, A_wqkv, A_wo, B_wqkv, B_wo, gw)
    return out.reshape(1, S, D)
```

```python
import jax
import jax.numpy as jnp
import numpy as np
import jax.experimental.pallas as pl
import jax.experimental.pallas.tpu as pltpu

S = 2048
D = 640
H = 32
DH = 20
NLT = D // 128
R = 256
QC = 64
NCH = R // QC
NPAIR = H // 2
WA = 256
HB = 16
RB = 16
LINK = 1
NEG = -1e30
LOG2E = 1.4426950408889634
QSCALE = float(DH ** -0.5) * LOG2E
BF = jnp.bfloat16
F32 = jnp.float32


def _pair_tile(p):
    c0 = 40 * p
    t0, off = divmod(c0, 128)
    if off + 40 <= 128:
        return (t0, t0, 0), off
    return (t0, t0 + 1, off), off


_TILES = []
_PAIR = []
for _p in range(NPAIR):
    _t, _o = _pair_tile(_p)
    if _t not in _TILES:
        _TILES.append(_t)
    _PAIR.append((_TILES.index(_t), _o))
NT = len(_TILES)


def _u32(x):
    return pltpu.bitcast(x, jnp.uint32)


def _bf(x):
    return pltpu.bitcast(x, BF)


def _build_tiles(y):
    rows = y.shape[0]
    lane = jax.lax.broadcasted_iota(jnp.int32, (rows, 128), 1)
    out = []
    for (a, b, split) in _TILES:
        ta = y[:, a * 128:(a + 1) * 128]
        if a != b:
            ta = jnp.where(lane >= split, ta, y[:, b * 128:(b + 1) * 128])
        out.append(ta.astype(BF))
    return out


def _nt_dot(a, b):
    return jax.lax.dot_general(a, b, (((1,), (1,)), ((), ())), preferred_element_type=F32)


def _dot(a, b):
    return jnp.dot(a, b, preferred_element_type=F32)


def kernel(x_ref, wa_hbm, woa_hbm, wb_hbm, wob_hbm, gw_ref, o_ref,
           wa_ref, woa_ref, wb_ref, wob_ref, sems,
           qa_ref, ka_ref, vta_ref, ot_ref, oa_ref, s_ref, p_ref, l_ref,
           wbt_ref, wobp_ref, tmp_ref, qb_ref, kb_ref, vb_ref, ob_ref, acc_ref):
    t = pl.program_id(0)
    x = x_ref[...]
    not_first = t > 0
    row0 = pl.multiple_of(t * R, R)

    phase = pl.when(t >= 0)

    def sec(ref, i):
        return ref.at[:, pl.ds(i * D, D)]

    copies = [pltpu.make_async_copy(sec(wb_hbm, i), wb_ref.at[i], sems.at[i]) for i in range(3)]
    copies += [pltpu.make_async_copy(sec(wa_hbm, i), wa_ref.at[i], sems.at[3 + i]) for i in range(3)]
    copies += [pltpu.make_async_copy(wob_hbm, wob_ref, sems.at[6]),
               pltpu.make_async_copy(woa_hbm, woa_ref, sems.at[7])]

    @pl.when(t == 0)
    def _():
        copies[0].start()
        copies[1].start()
        ka_ref[:, 0:WA, :] = jnp.zeros((NT, WA, 128), BF)
        for j in range(WA // 128):
            vta_ref[j] = jnp.zeros((D, 128), BF)
        kb_ref[:, 0:HB, :] = jnp.zeros((NLT, HB, 128), F32)
        vb_ref[:, 0:HB, :] = jnp.zeros((NLT, HB, 128), F32)

    def permute_rows(dst_ref):
        for c in range(NLT):
            for d in range(DH):
                dst_ref[c, d * H:(d + 1) * H, :] = tmp_ref[c, pl.ds(d, H, stride=DH), :].astype(BF)

    for i, dst in enumerate((qb_ref, kb_ref, vb_ref)):
        @pl.when(t == 0)
        def _():
            copies[i].wait()
            copies[i + 2].start()
            for c in range(NLT):
                for n in range(NLT):
                    w = wb_ref[i, c * 128:(c + 1) * 128, n * 128:(n + 1) * 128]
                    tmp_ref[c, n * 128:(n + 1) * 128, :] = w.astype(F32).T
            permute_rows(wbt_ref.at[i])

        y = None
        for c in range(NLT):
            z = _nt_dot(x[:, c * 128:(c + 1) * 128], wbt_ref[i, c])
            y = z if y is None else y + z
        for c in range(NLT):
            if i == 0:
                dst[c] = y[:, c * 128:(c + 1) * 128] * QSCALE
            else:
                dst[c, pl.ds(row0 + HB, R), :] = y[:, c * 128:(c + 1) * 128]

    @pl.when(t == 0)
    def _():
        copies[5].start()
        copies[6].start()
        copies[7].start()
        for cp in copies[3:7]:
            cp.wait()
        for c in range(NLT):
            tmp_ref[c] = wob_ref[:, c * 128:(c + 1) * 128].astype(F32)
        permute_rows(wobp_ref)

    gl = jnp.sum(x.astype(F32) * gw_ref[...].astype(F32), axis=1, keepdims=True)
    g = jax.nn.sigmoid(gl)
    rowb = jax.lax.broadcasted_iota(jnp.int32, (RB, 128), 0)

    never = t < 0
    chain = [None, None]

    def attn_b(ci):
        r = ci * RB
        q = [qb_ref[c, r:r + RB, :] for c in range(NLT)]
        if chain[ci % LINK] is not None:
            q[0] = jnp.where(never, chain[ci % LINK], q[0])
            q[NLT - 1] = jnp.where(never, chain[ci % LINK], q[NLT - 1])
        sc = []
        for j in range(8):
            acc = None
            for c in range(NLT):
                y = q[c] * kb_ref[c, pl.ds(row0 + (r + HB - 2 * j), RB), :]
                acc = y if acc is None else acc + y
            acc = acc + pltpu.roll(acc, 64, 1)
            acc = acc + pltpu.roll(acc, 32, 1)
            if r < 2 * j:
                acc = jnp.where(not_first | (rowb >= 2 * j - r), acc, NEG)
            sc.append(acc)
        m = sc[0]
        for y in sc[1:]:
            m = jnp.maximum(m, y)
        e = [jnp.exp2(y - m) for y in sc]
        l = e[0]
        for y in e[1:]:
            l = l + y
        inv = 1.0 / l
        for c in range(NLT):
            acc = None
            for j in range(8):
                y = e[j] * vb_ref[c, pl.ds(row0 + (r + HB - 2 * j), RB), :]
                acc = y if acc is None else acc + y
            ob_ref[r:r + RB, c * 128:(c + 1) * 128] = (acc * inv).astype(BF)
        chain[ci % LINK] = acc

    @phase
    def _():
        nb = R // RB
        q = _dot(x, wa_ref[0]) * QSCALE
        for i, tl in enumerate(_build_tiles(q)):
            qa_ref[i] = tl
        for ci in range(0, nb // 3):
            attn_b(ci)
        k = _dot(x, wa_ref[1])
        for i, tl in enumerate(_build_tiles(k)):
            ka_ref[i, pl.ds(row0 + WA, R), :] = tl
        for ci in range(nb // 3, 2 * nb // 3):
            attn_b(ci)
        va = _dot(x, wa_ref[2]).astype(BF)
        for j in range(R // 128):
            vta_ref[t * (R // 128) + WA // 128 + j] = va[j * 128:(j + 1) * 128, :].T
        for ci in range(2 * nb // 3, nb):
            attn_b(ci)

        for c in range(NLT):
            acc_ref[:, c * 128:(c + 1) * 128] = (1.0 - g) * _dot(ob_ref[...], wobp_ref[c])

    lane128 = jax.lax.broadcasted_iota(jnp.int32, (QC, 128), 1)
    row64 = jax.lax.broadcasted_iota(jnp.int32, (QC, 128), 0)
    lower = row64 <= (lane128 & (QC - 1))
    lane32 = jax.lax.broadcasted_iota(jnp.int32, (QC // 2, 128), 1)
    row48 = jax.lax.broadcasted_iota(jnp.int32, (48, 128), 0)
    lane48 = jax.lax.broadcasted_iota(jnp.int32, (48, 128), 1)
    left = lane48 < 64

    def masked_q(p, i):
        tix, off = _PAIR[p]
        qt = _u32(qa_ref[tix, i * QC:(i + 1) * QC, :])
        rel = (lane32 - off) & 127
        ones = jnp.uint32(0xFFFFFFFF)
        m0 = jnp.where(rel < DH, ones, jnp.uint32(0))
        m1 = jnp.where((rel >= DH) & (rel < 2 * DH), ones, jnp.uint32(0))
        return _bf(jnp.concatenate([qt & m0, qt & m1], axis=0))

    def qk_a(sl, u, p, i):
        kk = ka_ref[_PAIR[p][0], pl.ds(row0 + i * QC, WA + QC), :]
        s_ref[sl, u] = _nt_dot(kk, masked_q(p, i))

    def sm_a(sl, u, p, i):
        def chunk(c):
            v = s_ref[sl, u, c * QC:(c + 1) * QC, :]
            if c < NCH - i:
                v = jnp.where(not_first, v, NEG)
            return v
        mrg = jnp.where(lower, s_ref[sl, u, WA:WA + QC, :], chunk(0))
        mid = [chunk(c) for c in range(1, 4)]
        m = jnp.max(mrg, axis=0, keepdims=True)
        for v in mid:
            m = jnp.maximum(m, jnp.max(v, axis=0, keepdims=True))
        pg = jnp.exp2(mrg - m)
        l = jnp.sum(pg, axis=0, keepdims=True)
        o = QC * (i % 2)
        p_ref[sl, u, o:o + QC, :] = jnp.where(lower, 0.0, pg).astype(BF)
        p_ref[sl, u, o + WA:o + WA + QC, :] = jnp.where(lower, pg, 0.0).astype(BF)
        for c, v in enumerate(mid):
            pm = jnp.exp2(v - m)
            l = l + jnp.sum(pm, axis=0, keepdims=True)
            p_ref[sl, u, o + (c + 1) * QC:o + (c + 2) * QC, :] = pm.astype(BF)
        z = (WA + QC) if i % 2 == 0 else 0
        p_ref[sl, u, z:z + QC, :] = jnp.zeros((QC, 128), BF)
        l_ref[sl, u] = jnp.broadcast_to(1.0 / l, (8, 128))

    def pv_a(sl, u, p, i):
        r0 = 40 * p - 8 * (p % 2)
        c0 = t * (R // 128) + i // 2
        acc = None
        for j in range(3):
            y = _dot(vta_ref[c0 + j, r0:r0 + 48, :], p_ref[sl, u, j * 128:(j + 1) * 128, :])
            acc = y if acc is None else acc + y
        return acc * l_ref[sl, u][0:1]

    def put(p, mm, r_e, r_o):
        sh = 8 * (p % 2)
        h0 = (row48 - sh) < DH
        tt = jnp.where(left, jnp.where(h0, r_e, pltpu.roll(r_e, 64, 1)),
                       jnp.where(h0, pltpu.roll(r_o, 64, 1), r_o))
        ot_ref[40 * p:40 * p + 40, mm * 128:(mm + 1) * 128] = tt[sh:sh + 40]
        for c in range(NLT):
            if 40 * p < (c + 1) * 128 <= 40 * p + 40:
                oa_ref[mm * 128:(mm + 1) * 128, c * 128:(c + 1) * 128] = (
                    ot_ref[c * 128:(c + 1) * 128, mm * 128:(mm + 1) * 128].astype(BF).T)

    @phase
    def _():
        for n in range(NPAIR + 2):
            res = {}
            for u in range(NCH):
                if n < NPAIR:
                    qk_a(n % 2, u, n, u)
                if 1 <= n <= NPAIR:
                    sm_a((n - 1) % 2, u, n - 1, u)
                if n >= 2:
                    res[u] = pv_a((n - 2) % 2, u, n - 2, u)
                    if u % 2:
                        put(n - 2, u // 2, res[u - 1], res[u])

    @pl.when(t == 0)
    def _():
        copies[7].wait()

    a = _dot(oa_ref[...], woa_ref[...])
    o_ref[...] = (g * a + acc_ref[...]).astype(o_ref.dtype)


@jax.jit
def pallas_gated_mix__sliding_block__sliding_local_dilated__prompt_kernel(
    A_x: jax.Array,
    A_wqkv: jax.Array,
    A_wo: jax.Array,
    B_x: jax.Array,
    B_wqkv: jax.Array,
    B_wo: jax.Array,
    gate_w: jax.Array,
):
    del B_x
    x = A_x.reshape(S, D)
    gw = gate_w.reshape(1, D)
    hbm = pl.BlockSpec(memory_space=pl.ANY)
    out = pl.pallas_call(
        kernel,
        grid=(S // R,),
        in_specs=[
            pl.BlockSpec((R, D), lambda t: (t, 0)),
            hbm, hbm, hbm, hbm, pl.BlockSpec((1, D), lambda t: (0, 0)),
        ],
        out_specs=pl.BlockSpec((R, D), lambda t: (t, 0)),
        out_shape=jax.ShapeDtypeStruct((S, D), BF),
        scratch_shapes=[
            pltpu.VMEM((3, D, D), BF),
            pltpu.VMEM((D, D), BF),
            pltpu.VMEM((3, D, D), BF),
            pltpu.VMEM((D, D), BF),
            pltpu.SemaphoreType.DMA((8,)),
            pltpu.VMEM((NT, R, 128), BF),
            pltpu.VMEM((NT, WA + S, 128), BF),
            pltpu.VMEM(((WA + S) // 128, D, 128), BF),
            pltpu.VMEM((D, R), F32),
            pltpu.VMEM((R, D), BF),
            pltpu.VMEM((2, NCH, WA + QC, 128), F32),
            pltpu.VMEM((2, NCH, 384, 128), BF),
            pltpu.VMEM((2, NCH, 8, 128), F32),
            pltpu.VMEM((3, NLT, D, 128), BF),
            pltpu.VMEM((NLT, D, 128), BF),
            pltpu.VMEM((NLT, D, 128), F32),
            pltpu.VMEM((NLT, R, 128), F32),
            pltpu.VMEM((NLT, HB + S, 128), F32),
            pltpu.VMEM((NLT, HB + S, 128), F32),
            pltpu.VMEM((R, D), BF),
            pltpu.VMEM((R, D), F32),
        ],
        compiler_params=pltpu.CompilerParams(
            dimension_semantics=("arbitrary",),
            vmem_limit_bytes=100 * 1024 * 1024,
        ),
        name="gated_mix_attn",
    )(x, A_wqkv, A_wo, B_wqkv, B_wo, gw)
    return out.reshape(1, S, D)
```

```python
import jax
import jax.numpy as jnp
import numpy as np
import jax.experimental.pallas as pl
import jax.experimental.pallas.tpu as pltpu

S = 2048
D = 640
H = 32
DH = 20
NLT = D // 128
R = 256
QC = 64
NCH = R // QC
NPAIR = H // 2
WA = 256
HB = 16
RB = 16
LINK = 1
NEG = -1e30
LOG2E = 1.4426950408889634
QSCALE = float(DH ** -0.5) * LOG2E
BF = jnp.bfloat16
F32 = jnp.float32


def _pair_tile(p):
    c0 = 40 * p
    t0, off = divmod(c0, 128)
    if off + 40 <= 128:
        return (t0, t0, 0), off
    return (t0, t0 + 1, off), off


_TILES = []
_PAIR = []
for _p in range(NPAIR):
    _t, _o = _pair_tile(_p)
    if _t not in _TILES:
        _TILES.append(_t)
    _PAIR.append((_TILES.index(_t), _o))
NT = len(_TILES)


def _u32(x):
    return pltpu.bitcast(x, jnp.uint32)


def _bf(x):
    return pltpu.bitcast(x, BF)


def _build_tiles(y):
    rows = y.shape[0]
    lane = jax.lax.broadcasted_iota(jnp.int32, (rows, 128), 1)
    out = []
    for (a, b, split) in _TILES:
        ta = y[:, a * 128:(a + 1) * 128]
        if a != b:
            ta = jnp.where(lane >= split, ta, y[:, b * 128:(b + 1) * 128])
        out.append(ta.astype(BF))
    return out


def _nt_dot(a, b):
    return jax.lax.dot_general(a, b, (((1,), (1,)), ((), ())), preferred_element_type=F32)


def _dot(a, b):
    return jnp.dot(a, b, preferred_element_type=F32)


def kernel(x_ref, wa_hbm, woa_hbm, wb_hbm, wob_hbm, gw_ref, o_ref,
           wa_ref, woa_ref, wb_ref, wob_ref, sems,
           qa_ref, ka_ref, vta_ref, ot_ref, oa_ref, s_ref, p_ref, l_ref,
           wbt_ref, wobp_ref, tmp_ref, qb_ref, kb_ref, vb_ref, ob_ref):
    t = pl.program_id(0)
    x = x_ref[...]
    not_first = t > 0
    row0 = pl.multiple_of(t * R, R)

    phase = pl.when(t >= 0)

    def sec(ref, i):
        return ref.at[:, pl.ds(i * D, D)]

    copies = [pltpu.make_async_copy(sec(wb_hbm, i), wb_ref.at[i], sems.at[i]) for i in range(3)]
    copies += [pltpu.make_async_copy(sec(wa_hbm, i), wa_ref.at[i], sems.at[3 + i]) for i in range(3)]
    copies += [pltpu.make_async_copy(wob_hbm, wob_ref, sems.at[6]),
               pltpu.make_async_copy(woa_hbm, woa_ref, sems.at[7])]

    @pl.when(t == 0)
    def _():
        copies[0].start()
        copies[1].start()
        ka_ref[:, 0:WA, :] = jnp.zeros((NT, WA, 128), BF)
        for j in range(WA // 128):
            vta_ref[j] = jnp.zeros((D, 128), BF)
        kb_ref[:, 0:HB, :] = jnp.zeros((NLT, HB, 128), F32)
        vb_ref[:, 0:HB, :] = jnp.zeros((NLT, HB, 128), F32)

    def permute_rows(dst_ref):
        for c in range(NLT):
            for d in range(DH):
                dst_ref[c, d * H:(d + 1) * H, :] = tmp_ref[c, pl.ds(d, H, stride=DH), :].astype(BF)

    for i, dst in enumerate((qb_ref, kb_ref, vb_ref)):
        @pl.when(t == 0)
        def _():
            copies[i].wait()
            copies[2 * i + 2].start()
            copies[2 * i + 3].start()
            for c in range(NLT):
                for n in range(NLT):
                    w = wb_ref[i, c * 128:(c + 1) * 128, n * 128:(n + 1) * 128]
                    tmp_ref[c, n * 128:(n + 1) * 128, :] = w.astype(F32).T
            permute_rows(wbt_ref.at[i])

        y = None
        for c in range(NLT):
            z = _nt_dot(x[:, c * 128:(c + 1) * 128], wbt_ref[i, c])
            y = z if y is None else y + z
        for c in range(NLT):
            if i == 0:
                dst[c] = y[:, c * 128:(c + 1) * 128] * QSCALE
            else:
                dst[c, pl.ds(row0 + HB, R), :] = y[:, c * 128:(c + 1) * 128]

    @pl.when(t == 0)
    def _():
        for cp in copies[3:6]:
            cp.wait()

    gl = jnp.sum(x.astype(F32) * gw_ref[...].astype(F32), axis=1, keepdims=True)
    g = jax.nn.sigmoid(gl)
    rowb = jax.lax.broadcasted_iota(jnp.int32, (RB, 128), 0)

    never = t < 0
    chain = [None, None]

    def attn_b(ci):
        r = ci * RB
        q = [qb_ref[c, r:r + RB, :] for c in range(NLT)]
        if chain[ci % LINK] is not None:
            q[0] = jnp.where(never, chain[ci % LINK], q[0])
            q[NLT - 1] = jnp.where(never, chain[ci % LINK], q[NLT - 1])
        sc = []
        for j in range(8):
            acc = None
            for c in range(NLT):
                y = q[c] * kb_ref[c, pl.ds(row0 + (r + HB - 2 * j), RB), :]
                acc = y if acc is None else acc + y
            acc = acc + pltpu.roll(acc, 64, 1)
            acc = acc + pltpu.roll(acc, 32, 1)
            if r < 2 * j:
                acc = jnp.where(not_first | (rowb >= 2 * j - r), acc, NEG)
            sc.append(acc)
        m = sc[0]
        for y in sc[1:]:
            m = jnp.maximum(m, y)
        e = [jnp.exp2(y - m) for y in sc]
        l = e[0]
        for y in e[1:]:
            l = l + y
        inv = 1.0 / l
        for c in range(NLT):
            acc = None
            for j in range(8):
                y = e[j] * vb_ref[c, pl.ds(row0 + (r + HB - 2 * j), RB), :]
                acc = y if acc is None else acc + y
            ob_ref[r:r + RB, c * 128:(c + 1) * 128] = (acc * inv).astype(BF)
        chain[ci % LINK] = acc

    @phase
    def _():
        nb = R // RB
        q = _dot(x, wa_ref[0]) * QSCALE
        for i, tl in enumerate(_build_tiles(q)):
            qa_ref[i] = tl
        for ci in range(0, nb // 3):
            attn_b(ci)
        k = _dot(x, wa_ref[1])
        for i, tl in enumerate(_build_tiles(k)):
            ka_ref[i, pl.ds(row0 + WA, R), :] = tl
        for ci in range(nb // 3, 2 * nb // 3):
            attn_b(ci)
        va = _dot(x, wa_ref[2]).astype(BF)
        for j in range(R // 128):
            vta_ref[t * (R // 128) + WA // 128 + j] = va[j * 128:(j + 1) * 128, :].T
        for ci in range(2 * nb // 3, nb):
            attn_b(ci)


    lane128 = jax.lax.broadcasted_iota(jnp.int32, (QC, 128), 1)
    row64 = jax.lax.broadcasted_iota(jnp.int32, (QC, 128), 0)
    lower = row64 <= (lane128 & (QC - 1))
    lane32 = jax.lax.broadcasted_iota(jnp.int32, (QC // 2, 128), 1)
    row48 = jax.lax.broadcasted_iota(jnp.int32, (48, 128), 0)
    lane48 = jax.lax.broadcasted_iota(jnp.int32, (48, 128), 1)
    left = lane48 < 64

    def masked_q(p, i):
        tix, off = _PAIR[p]
        qt = _u32(qa_ref[tix, i * QC:(i + 1) * QC, :])
        rel = (lane32 - off) & 127
        ones = jnp.uint32(0xFFFFFFFF)
        m0 = jnp.where(rel < DH, ones, jnp.uint32(0))
        m1 = jnp.where((rel >= DH) & (rel < 2 * DH), ones, jnp.uint32(0))
        return _bf(jnp.concatenate([qt & m0, qt & m1], axis=0))

    def qk_a(sl, u, p, i):
        kk = ka_ref[_PAIR[p][0], pl.ds(row0 + i * QC, WA + QC), :]
        s_ref[sl, u] = _nt_dot(kk, masked_q(p, i))

    def sm_a(sl, u, p, i):
        def chunk(c):
            v = s_ref[sl, u, c * QC:(c + 1) * QC, :]
            if c < NCH - i:
                v = jnp.where(not_first, v, NEG)
            return v
        mrg = jnp.where(lower, s_ref[sl, u, WA:WA + QC, :], chunk(0))
        mid = [chunk(c) for c in range(1, 4)]
        m = jnp.max(mrg, axis=0, keepdims=True)
        for v in mid:
            m = jnp.maximum(m, jnp.max(v, axis=0, keepdims=True))
        pg = jnp.exp2(mrg - m)
        l = jnp.sum(pg, axis=0, keepdims=True)
        o = QC * (i % 2)
        p_ref[sl, u, o:o + QC, :] = jnp.where(lower, 0.0, pg).astype(BF)
        p_ref[sl, u, o + WA:o + WA + QC, :] = jnp.where(lower, pg, 0.0).astype(BF)
        for c, v in enumerate(mid):
            pm = jnp.exp2(v - m)
            l = l + jnp.sum(pm, axis=0, keepdims=True)
            p_ref[sl, u, o + (c + 1) * QC:o + (c + 2) * QC, :] = pm.astype(BF)
        z = (WA + QC) if i % 2 == 0 else 0
        p_ref[sl, u, z:z + QC, :] = jnp.zeros((QC, 128), BF)
        l_ref[sl, u] = jnp.broadcast_to(1.0 / l, (8, 128))

    def pv_a(sl, u, p, i):
        r0 = 40 * p - 8 * (p % 2)
        c0 = t * (R // 128) + i // 2
        acc = None
        for j in range(3):
            y = _dot(vta_ref[c0 + j, r0:r0 + 48, :], p_ref[sl, u, j * 128:(j + 1) * 128, :])
            acc = y if acc is None else acc + y
        return acc * l_ref[sl, u][0:1]

    def put(p, mm, r_e, r_o):
        sh = 8 * (p % 2)
        h0 = (row48 - sh) < DH
        tt = jnp.where(left, jnp.where(h0, r_e, pltpu.roll(r_e, 64, 1)),
                       jnp.where(h0, pltpu.roll(r_o, 64, 1), r_o))
        ot_ref[40 * p:40 * p + 40, mm * 128:(mm + 1) * 128] = tt[sh:sh + 40]
        for c in range(NLT):
            if 40 * p < (c + 1) * 128 <= 40 * p + 40:
                oa_ref[mm * 128:(mm + 1) * 128, c * 128:(c + 1) * 128] = (
                    ot_ref[c * 128:(c + 1) * 128, mm * 128:(mm + 1) * 128].astype(BF).T)

    @phase
    def _():
        for n in range(NPAIR + 2):
            res = {}
            for u in range(NCH):
                if n < NPAIR:
                    qk_a(n % 2, u, n, u)
                if 1 <= n <= NPAIR:
                    sm_a((n - 1) % 2, u, n - 1, u)
                if n >= 2:
                    res[u] = pv_a((n - 2) % 2, u, n - 2, u)
                    if u % 2:
                        put(n - 2, u // 2, res[u - 1], res[u])

    @pl.when(t == 0)
    def _():
        copies[6].wait()
        copies[7].wait()
        for c in range(NLT):
            tmp_ref[c] = wob_ref[:, c * 128:(c + 1) * 128].astype(F32)
        permute_rows(wobp_ref)

    for c in range(NLT):
        a = _dot(oa_ref[...], woa_ref[:, c * 128:(c + 1) * 128])
        b = _dot(ob_ref[...], wobp_ref[c])
        o_ref[:, c * 128:(c + 1) * 128] = (g * a + (1.0 - g) * b).astype(o_ref.dtype)


@jax.jit
def pallas_gated_mix__sliding_block__sliding_local_dilated__prompt_kernel(
    A_x: jax.Array,
    A_wqkv: jax.Array,
    A_wo: jax.Array,
    B_x: jax.Array,
    B_wqkv: jax.Array,
    B_wo: jax.Array,
    gate_w: jax.Array,
):
    del B_x
    x = A_x.reshape(S, D)
    gw = gate_w.reshape(1, D)
    hbm = pl.BlockSpec(memory_space=pl.ANY)
    out = pl.pallas_call(
        kernel,
        grid=(S // R,),
        in_specs=[
            pl.BlockSpec((R, D), lambda t: (t, 0)),
            hbm, hbm, hbm, hbm, pl.BlockSpec((1, D), lambda t: (0, 0)),
        ],
        out_specs=pl.BlockSpec((R, D), lambda t: (t, 0)),
        out_shape=jax.ShapeDtypeStruct((S, D), BF),
        scratch_shapes=[
            pltpu.VMEM((3, D, D), BF),
            pltpu.VMEM((D, D), BF),
            pltpu.VMEM((3, D, D), BF),
            pltpu.VMEM((D, D), BF),
            pltpu.SemaphoreType.DMA((8,)),
            pltpu.VMEM((NT, R, 128), BF),
            pltpu.VMEM((NT, WA + S, 128), BF),
            pltpu.VMEM(((WA + S) // 128, D, 128), BF),
            pltpu.VMEM((D, R), F32),
            pltpu.VMEM((R, D), BF),
            pltpu.VMEM((2, NCH, WA + QC, 128), F32),
            pltpu.VMEM((2, NCH, 384, 128), BF),
            pltpu.VMEM((2, NCH, 8, 128), F32),
            pltpu.VMEM((3, NLT, D, 128), BF),
            pltpu.VMEM((NLT, D, 128), BF),
            pltpu.VMEM((NLT, D, 128), F32),
            pltpu.VMEM((NLT, R, 128), F32),
            pltpu.VMEM((NLT, HB + S, 128), F32),
            pltpu.VMEM((NLT, HB + S, 128), F32),
            pltpu.VMEM((R, D), BF),
        ],
        compiler_params=pltpu.CompilerParams(
            dimension_semantics=("arbitrary",),
            vmem_limit_bytes=100 * 1024 * 1024,
        ),
        name="gated_mix_attn",
    )(x, A_wqkv, A_wo, B_wqkv, B_wo, gw)
    return out.reshape(1, S, D)
```

```python
import jax
import jax.numpy as jnp
import numpy as np
import jax.experimental.pallas as pl
import jax.experimental.pallas.tpu as pltpu

S = 2048
D = 640
H = 32
DH = 20
NLT = D // 128
R = 256
QC = 64
NCH = R // QC
NPAIR = H // 2
WA = 256
HB = 16
RB = 16
LINK = 1
NEG = -1e30
LOG2E = 1.4426950408889634
QSCALE = float(DH ** -0.5) * LOG2E
BF = jnp.bfloat16
F32 = jnp.float32


def _pair_tile(p):
    c0 = 40 * p
    t0, off = divmod(c0, 128)
    if off + 40 <= 128:
        return (t0, t0, 0), off
    return (t0, t0 + 1, off), off


_TILES = []
_PAIR = []
for _p in range(NPAIR):
    _t, _o = _pair_tile(_p)
    if _t not in _TILES:
        _TILES.append(_t)
    _PAIR.append((_TILES.index(_t), _o))
NT = len(_TILES)


def _u32(x):
    return pltpu.bitcast(x, jnp.uint32)


def _bf(x):
    return pltpu.bitcast(x, BF)


def _build_tiles(y):
    rows = y.shape[0]
    lane = jax.lax.broadcasted_iota(jnp.int32, (rows, 128), 1)
    out = []
    for (a, b, split) in _TILES:
        ta = y[:, a * 128:(a + 1) * 128]
        if a != b:
            ta = jnp.where(lane >= split, ta, y[:, b * 128:(b + 1) * 128])
        out.append(ta.astype(BF))
    return out


def _nt_dot(a, b):
    return jax.lax.dot_general(a, b, (((1,), (1,)), ((), ())), preferred_element_type=F32)


def _dot(a, b):
    return jnp.dot(a, b, preferred_element_type=F32)


def kernel(x_hbm, wa_hbm, woa_hbm, wb_hbm, wob_hbm, gw_hbm, o_ref,
           x_ref, gw_ref, wa_ref, woa_ref, wb_ref, wob_ref, sems,
           qa_ref, ka_ref, vta_ref, ot_ref, oa_ref, s_ref, p_ref, l_ref,
           wbt_ref, wobp_ref, tmp_ref, qb_ref, kb_ref, vb_ref, ob_ref):
    t = pl.program_id(0)
    not_first = t > 0
    row0 = pl.multiple_of(t * R, R)

    phase = pl.when(t >= 0)

    def sec(ref, i):
        return ref.at[:, pl.ds(i * D, D)]

    copies = [pltpu.make_async_copy(sec(wb_hbm, i), wb_ref.at[i], sems.at[i]) for i in range(3)]
    copies += [pltpu.make_async_copy(sec(wa_hbm, i), wa_ref.at[i], sems.at[3 + i]) for i in range(3)]
    copies += [pltpu.make_async_copy(wob_hbm, wob_ref, sems.at[6]),
               pltpu.make_async_copy(woa_hbm, woa_ref, sems.at[7])]
    x_first = pltpu.make_async_copy(x_hbm.at[pl.ds(0, R)], x_ref.at[pl.ds(0, R)], sems.at[8])
    x_rest = pltpu.make_async_copy(x_hbm.at[pl.ds(R, S - R)], x_ref.at[pl.ds(R, S - R)], sems.at[9])
    gw_copy = pltpu.make_async_copy(gw_hbm, gw_ref, sems.at[10])

    @pl.when(t == 0)
    def _():
        x_first.start()
        copies[0].start()
        copies[1].start()
        gw_copy.start()
        ka_ref[:, 0:WA, :] = jnp.zeros((NT, WA, 128), BF)
        for j in range(WA // 128):
            vta_ref[j] = jnp.zeros((D, 128), BF)
        kb_ref[:, 0:HB, :] = jnp.zeros((NLT, HB, 128), F32)
        vb_ref[:, 0:HB, :] = jnp.zeros((NLT, HB, 128), F32)

        x_first.wait()
        gw_copy.wait()

    @pl.when(t == 1)
    def _():
        x_rest.wait()

    x = x_ref[pl.ds(row0, R), :]

    def permute_rows(dst_ref):
        for c in range(NLT):
            for d in range(DH):
                dst_ref[c, d * H:(d + 1) * H, :] = tmp_ref[c, pl.ds(d, H, stride=DH), :].astype(BF)

    @pl.when(t == 0)
    def _():
        for i in range(3):
            copies[i].wait()
            copies[2 * i + 2].start()
            copies[2 * i + 3].start()
            for c in range(NLT):
                for n in range(NLT):
                    w = wb_ref[i, c * 128:(c + 1) * 128, n * 128:(n + 1) * 128]
                    tmp_ref[c, n * 128:(n + 1) * 128, :] = w.astype(F32).T
            permute_rows(wbt_ref.at[i])

    for i, dst in enumerate((qb_ref, kb_ref, vb_ref)):
        y = None
        for c in range(NLT):
            z = _nt_dot(x[:, c * 128:(c + 1) * 128], wbt_ref[i, c])
            y = z if y is None else y + z
        for c in range(NLT):
            if i == 0:
                dst[c] = y[:, c * 128:(c + 1) * 128] * QSCALE
            else:
                dst[c, pl.ds(row0 + HB, R), :] = y[:, c * 128:(c + 1) * 128]

    @pl.when(t == 0)
    def _():
        x_rest.start()
        for cp in copies[3:6]:
            cp.wait()

    rowb = jax.lax.broadcasted_iota(jnp.int32, (RB, 128), 0)

    never = t < 0
    chain = [None, None]

    def attn_b(ci):
        r = ci * RB
        q = [qb_ref[c, r:r + RB, :] for c in range(NLT)]
        if chain[ci % LINK] is not None:
            q[0] = jnp.where(never, chain[ci % LINK], q[0])
            q[NLT - 1] = jnp.where(never, chain[ci % LINK], q[NLT - 1])
        sc = []
        for j in range(8):
            acc = None
            for c in range(NLT):
                y = q[c] * kb_ref[c, pl.ds(row0 + (r + HB - 2 * j), RB), :]
                acc = y if acc is None else acc + y
            acc = acc + pltpu.roll(acc, 64, 1)
            acc = acc + pltpu.roll(acc, 32, 1)
            if r < 2 * j:
                acc = jnp.where(not_first | (rowb >= 2 * j - r), acc, NEG)
            sc.append(acc)
        m = sc[0]
        for y in sc[1:]:
            m = jnp.maximum(m, y)
        e = [jnp.exp2(y - m) for y in sc]
        l = e[0]
        for y in e[1:]:
            l = l + y
        inv = 1.0 / l
        for c in range(NLT):
            acc = None
            for j in range(8):
                y = e[j] * vb_ref[c, pl.ds(row0 + (r + HB - 2 * j), RB), :]
                acc = y if acc is None else acc + y
            ob_ref[r:r + RB, c * 128:(c + 1) * 128] = (acc * inv).astype(BF)
        chain[ci % LINK] = acc

    @phase
    def _():
        nb = R // RB
        q = _dot(x, wa_ref[0]) * QSCALE
        for i, tl in enumerate(_build_tiles(q)):
            qa_ref[i] = tl
        for ci in range(0, nb // 3):
            attn_b(ci)
        k = _dot(x, wa_ref[1])
        for i, tl in enumerate(_build_tiles(k)):
            ka_ref[i, pl.ds(row0 + WA, R), :] = tl
        for ci in range(nb // 3, 2 * nb // 3):
            attn_b(ci)
        va = _dot(x, wa_ref[2]).astype(BF)
        for j in range(R // 128):
            vta_ref[t * (R // 128) + WA // 128 + j] = va[j * 128:(j + 1) * 128, :].T
        for ci in range(2 * nb // 3, nb):
            attn_b(ci)


    lane128 = jax.lax.broadcasted_iota(jnp.int32, (QC, 128), 1)
    row64 = jax.lax.broadcasted_iota(jnp.int32, (QC, 128), 0)
    lower = row64 <= (lane128 & (QC - 1))
    lane32 = jax.lax.broadcasted_iota(jnp.int32, (QC // 2, 128), 1)
    row48 = jax.lax.broadcasted_iota(jnp.int32, (48, 128), 0)
    lane48 = jax.lax.broadcasted_iota(jnp.int32, (48, 128), 1)
    left = lane48 < 64

    def masked_q(p, i):
        tix, off = _PAIR[p]
        qt = _u32(qa_ref[tix, i * QC:(i + 1) * QC, :])
        rel = (lane32 - off) & 127
        ones = jnp.uint32(0xFFFFFFFF)
        m0 = jnp.where(rel < DH, ones, jnp.uint32(0))
        m1 = jnp.where((rel >= DH) & (rel < 2 * DH), ones, jnp.uint32(0))
        return _bf(jnp.concatenate([qt & m0, qt & m1], axis=0))

    def qk_a(sl, u, p, i):
        kk = ka_ref[_PAIR[p][0], pl.ds(row0 + i * QC, WA + QC), :]
        s_ref[sl, u] = _nt_dot(kk, masked_q(p, i))

    def sm_a(sl, u, p, i):
        def chunk(c):
            v = s_ref[sl, u, c * QC:(c + 1) * QC, :]
            if c < NCH - i:
                v = jnp.where(not_first, v, NEG)
            return v
        mrg = jnp.where(lower, s_ref[sl, u, WA:WA + QC, :], chunk(0))
        mid = [chunk(c) for c in range(1, 4)]
        m = jnp.max(mrg, axis=0, keepdims=True)
        for v in mid:
            m = jnp.maximum(m, jnp.max(v, axis=0, keepdims=True))
        pg = jnp.exp2(mrg - m)
        l = jnp.sum(pg, axis=0, keepdims=True)
        o = QC * (i % 2)
        p_ref[sl, u, o:o + QC, :] = jnp.where(lower, 0.0, pg).astype(BF)
        p_ref[sl, u, o + WA:o + WA + QC, :] = jnp.where(lower, pg, 0.0).astype(BF)
        for c, v in enumerate(mid):
            pm = jnp.exp2(v - m)
            l = l + jnp.sum(pm, axis=0, keepdims=True)
            p_ref[sl, u, o + (c + 1) * QC:o + (c + 2) * QC, :] = pm.astype(BF)
        z = (WA + QC) if i % 2 == 0 else 0
        p_ref[sl, u, z:z + QC, :] = jnp.zeros((QC, 128), BF)
        l_ref[sl, u] = jnp.broadcast_to(1.0 / l, (8, 128))

    def pv_a(sl, u, p, i):
        r0 = 40 * p - 8 * (p % 2)
        c0 = t * (R // 128) + i // 2
        acc = None
        for j in range(3):
            y = _dot(vta_ref[c0 + j, r0:r0 + 48, :], p_ref[sl, u, j * 128:(j + 1) * 128, :])
            acc = y if acc is None else acc + y
        return acc * l_ref[sl, u][0:1]

    def put(p, mm, r_e, r_o):
        sh = 8 * (p % 2)
        h0 = (row48 - sh) < DH
        tt = jnp.where(left, jnp.where(h0, r_e, pltpu.roll(r_e, 64, 1)),
                       jnp.where(h0, pltpu.roll(r_o, 64, 1), r_o))
        ot_ref[40 * p:40 * p + 40, mm * 128:(mm + 1) * 128] = tt[sh:sh + 40]
        for c in range(NLT):
            if 40 * p < (c + 1) * 128 <= 40 * p + 40:
                oa_ref[mm * 128:(mm + 1) * 128, c * 128:(c + 1) * 128] = (
                    ot_ref[c * 128:(c + 1) * 128, mm * 128:(mm + 1) * 128].astype(BF).T)

    @phase
    def _():
        for n in range(NPAIR + 2):
            res = {}
            for u in range(NCH):
                if n < NPAIR:
                    qk_a(n % 2, u, n, u)
                if 1 <= n <= NPAIR:
                    sm_a((n - 1) % 2, u, n - 1, u)
                if n >= 2:
                    res[u] = pv_a((n - 2) % 2, u, n - 2, u)
                    if u % 2:
                        put(n - 2, u // 2, res[u - 1], res[u])

    @pl.when(t == 0)
    def _():
        copies[6].wait()
        copies[7].wait()
        for c in range(NLT):
            tmp_ref[c] = wob_ref[:, c * 128:(c + 1) * 128].astype(F32)
        permute_rows(wobp_ref)

    gl = jnp.sum(x.astype(F32) * gw_ref[...].astype(F32), axis=1, keepdims=True)
    g = jax.nn.sigmoid(gl)
    for c in range(NLT):
        a = _dot(oa_ref[...], woa_ref[:, c * 128:(c + 1) * 128])
        b = _dot(ob_ref[...], wobp_ref[c])
        o_ref[:, c * 128:(c + 1) * 128] = (g * a + (1.0 - g) * b).astype(o_ref.dtype)


@jax.jit
def pallas_gated_mix__sliding_block__sliding_local_dilated__prompt_kernel(
    A_x: jax.Array,
    A_wqkv: jax.Array,
    A_wo: jax.Array,
    B_x: jax.Array,
    B_wqkv: jax.Array,
    B_wo: jax.Array,
    gate_w: jax.Array,
):
    del B_x
    x = A_x.reshape(S, D)
    gw = gate_w.reshape(1, D)
    hbm = pl.BlockSpec(memory_space=pl.ANY)
    out = pl.pallas_call(
        kernel,
        grid=(S // R,),
        in_specs=[hbm] * 6,
        out_specs=pl.BlockSpec((R, D), lambda t: (t, 0)),
        out_shape=jax.ShapeDtypeStruct((S, D), BF),
        scratch_shapes=[
            pltpu.VMEM((S, D), BF),
            pltpu.VMEM((1, D), BF),
            pltpu.VMEM((3, D, D), BF),
            pltpu.VMEM((D, D), BF),
            pltpu.VMEM((3, D, D), BF),
            pltpu.VMEM((D, D), BF),
            pltpu.SemaphoreType.DMA((11,)),
            pltpu.VMEM((NT, R, 128), BF),
            pltpu.VMEM((NT, WA + S, 128), BF),
            pltpu.VMEM(((WA + S) // 128, D, 128), BF),
            pltpu.VMEM((D, R), F32),
            pltpu.VMEM((R, D), BF),
            pltpu.VMEM((2, NCH, WA + QC, 128), F32),
            pltpu.VMEM((2, NCH, 384, 128), BF),
            pltpu.VMEM((2, NCH, 8, 128), F32),
            pltpu.VMEM((3, NLT, D, 128), BF),
            pltpu.VMEM((NLT, D, 128), BF),
            pltpu.VMEM((NLT, D, 128), F32),
            pltpu.VMEM((NLT, R, 128), F32),
            pltpu.VMEM((NLT, HB + S, 128), F32),
            pltpu.VMEM((NLT, HB + S, 128), F32),
            pltpu.VMEM((R, D), BF),
        ],
        compiler_params=pltpu.CompilerParams(
            dimension_semantics=("arbitrary",),
            vmem_limit_bytes=100 * 1024 * 1024,
        ),
        name="gated_mix_attn",
    )(x, A_wqkv, A_wo, B_wqkv, B_wo, gw)
    return out.reshape(1, S, D)
```

```python
import jax
import jax.numpy as jnp
import numpy as np
import jax.experimental.pallas as pl
import jax.experimental.pallas.tpu as pltpu

S = 2048
D = 640
H = 32
DH = 20
NLT = D // 128
R = 256
QC = 64
NCH = R // QC
NPAIR = H // 2
WA = 256
HB = 16
RB = 16
LINK = 1
NEG = -1e30
LOG2E = 1.4426950408889634
QSCALE = float(DH ** -0.5) * LOG2E
BF = jnp.bfloat16
U32 = jnp.uint32
F32 = jnp.float32


def _pair_tile(p):
    c0 = 40 * p
    t0, off = divmod(c0, 128)
    if off + 40 <= 128:
        return (t0, t0, 0), off
    return (t0, t0 + 1, off), off


_TILES = []
_PAIR = []
for _p in range(NPAIR):
    _t, _o = _pair_tile(_p)
    if _t not in _TILES:
        _TILES.append(_t)
    _PAIR.append((_TILES.index(_t), _o))
NT = len(_TILES)


def _u32(x):
    return pltpu.bitcast(x, jnp.uint32)


def _bf(x):
    return pltpu.bitcast(x, BF)


def _build_tiles(y):
    rows = y.shape[0]
    lane = jax.lax.broadcasted_iota(jnp.int32, (rows, 128), 1)
    out = []
    for (a, b, split) in _TILES:
        ta = y[:, a * 128:(a + 1) * 128]
        if a != b:
            ta = jnp.where(lane >= split, ta, y[:, b * 128:(b + 1) * 128])
        out.append(_u32(ta.astype(BF)))
    return out


def _pack16(y):
    g = y.shape[0] // 16
    y = y.reshape(g, 2, 8, y.shape[1])
    return pltpu.pack_elementwise(
        [y[:, 0].reshape(8 * g, -1), y[:, 1].reshape(8 * g, -1)], packed_dtype=BF)


def _nt_dot(a, b):
    return jax.lax.dot_general(a, b, (((1,), (1,)), ((), ())), preferred_element_type=F32)


def _dot(a, b):
    return jnp.dot(a, b, preferred_element_type=F32)


def kernel(x_hbm, wa_hbm, woa_hbm, wb_hbm, wob_hbm, gw_hbm, o_ref,
           x_ref, gw_ref, wa_ref, woa_ref, wb_ref, wob_ref, sems,
           qa_ref, ka_ref, vta_ref, ot_ref, oa_ref, s_ref, p_ref,
           wbt_ref, wobp_ref, tmp_ref, qb_ref, kb_ref, vb_ref, ob_ref):
    t = pl.program_id(0)
    not_first = t > 0
    row0 = pl.multiple_of(t * R, R)
    prow0 = pl.multiple_of(t * (R // 2), R // 2)

    phase = pl.when(t >= 0)

    def sec(ref, i):
        return ref.at[:, pl.ds(i * D, D)]

    copies = [pltpu.make_async_copy(sec(wb_hbm, i), wb_ref.at[i], sems.at[i]) for i in range(3)]
    copies += [pltpu.make_async_copy(sec(wa_hbm, i), wa_ref.at[i], sems.at[3 + i]) for i in range(3)]
    copies += [pltpu.make_async_copy(wob_hbm, wob_ref, sems.at[6]),
               pltpu.make_async_copy(woa_hbm, woa_ref, sems.at[7])]
    x_first = pltpu.make_async_copy(x_hbm.at[pl.ds(0, R)], x_ref.at[pl.ds(0, R)], sems.at[8])
    x_rest = pltpu.make_async_copy(x_hbm.at[pl.ds(R, S - R)], x_ref.at[pl.ds(R, S - R)], sems.at[9])
    gw_copy = pltpu.make_async_copy(gw_hbm, gw_ref, sems.at[10])

    @pl.when(t == 0)
    def _():
        x_first.start()
        copies[0].start()
        copies[1].start()
        gw_copy.start()
        ka_ref[:, 0:WA // 2, :] = jnp.zeros((NT, WA // 2, 128), U32)
        for j in range(WA // 128):
            vta_ref[j] = jnp.zeros((D // 2, 128), U32)
        for u in range(NCH):
            z = (WA + QC) // 2 if u % 2 == 0 else 0
            p_ref[:, u, z:z + QC // 2, :] = jnp.zeros((2, QC // 2, 128), U32)
        kb_ref[:, 0:HB, :] = jnp.zeros((NLT, HB, 128), F32)
        vb_ref[:, 0:HB, :] = jnp.zeros((NLT, HB, 128), F32)

        x_first.wait()
        gw_copy.wait()

    @pl.when(t == 1)
    def _():
        x_rest.wait()

    x = x_ref[pl.ds(row0, R), :]

    def permute_rows(dst_ref):
        for c in range(NLT):
            for d in range(DH):
                dst_ref[c, d * H:(d + 1) * H, :] = tmp_ref[c, pl.ds(d, H, stride=DH), :].astype(BF)

    @pl.when(t == 0)
    def _():
        for i in range(3):
            copies[i].wait()
            copies[2 * i + 2].start()
            copies[2 * i + 3].start()
            for c in range(NLT):
                for n in range(NLT):
                    w = wb_ref[i, c * 128:(c + 1) * 128, n * 128:(n + 1) * 128]
                    tmp_ref[c, n * 128:(n + 1) * 128, :] = w.astype(F32).T
            permute_rows(wbt_ref.at[i])

    for i, dst in enumerate((qb_ref, kb_ref, vb_ref)):
        y = None
        for c in range(NLT):
            z = _nt_dot(x[:, c * 128:(c + 1) * 128], wbt_ref[i, c])
            y = z if y is None else y + z
        for c in range(NLT):
            if i == 0:
                dst[c] = y[:, c * 128:(c + 1) * 128] * QSCALE
            else:
                dst[c, pl.ds(row0 + HB, R), :] = y[:, c * 128:(c + 1) * 128]

    @pl.when(t == 0)
    def _():
        x_rest.start()
        for cp in copies[3:6]:
            cp.wait()

    rowb = jax.lax.broadcasted_iota(jnp.int32, (RB, 128), 0)

    never = t < 0
    chain = [None, None]

    def attn_b(ci):
        r = ci * RB
        q = [qb_ref[c, r:r + RB, :] for c in range(NLT)]
        if chain[ci % LINK] is not None:
            q[0] = jnp.where(never, chain[ci % LINK], q[0])
            q[NLT - 1] = jnp.where(never, chain[ci % LINK], q[NLT - 1])
        sc = []
        for j in range(8):
            acc = None
            for c in range(NLT):
                y = q[c] * kb_ref[c, pl.ds(row0 + (r + HB - 2 * j), RB), :]
                acc = y if acc is None else acc + y
            acc = acc + pltpu.roll(acc, 64, 1)
            acc = acc + pltpu.roll(acc, 32, 1)
            if r < 2 * j:
                acc = jnp.where(not_first | (rowb >= 2 * j - r), acc, NEG)
            sc.append(acc)
        m = sc[0]
        for y in sc[1:]:
            m = jnp.maximum(m, y)
        e = [jnp.exp2(y - m) for y in sc]
        l = e[0]
        for y in e[1:]:
            l = l + y
        inv = 1.0 / l
        for c in range(NLT):
            acc = None
            for j in range(8):
                y = e[j] * vb_ref[c, pl.ds(row0 + (r + HB - 2 * j), RB), :]
                acc = y if acc is None else acc + y
            ob_ref[r:r + RB, c * 128:(c + 1) * 128] = (acc * inv).astype(BF)
        chain[ci % LINK] = acc

    @phase
    def _():
        nb = R // RB
        q = _dot(x, wa_ref[0]) * QSCALE
        for i, tl in enumerate(_build_tiles(q)):
            qa_ref[i] = tl
        for ci in range(0, nb // 3):
            attn_b(ci)
        k = _dot(x, wa_ref[1])
        for i, tl in enumerate(_build_tiles(k)):
            ka_ref[i, pl.ds(prow0 + WA // 2, R // 2), :] = tl
        for ci in range(nb // 3, 2 * nb // 3):
            attn_b(ci)
        va = _bf(_pack16(_dot(x, wa_ref[2])).astype(U32))
        for j in range(R // 128):
            vta_ref[t * (R // 128) + WA // 128 + j] = _u32(va[j * 128:(j + 1) * 128, :].T)
        for ci in range(2 * nb // 3, nb):
            attn_b(ci)


    lane128 = jax.lax.broadcasted_iota(jnp.int32, (QC, 128), 1)
    row64 = jax.lax.broadcasted_iota(jnp.int32, (QC, 128), 0)
    lower = row64 <= (lane128 & (QC - 1))
    lane32 = jax.lax.broadcasted_iota(jnp.int32, (QC // 2, 128), 1)
    row48 = jax.lax.broadcasted_iota(jnp.int32, (48, 128), 0)
    lane48 = jax.lax.broadcasted_iota(jnp.int32, (48, 128), 1)
    left = lane48 < 64

    def masked_q(p, i):
        tix, off = _PAIR[p]
        qt = qa_ref[tix, i * QC // 2:(i + 1) * QC // 2, :]
        rel = (lane32 - off) & 127
        ones = jnp.uint32(0xFFFFFFFF)
        m0 = jnp.where(rel < DH, ones, jnp.uint32(0))
        m1 = jnp.where((rel >= DH) & (rel < 2 * DH), ones, jnp.uint32(0))
        return _bf(jnp.concatenate([qt & m0, qt & m1], axis=0))

    def qk_a(sl, u, p, i):
        kk = _bf(ka_ref[_PAIR[p][0], pl.ds(prow0 + i * QC // 2, (WA + QC) // 2), :])
        s_ref[sl, u] = _nt_dot(kk, masked_q(p, i))

    def sm_a(sl, u, i, first):
        def chunk(c):
            if first and c < NCH - i:
                return None
            return s_ref[sl, u, c * QC:(c + 1) * QC, :]

        def put_p(c, v):
            o = (QC * (i % 2) + c * QC) // 2
            p_ref[sl, u, o:o + QC // 2, :] = (
                jnp.zeros((QC // 2, 128), U32) if v is None else _pack16(v).astype(U32))

        mrg = jnp.where(lower, s_ref[sl, u, WA:WA + QC, :], NEG if chunk(0) is None else chunk(0))
        mid = [chunk(c) for c in range(1, 4)]
        m = jnp.max(mrg, axis=0, keepdims=True)
        for v in mid:
            if v is not None:
                m = jnp.maximum(m, jnp.max(v, axis=0, keepdims=True))
        pg = jnp.exp2(mrg - m)
        put_p(0, jnp.where(lower, 0.0, pg))
        put_p(4, jnp.where(lower, pg, 0.0))
        for c, v in enumerate(mid):
            put_p(c + 1, None if v is None else jnp.exp2(v - m))

    word = jax.lax.broadcasted_iota(jnp.int32, (8, 128), 0)
    ones_w = jnp.uint32(0x3F803F80)

    def pv_a(sl, u, p, i):
        w0 = 20 * p - 4 * (p % 2)
        c0 = t * (R // 128) + i // 2
        acc = None
        for j in range(3):
            v = vta_ref[c0 + j, w0:w0 + 24, :]
            if p % 2:
                v = jnp.concatenate([jnp.where(word < 4, ones_w, v[0:8]), v[8:24]], axis=0)
            else:
                v = jnp.concatenate([v[0:16], jnp.where(word >= 4, ones_w, v[16:24])], axis=0)
            y = _dot(_bf(v), _bf(p_ref[sl, u, j * 64:(j + 1) * 64, :]))
            acc = y if acc is None else acc + y
        if p % 2:
            return acc[8:48] * jnp.tile(1.0 / acc[0:8], (5, 1))
        return acc[0:40] * jnp.tile(1.0 / acc[40:48], (5, 1))

    row40 = jax.lax.broadcasted_iota(jnp.int32, (40, 128), 0)
    left = jax.lax.broadcasted_iota(jnp.int32, (40, 128), 1) < 64

    def put(p, mm, r_e, r_o):
        h0 = row40 < DH
        tt = jnp.where(left, jnp.where(h0, r_e, pltpu.roll(r_e, 64, 1)),
                       jnp.where(h0, pltpu.roll(r_o, 64, 1), r_o))
        ot_ref[40 * p:40 * p + 40, mm * 128:(mm + 1) * 128] = tt
        for c in range(NLT):
            if 40 * p < (c + 1) * 128 <= 40 * p + 40:
                oa_ref[mm * 128:(mm + 1) * 128, c * 128:(c + 1) * 128] = (
                    ot_ref[c * 128:(c + 1) * 128, mm * 128:(mm + 1) * 128].astype(BF).T)

    def attn_a(first):
        for n in range(NPAIR + 2):
            res = {}
            for u in range(NCH):
                if n < NPAIR:
                    qk_a(n % 2, u, n, u)
                if 1 <= n <= NPAIR:
                    sm_a((n - 1) % 2, u, u, first)
                if n >= 2:
                    res[u] = pv_a((n - 2) % 2, u, n - 2, u)
                    if u % 2:
                        put(n - 2, u // 2, res[u - 1], res[u])

    pl.when(t == 0)(lambda: attn_a(True))
    pl.when(t > 0)(lambda: attn_a(False))

    @pl.when(t == 0)
    def _():
        copies[6].wait()
        copies[7].wait()
        for c in range(NLT):
            tmp_ref[c] = wob_ref[:, c * 128:(c + 1) * 128].astype(F32)
        permute_rows(wobp_ref)

    gl = jnp.sum(x.astype(F32) * gw_ref[...].astype(F32), axis=1, keepdims=True)
    g = jax.nn.sigmoid(gl)
    for c in range(NLT):
        a = _dot(oa_ref[...], woa_ref[:, c * 128:(c + 1) * 128])
        b = _dot(ob_ref[...], wobp_ref[c])
        o_ref[:, c * 128:(c + 1) * 128] = (g * a + (1.0 - g) * b).astype(o_ref.dtype)


@jax.jit
def pallas_gated_mix__sliding_block__sliding_local_dilated__prompt_kernel(
    A_x: jax.Array,
    A_wqkv: jax.Array,
    A_wo: jax.Array,
    B_x: jax.Array,
    B_wqkv: jax.Array,
    B_wo: jax.Array,
    gate_w: jax.Array,
):
    del B_x
    x = A_x.reshape(S, D)
    gw = gate_w.reshape(1, D)
    hbm = pl.BlockSpec(memory_space=pl.ANY)
    out = pl.pallas_call(
        kernel,
        grid=(S // R,),
        in_specs=[hbm] * 6,
        out_specs=pl.BlockSpec((R, D), lambda t: (t, 0)),
        out_shape=jax.ShapeDtypeStruct((S, D), BF),
        scratch_shapes=[
            pltpu.VMEM((S, D), BF),
            pltpu.VMEM((1, D), BF),
            pltpu.VMEM((3, D, D), BF),
            pltpu.VMEM((D, D), BF),
            pltpu.VMEM((3, D, D), BF),
            pltpu.VMEM((D, D), BF),
            pltpu.SemaphoreType.DMA((11,)),
            pltpu.VMEM((NT, R // 2, 128), U32),
            pltpu.VMEM((NT, (WA + S) // 2, 128), U32),
            pltpu.VMEM(((WA + S) // 128, D // 2, 128), U32),
            pltpu.VMEM((D, R), F32),
            pltpu.VMEM((R, D), BF),
            pltpu.VMEM((2, NCH, WA + QC, 128), F32),
            pltpu.VMEM((2, NCH, 192, 128), U32),
            pltpu.VMEM((3, NLT, D, 128), BF),
            pltpu.VMEM((NLT, D, 128), BF),
            pltpu.VMEM((NLT, D, 128), F32),
            pltpu.VMEM((NLT, R, 128), F32),
            pltpu.VMEM((NLT, HB + S, 128), F32),
            pltpu.VMEM((NLT, HB + S, 128), F32),
            pltpu.VMEM((R, D), BF),
        ],
        compiler_params=pltpu.CompilerParams(
            dimension_semantics=("arbitrary",),
            vmem_limit_bytes=100 * 1024 * 1024,
        ),
        name="gated_mix_attn",
    )(x, A_wqkv, A_wo, B_wqkv, B_wo, gw)
    return out.reshape(1, S, D)
```

```python
import jax
import jax.numpy as jnp
import numpy as np
import jax.experimental.pallas as pl
import jax.experimental.pallas.tpu as pltpu

S = 2048
D = 640
H = 32
DH = 20
NLT = D // 128
R = 512
QC = 64
NU = 4
NBAT = R // (QC * NU)
NPAIR = H // 2
WA = 256
HB = 16
RB = 16
NB1 = 18
LINK = 1
NEG = -1e30
LOG2E = 1.4426950408889634
QSCALE = float(DH ** -0.5) * LOG2E
BF = jnp.bfloat16
U32 = jnp.uint32
F32 = jnp.float32


def _pair_tile(p):
    c0 = 40 * p
    t0, off = divmod(c0, 128)
    if off + 40 <= 128:
        return (t0, t0, 0), off
    return (t0, t0 + 1, off), off


_TILES = []
_PAIR = []
for _p in range(NPAIR):
    _t, _o = _pair_tile(_p)
    if _t not in _TILES:
        _TILES.append(_t)
    _PAIR.append((_TILES.index(_t), _o))
NT = len(_TILES)


def _u32(x):
    return pltpu.bitcast(x, jnp.uint32)


def _bf(x):
    return pltpu.bitcast(x, BF)


def _build_tiles(y):
    rows = y.shape[0]
    lane = jax.lax.broadcasted_iota(jnp.int32, (rows, 128), 1)
    out = []
    for (a, b, split) in _TILES:
        ta = y[:, a * 128:(a + 1) * 128]
        if a != b:
            ta = jnp.where(lane >= split, ta, y[:, b * 128:(b + 1) * 128])
        out.append(_u32(ta.astype(BF)))
    return out


def _pack16(y):
    g = y.shape[0] // 16
    y = y.reshape(g, 2, 8, y.shape[1])
    return pltpu.pack_elementwise(
        [y[:, 0].reshape(8 * g, -1), y[:, 1].reshape(8 * g, -1)], packed_dtype=BF)


def _nt_dot(a, b):
    return jax.lax.dot_general(a, b, (((1,), (1,)), ((), ())), preferred_element_type=F32)


def _dot(a, b):
    return jnp.dot(a, b, preferred_element_type=F32)


def kernel(x_hbm, wa_hbm, woa_hbm, wb_hbm, wob_hbm, gw_hbm, o_ref,
           x_ref, gw_ref, wa_ref, woa_ref, wb_ref, wob_ref, sems,
           qa_ref, ka_ref, vta_ref, ot_ref, oa_ref, s_ref, p_ref,
           wbt_ref, wobp_ref, tmp_ref, qb_ref, kb_ref, vb_ref, ob_ref):
    t = pl.program_id(0)
    not_first = t > 0
    row0 = pl.multiple_of(t * R, R)
    prow0 = pl.multiple_of(t * (R // 2), R // 2)

    phase = pl.when(t >= 0)

    def sec(ref, i):
        return ref.at[:, pl.ds(i * D, D)]

    copies = [pltpu.make_async_copy(sec(wb_hbm, i), wb_ref.at[i], sems.at[i]) for i in range(3)]
    copies += [pltpu.make_async_copy(sec(wa_hbm, i), wa_ref.at[i], sems.at[3 + i]) for i in range(3)]
    copies += [pltpu.make_async_copy(wob_hbm, wob_ref, sems.at[6]),
               pltpu.make_async_copy(woa_hbm, woa_ref, sems.at[7])]
    x_first = pltpu.make_async_copy(x_hbm.at[pl.ds(0, R)], x_ref.at[pl.ds(0, R)], sems.at[8])
    x_rest = pltpu.make_async_copy(x_hbm.at[pl.ds(R, S - R)], x_ref.at[pl.ds(R, S - R)], sems.at[9])
    gw_copy = pltpu.make_async_copy(gw_hbm, gw_ref, sems.at[10])

    @pl.when(t == 0)
    def _():
        x_first.start()
        copies[0].start()
        copies[1].start()
        gw_copy.start()
        ka_ref[:, 0:WA // 2, :] = jnp.zeros((NT, WA // 2, 128), U32)
        for j in range(WA // 128):
            vta_ref[j] = jnp.zeros((D // 2, 128), U32)
        for u in range(NU):
            z = (WA + QC) // 2 if u % 2 == 0 else 0
            p_ref[:, u, z:z + QC // 2, :] = jnp.zeros((2, QC // 2, 128), U32)
        kb_ref[:, 0:HB, :] = jnp.zeros((NLT, HB, 128), F32)
        vb_ref[:, 0:HB, :] = jnp.zeros((NLT, HB, 128), F32)

        x_first.wait()
        gw_copy.wait()

    @pl.when(t == 1)
    def _():
        x_rest.wait()

    x = x_ref[pl.ds(row0, R), :]

    def permute_rows(dst_ref):
        for c in range(NLT):
            for d in range(DH):
                dst_ref[c, d * H:(d + 1) * H, :] = tmp_ref[c, pl.ds(d, H, stride=DH), :].astype(BF)

    @pl.when(t == 0)
    def _():
        for i in range(3):
            copies[i].wait()
            copies[2 * i + 2].start()
            copies[2 * i + 3].start()
            for c in range(NLT):
                for n in range(NLT):
                    w = wb_ref[i, c * 128:(c + 1) * 128, n * 128:(n + 1) * 128]
                    tmp_ref[c, n * 128:(n + 1) * 128, :] = w.astype(F32).T
            permute_rows(wbt_ref.at[i])

    for i, dst in enumerate((qb_ref, kb_ref, vb_ref)):
        y = None
        for c in range(NLT):
            z = _nt_dot(x[:, c * 128:(c + 1) * 128], wbt_ref[i, c])
            y = z if y is None else y + z
        for c in range(NLT):
            if i == 0:
                dst[c] = y[:, c * 128:(c + 1) * 128] * QSCALE
            else:
                dst[c, pl.ds(row0 + HB, R), :] = y[:, c * 128:(c + 1) * 128]

    @pl.when(t == 0)
    def _():
        x_rest.start()
        for cp in copies[3:6]:
            cp.wait()

    rowb = jax.lax.broadcasted_iota(jnp.int32, (RB, 128), 0)

    never = t < 0
    chain = [None, None]

    def attn_b(ci):
        r = ci * RB
        q = [qb_ref[c, r:r + RB, :] for c in range(NLT)]
        if chain[ci % LINK] is not None:
            q[0] = jnp.where(never, chain[ci % LINK], q[0])
            q[NLT - 1] = jnp.where(never, chain[ci % LINK], q[NLT - 1])
        sc = []
        for j in range(8):
            acc = None
            for c in range(NLT):
                y = q[c] * kb_ref[c, pl.ds(row0 + (r + HB - 2 * j), RB), :]
                acc = y if acc is None else acc + y
            acc = acc + pltpu.roll(acc, 64, 1)
            acc = acc + pltpu.roll(acc, 32, 1)
            if r < 2 * j:
                acc = jnp.where(not_first | (rowb >= 2 * j - r), acc, NEG)
            sc.append(acc)
        m = sc[0]
        for y in sc[1:]:
            m = jnp.maximum(m, y)
        e = [jnp.exp2(y - m) for y in sc]
        l = e[0]
        for y in e[1:]:
            l = l + y
        inv = 1.0 / l
        for c in range(NLT):
            acc = None
            for j in range(8):
                y = e[j] * vb_ref[c, pl.ds(row0 + (r + HB - 2 * j), RB), :]
                acc = y if acc is None else acc + y
            ob_ref[r:r + RB, c * 128:(c + 1) * 128] = (acc * inv).astype(BF)
        chain[ci % LINK] = acc

    @phase
    def _():
        q = _dot(x, wa_ref[0]) * QSCALE
        for i, tl in enumerate(_build_tiles(q)):
            qa_ref[i] = tl
        for ci in range(0, NB1 // 3):
            attn_b(ci)
        k = _dot(x, wa_ref[1])
        for i, tl in enumerate(_build_tiles(k)):
            ka_ref[i, pl.ds(prow0 + WA // 2, R // 2), :] = tl
        for ci in range(NB1 // 3, 2 * NB1 // 3):
            attn_b(ci)
        va = _bf(_pack16(_dot(x, wa_ref[2])).astype(U32))
        for j in range(R // 128):
            vta_ref[t * (R // 128) + WA // 128 + j] = _u32(va[j * 128:(j + 1) * 128, :].T)
        for ci in range(2 * NB1 // 3, NB1):
            attn_b(ci)


    lane128 = jax.lax.broadcasted_iota(jnp.int32, (QC, 128), 1)
    row64 = jax.lax.broadcasted_iota(jnp.int32, (QC, 128), 0)
    lower = row64 <= (lane128 & (QC - 1))
    lane32 = jax.lax.broadcasted_iota(jnp.int32, (QC // 2, 128), 1)
    row48 = jax.lax.broadcasted_iota(jnp.int32, (48, 128), 0)
    lane48 = jax.lax.broadcasted_iota(jnp.int32, (48, 128), 1)
    left = lane48 < 64

    def masked_q(p, i):
        tix, off = _PAIR[p]
        qt = qa_ref[tix, i * QC // 2:(i + 1) * QC // 2, :]
        rel = (lane32 - off) & 127
        ones = jnp.uint32(0xFFFFFFFF)
        m0 = jnp.where(rel < DH, ones, jnp.uint32(0))
        m1 = jnp.where((rel >= DH) & (rel < 2 * DH), ones, jnp.uint32(0))
        return _bf(jnp.concatenate([qt & m0, qt & m1], axis=0))

    def qk_a(sl, u, p, i):
        kk = _bf(ka_ref[_PAIR[p][0], pl.ds(prow0 + i * QC // 2, (WA + QC) // 2), :])
        s_ref[sl, u] = _nt_dot(kk, masked_q(p, i))

    def sm_a(sl, u, i, first):
        def chunk(c):
            if first and c < WA // QC - i:
                return None
            return s_ref[sl, u, c * QC:(c + 1) * QC, :]

        def put_p(c, v):
            o = (QC * (i % 2) + c * QC) // 2
            p_ref[sl, u, o:o + QC // 2, :] = (
                jnp.zeros((QC // 2, 128), U32) if v is None else _pack16(v).astype(U32))

        mrg = jnp.where(lower, s_ref[sl, u, WA:WA + QC, :], NEG if chunk(0) is None else chunk(0))
        mid = [chunk(c) for c in range(1, 4)]
        m = jnp.max(mrg, axis=0, keepdims=True)
        for v in mid:
            if v is not None:
                m = jnp.maximum(m, jnp.max(v, axis=0, keepdims=True))
        pg = jnp.exp2(mrg - m)
        put_p(0, jnp.where(lower, 0.0, pg))
        put_p(4, jnp.where(lower, pg, 0.0))
        for c, v in enumerate(mid):
            put_p(c + 1, None if v is None else jnp.exp2(v - m))

    word = jax.lax.broadcasted_iota(jnp.int32, (8, 128), 0)
    ones_w = jnp.uint32(0x3F803F80)

    def pv_a(sl, u, p, i):
        w0 = 20 * p - 4 * (p % 2)
        c0 = t * (R // 128) + i // 2
        acc = None
        for j in range(3):
            v = vta_ref[c0 + j, w0:w0 + 24, :]
            if p % 2:
                v = jnp.concatenate([jnp.where(word < 4, ones_w, v[0:8]), v[8:24]], axis=0)
            else:
                v = jnp.concatenate([v[0:16], jnp.where(word >= 4, ones_w, v[16:24])], axis=0)
            y = _dot(_bf(v), _bf(p_ref[sl, u, j * 64:(j + 1) * 64, :]))
            acc = y if acc is None else acc + y
        if p % 2:
            return acc[8:48] * jnp.tile(1.0 / acc[0:8], (5, 1))
        return acc[0:40] * jnp.tile(1.0 / acc[40:48], (5, 1))

    row40 = jax.lax.broadcasted_iota(jnp.int32, (40, 128), 0)
    left = jax.lax.broadcasted_iota(jnp.int32, (40, 128), 1) < 64

    def put(p, mm, r_e, r_o):
        h0 = row40 < DH
        tt = jnp.where(left, jnp.where(h0, r_e, pltpu.roll(r_e, 64, 1)),
                       jnp.where(h0, pltpu.roll(r_o, 64, 1), r_o))
        ot_ref[40 * p:40 * p + 40, mm * 128:(mm + 1) * 128] = tt
        for c in range(NLT):
            if 40 * p < (c + 1) * 128 <= 40 * p + 40:
                oa_ref[mm * 128:(mm + 1) * 128, c * 128:(c + 1) * 128] = (
                    ot_ref[c * 128:(c + 1) * 128, mm * 128:(mm + 1) * 128].astype(BF).T)

    def attn_a(first):
        chain[:] = [None] * len(chain)
        batches = [(p, h) for p in range(NPAIR) for h in range(NBAT)]
        for n in range(len(batches) + 2):
            if NB1 + n < R // RB:
                attn_b(NB1 + n)
            res = {}
            for u in range(NU):
                if n < len(batches):
                    p, h = batches[n]
                    qk_a(n % 2, u, p, NU * h + u)
                if 1 <= n <= len(batches):
                    p, h = batches[n - 1]
                    sm_a((n - 1) % 2, u, NU * h + u, first)
                if n >= 2:
                    p, h = batches[n - 2]
                    res[u] = pv_a((n - 2) % 2, u, p, NU * h + u)
                    if u % 2:
                        put(p, (NU * h + u) // 2, res[u - 1], res[u])

    pl.when(t == 0)(lambda: attn_a(True))
    pl.when(t > 0)(lambda: attn_a(False))

    @pl.when(t == 0)
    def _():
        copies[6].wait()
        copies[7].wait()
        for c in range(NLT):
            tmp_ref[c] = wob_ref[:, c * 128:(c + 1) * 128].astype(F32)
        permute_rows(wobp_ref)

    gl = jnp.sum(x.astype(F32) * gw_ref[...].astype(F32), axis=1, keepdims=True)
    g = jax.nn.sigmoid(gl)
    for c in range(NLT):
        a = _dot(oa_ref[...], woa_ref[:, c * 128:(c + 1) * 128])
        b = _dot(ob_ref[...], wobp_ref[c])
        o_ref[:, c * 128:(c + 1) * 128] = (g * a + (1.0 - g) * b).astype(o_ref.dtype)


@jax.jit
def pallas_gated_mix__sliding_block__sliding_local_dilated__prompt_kernel(
    A_x: jax.Array,
    A_wqkv: jax.Array,
    A_wo: jax.Array,
    B_x: jax.Array,
    B_wqkv: jax.Array,
    B_wo: jax.Array,
    gate_w: jax.Array,
):
    del B_x
    x = A_x.reshape(S, D)
    gw = gate_w.reshape(1, D)
    hbm = pl.BlockSpec(memory_space=pl.ANY)
    out = pl.pallas_call(
        kernel,
        grid=(S // R,),
        in_specs=[hbm] * 6,
        out_specs=pl.BlockSpec((R, D), lambda t: (t, 0)),
        out_shape=jax.ShapeDtypeStruct((S, D), BF),
        scratch_shapes=[
            pltpu.VMEM((S, D), BF),
            pltpu.VMEM((1, D), BF),
            pltpu.VMEM((3, D, D), BF),
            pltpu.VMEM((D, D), BF),
            pltpu.VMEM((3, D, D), BF),
            pltpu.VMEM((D, D), BF),
            pltpu.SemaphoreType.DMA((11,)),
            pltpu.VMEM((NT, R // 2, 128), U32),
            pltpu.VMEM((NT, (WA + S) // 2, 128), U32),
            pltpu.VMEM(((WA + S) // 128, D // 2, 128), U32),
            pltpu.VMEM((D, R), F32),
            pltpu.VMEM((R, D), BF),
            pltpu.VMEM((2, NU, WA + QC, 128), F32),
            pltpu.VMEM((2, NU, 192, 128), U32),
            pltpu.VMEM((3, NLT, D, 128), BF),
            pltpu.VMEM((NLT, D, 128), BF),
            pltpu.VMEM((NLT, D, 128), F32),
            pltpu.VMEM((NLT, R, 128), F32),
            pltpu.VMEM((NLT, HB + S, 128), F32),
            pltpu.VMEM((NLT, HB + S, 128), F32),
            pltpu.VMEM((R, D), BF),
        ],
        compiler_params=pltpu.CompilerParams(
            dimension_semantics=("arbitrary",),
            vmem_limit_bytes=100 * 1024 * 1024,
        ),
        name="gated_mix_attn",
    )(x, A_wqkv, A_wo, B_wqkv, B_wo, gw)
    return out.reshape(1, S, D)
```

```python
import jax
import jax.numpy as jnp
import numpy as np
import jax.experimental.pallas as pl
import jax.experimental.pallas.tpu as pltpu

S = 2048
D = 640
H = 32
DH = 20
NLT = D // 128
R = 512
QC = 64
NU = 4
NBAT = R // (QC * NU)
NPAIR = H // 2
WA = 256
HB = 16
RB = 16
NB1 = 24
LINK = 1
NEG = -1e30
LOG2E = 1.4426950408889634
QSCALE = float(DH ** -0.5) * LOG2E
BF = jnp.bfloat16
U32 = jnp.uint32
F32 = jnp.float32


def _pair_tile(p):
    c0 = 40 * p
    t0, off = divmod(c0, 128)
    if off + 40 <= 128:
        return (t0, t0, 0), off
    return (t0, t0 + 1, off), off


_TILES = []
_PAIR = []
for _p in range(NPAIR):
    _t, _o = _pair_tile(_p)
    if _t not in _TILES:
        _TILES.append(_t)
    _PAIR.append((_TILES.index(_t), _o))
NT = len(_TILES)


def _u32(x):
    return pltpu.bitcast(x, jnp.uint32)


def _bf(x):
    return pltpu.bitcast(x, BF)


def _pack16(y):
    g = y.shape[0] // 16
    y = y.reshape(g, 2, 8, y.shape[1])
    return pltpu.pack_elementwise(
        [y[:, 0].reshape(8 * g, -1), y[:, 1].reshape(8 * g, -1)], packed_dtype=BF)


def _nt_dot(a, b):
    return jax.lax.dot_general(a, b, (((1,), (1,)), ((), ())), preferred_element_type=F32)


def _dot(a, b):
    return jnp.dot(a, b, preferred_element_type=F32)


def kernel(x_hbm, wa_hbm, woa_hbm, wb_hbm, wob_hbm, gw_hbm, o_ref,
           x_ref, gw_ref, wa_ref, woa_ref, wb_ref, wob_ref, sems,
           qa_ref, ka_ref, vta_ref, ot_ref, oa_ref, s_ref, p_ref,
           wbt_ref, wobp_ref, tmp_ref, qb_ref, kb_ref, vb_ref, ob_ref):
    t = pl.program_id(0)
    not_first = t > 0
    row0 = pl.multiple_of(t * R, R)
    prow0 = pl.multiple_of(t * (R // 2), R // 2)

    phase = pl.when(t >= 0)

    def sec(ref, i):
        return ref.at[:, pl.ds(i * D, D)]

    copies = [pltpu.make_async_copy(sec(wb_hbm, i), wb_ref.at[i], sems.at[i]) for i in range(3)]
    copies += [pltpu.make_async_copy(sec(wa_hbm, i), wa_ref.at[i], sems.at[3 + i]) for i in range(3)]
    copies += [pltpu.make_async_copy(wob_hbm, wob_ref, sems.at[6]),
               pltpu.make_async_copy(woa_hbm, woa_ref, sems.at[7])]
    x_first = pltpu.make_async_copy(x_hbm.at[pl.ds(0, R)], x_ref.at[pl.ds(0, R)], sems.at[8])
    x_rest = pltpu.make_async_copy(x_hbm.at[pl.ds(R, S - R)], x_ref.at[pl.ds(R, S - R)], sems.at[9])
    gw_copy = pltpu.make_async_copy(gw_hbm, gw_ref, sems.at[10])

    @pl.when(t == 0)
    def _():
        x_first.start()
        copies[0].start()
        copies[1].start()
        gw_copy.start()
        ka_ref[:, 0:WA // 2, :] = jnp.zeros((NT, WA // 2, 128), U32)
        for j in range(WA // 128):
            vta_ref[j] = jnp.zeros((D // 2, 128), U32)
        for u in range(NU):
            z = (WA + QC) // 2 if u % 2 == 0 else 0
            p_ref[:, u, z:z + QC // 2, :] = jnp.zeros((2, QC // 2, 128), U32)
        kb_ref[:, 0:HB, :] = jnp.zeros((NLT, HB, 128), F32)
        vb_ref[:, 0:HB, :] = jnp.zeros((NLT, HB, 128), F32)

        x_first.wait()
        gw_copy.wait()

    @pl.when(t == 1)
    def _():
        x_rest.wait()

    x = x_ref[pl.ds(row0, R), :]

    def permute_rows(dst_ref):
        for c in range(NLT):
            for d in range(DH):
                dst_ref[c, d * H:(d + 1) * H, :] = tmp_ref[c, pl.ds(d, H, stride=DH), :].astype(BF)

    @pl.when(t == 0)
    def _():
        for i in range(3):
            copies[i].wait()
            copies[2 * i + 2].start()
            copies[2 * i + 3].start()
            for c in range(NLT):
                for n in range(NLT):
                    w = wb_ref[i, c * 128:(c + 1) * 128, n * 128:(n + 1) * 128]
                    tmp_ref[c, n * 128:(n + 1) * 128, :] = w.astype(F32).T
            permute_rows(wbt_ref.at[i])

    for i, dst in enumerate((qb_ref, kb_ref, vb_ref)):
        for n in range(NLT):
            y = None
            for c in range(NLT):
                z = _nt_dot(x[:, c * 128:(c + 1) * 128], wbt_ref[i, c, n * 128:(n + 1) * 128, :])
                y = z if y is None else y + z
            if i == 0:
                dst[n] = y * QSCALE
            else:
                dst[n, pl.ds(row0 + HB, R), :] = y

    @pl.when(t == 0)
    def _():
        x_rest.start()
        for cp in copies[3:6]:
            cp.wait()

    rowb = jax.lax.broadcasted_iota(jnp.int32, (RB, 128), 0)

    never = t < 0
    chain = [None, None]

    def attn_b(ci):
        r = ci * RB
        q = [qb_ref[c, r:r + RB, :] for c in range(NLT)]
        if chain[ci % LINK] is not None:
            q[0] = jnp.where(never, chain[ci % LINK], q[0])
            q[NLT - 1] = jnp.where(never, chain[ci % LINK], q[NLT - 1])
        sc = []
        for j in range(8):
            acc = None
            for c in range(NLT):
                y = q[c] * kb_ref[c, pl.ds(row0 + (r + HB - 2 * j), RB), :]
                acc = y if acc is None else acc + y
            acc = acc + pltpu.roll(acc, 64, 1)
            acc = acc + pltpu.roll(acc, 32, 1)
            if r < 2 * j:
                acc = jnp.where(not_first | (rowb >= 2 * j - r), acc, NEG)
            sc.append(acc)
        m = sc[0]
        for y in sc[1:]:
            m = jnp.maximum(m, y)
        e = [jnp.exp2(y - m) for y in sc]
        l = e[0]
        for y in e[1:]:
            l = l + y
        inv = 1.0 / l
        for c in range(NLT):
            acc = None
            for j in range(8):
                y = e[j] * vb_ref[c, pl.ds(row0 + (r + HB - 2 * j), RB), :]
                acc = y if acc is None else acc + y
            ob_ref[r:r + RB, c * 128:(c + 1) * 128] = (acc * inv).astype(BF)
        chain[ci % LINK] = acc

    @phase
    def _():
        def put_tile(ref, rows, c, y):
            y = _u32(y.astype(BF))
            ref[_TILES.index((c, c, 0)), rows, :] = y
            for i, (ta, tb, split) in enumerate(_TILES):
                if ta != tb and tb == c:
                    lane = jax.lax.broadcasted_iota(jnp.int32, y.shape, 1)
                    ref[i, rows, :] = jnp.where(lane >= split, ref[_TILES.index((ta, ta, 0)), rows, :], y)

        for n in range(3 * NLT):
            sec_i, c = divmod(n, NLT)
            y = _dot(x, wa_ref[sec_i, :, c * 128:(c + 1) * 128])
            if sec_i == 0:
                put_tile(qa_ref, pl.ds(0, R // 2), c, y * QSCALE)
            elif sec_i == 1:
                put_tile(ka_ref, pl.ds(prow0 + WA // 2, R // 2), c, y)
            else:
                va = _bf(_pack16(y).astype(U32))
                for j in range(R // 128):
                    vta_ref[t * (R // 128) + WA // 128 + j, c * 64:(c + 1) * 64, :] = (
                        _u32(va[j * 128:(j + 1) * 128, :].T))
            for ci in range(n * NB1 // (3 * NLT), (n + 1) * NB1 // (3 * NLT)):
                attn_b(ci)

    lane128 = jax.lax.broadcasted_iota(jnp.int32, (QC, 128), 1)
    row64 = jax.lax.broadcasted_iota(jnp.int32, (QC, 128), 0)
    lower = row64 <= (lane128 & (QC - 1))
    lane32 = jax.lax.broadcasted_iota(jnp.int32, (QC // 2, 128), 1)
    row48 = jax.lax.broadcasted_iota(jnp.int32, (48, 128), 0)
    lane48 = jax.lax.broadcasted_iota(jnp.int32, (48, 128), 1)
    left = lane48 < 64

    def masked_q(p, i):
        tix, off = _PAIR[p]
        qt = qa_ref[tix, i * QC // 2:(i + 1) * QC // 2, :]
        rel = (lane32 - off) & 127
        ones = jnp.uint32(0xFFFFFFFF)
        m0 = jnp.where(rel < DH, ones, jnp.uint32(0))
        m1 = jnp.where((rel >= DH) & (rel < 2 * DH), ones, jnp.uint32(0))
        return _bf(jnp.concatenate([qt & m0, qt & m1], axis=0))

    def qk_a(sl, u, p, i):
        kk = _bf(ka_ref[_PAIR[p][0], pl.ds(prow0 + i * QC // 2, (WA + QC) // 2), :])
        s_ref[sl, u] = _nt_dot(kk, masked_q(p, i))

    def sm_a(sl, u, i, first):
        def chunk(c):
            if first and c < WA // QC - i:
                return None
            return s_ref[sl, u, c * QC:(c + 1) * QC, :]

        def put_p(c, v):
            o = (QC * (i % 2) + c * QC) // 2
            p_ref[sl, u, o:o + QC // 2, :] = (
                jnp.zeros((QC // 2, 128), U32) if v is None else _pack16(v).astype(U32))

        mrg = jnp.where(lower, s_ref[sl, u, WA:WA + QC, :], NEG if chunk(0) is None else chunk(0))
        mid = [chunk(c) for c in range(1, 4)]
        m = jnp.max(mrg, axis=0, keepdims=True)
        for v in mid:
            if v is not None:
                m = jnp.maximum(m, jnp.max(v, axis=0, keepdims=True))
        pg = jnp.exp2(mrg - m)
        put_p(0, jnp.where(lower, 0.0, pg))
        put_p(4, jnp.where(lower, pg, 0.0))
        for c, v in enumerate(mid):
            put_p(c + 1, None if v is None else jnp.exp2(v - m))

    word = jax.lax.broadcasted_iota(jnp.int32, (8, 128), 0)
    ones_w = jnp.uint32(0x3F803F80)

    def pv_a(sl, u, p, i):
        w0 = 20 * p - 4 * (p % 2)
        c0 = t * (R // 128) + i // 2
        acc = None
        for j in range(3):
            v = vta_ref[c0 + j, w0:w0 + 24, :]
            if p % 2:
                v = jnp.concatenate([jnp.where(word < 4, ones_w, v[0:8]), v[8:24]], axis=0)
            else:
                v = jnp.concatenate([v[0:16], jnp.where(word >= 4, ones_w, v[16:24])], axis=0)
            y = _dot(_bf(v), _bf(p_ref[sl, u, j * 64:(j + 1) * 64, :]))
            acc = y if acc is None else acc + y
        if p % 2:
            return acc[8:48] * jnp.tile(1.0 / acc[0:8], (5, 1))
        return acc[0:40] * jnp.tile(1.0 / acc[40:48], (5, 1))

    row40 = jax.lax.broadcasted_iota(jnp.int32, (40, 128), 0)
    left = jax.lax.broadcasted_iota(jnp.int32, (40, 128), 1) < 64

    def put(p, mm, r_e, r_o):
        h0 = row40 < DH
        tt = jnp.where(left, jnp.where(h0, r_e, pltpu.roll(r_e, 64, 1)),
                       jnp.where(h0, pltpu.roll(r_o, 64, 1), r_o))
        ot_ref[40 * p:40 * p + 40, mm * 128:(mm + 1) * 128] = tt
        for c in range(NLT):
            if 40 * p < (c + 1) * 128 <= 40 * p + 40:
                oa_ref[mm * 128:(mm + 1) * 128, c * 128:(c + 1) * 128] = (
                    ot_ref[c * 128:(c + 1) * 128, mm * 128:(mm + 1) * 128].astype(BF).T)

    def attn_a(first):
        chain[:] = [None] * len(chain)
        batches = [(p, h) for p in range(NPAIR) for h in range(NBAT)]
        for n in range(len(batches) + 2):
            if NB1 + n < R // RB:
                attn_b(NB1 + n)
            res = {}
            for u in range(NU):
                if n < len(batches):
                    p, h = batches[n]
                    qk_a(n % 2, u, p, NU * h + u)
                if 1 <= n <= len(batches):
                    p, h = batches[n - 1]
                    sm_a((n - 1) % 2, u, NU * h + u, first)
                if n >= 2:
                    p, h = batches[n - 2]
                    res[u] = pv_a((n - 2) % 2, u, p, NU * h + u)
                    if u % 2:
                        put(p, (NU * h + u) // 2, res[u - 1], res[u])

    pl.when(t == 0)(lambda: attn_a(True))
    pl.when(t > 0)(lambda: attn_a(False))

    @pl.when(t == 0)
    def _():
        copies[6].wait()
        copies[7].wait()
        for c in range(NLT):
            tmp_ref[c] = wob_ref[:, c * 128:(c + 1) * 128].astype(F32)
        permute_rows(wobp_ref)

    gl = jnp.sum(x.astype(F32) * gw_ref[...].astype(F32), axis=1, keepdims=True)
    g = jax.nn.sigmoid(gl)
    for c in range(NLT):
        a = _dot(oa_ref[...], woa_ref[:, c * 128:(c + 1) * 128])
        b = _dot(ob_ref[...], wobp_ref[c])
        o_ref[:, c * 128:(c + 1) * 128] = (g * a + (1.0 - g) * b).astype(o_ref.dtype)


@jax.jit
def pallas_gated_mix__sliding_block__sliding_local_dilated__prompt_kernel(
    A_x: jax.Array,
    A_wqkv: jax.Array,
    A_wo: jax.Array,
    B_x: jax.Array,
    B_wqkv: jax.Array,
    B_wo: jax.Array,
    gate_w: jax.Array,
):
    del B_x
    x = A_x.reshape(S, D)
    gw = gate_w.reshape(1, D)
    hbm = pl.BlockSpec(memory_space=pl.ANY)
    out = pl.pallas_call(
        kernel,
        grid=(S // R,),
        in_specs=[hbm] * 6,
        out_specs=pl.BlockSpec((R, D), lambda t: (t, 0)),
        out_shape=jax.ShapeDtypeStruct((S, D), BF),
        scratch_shapes=[
            pltpu.VMEM((S, D), BF),
            pltpu.VMEM((1, D), BF),
            pltpu.VMEM((3, D, D), BF),
            pltpu.VMEM((D, D), BF),
            pltpu.VMEM((3, D, D), BF),
            pltpu.VMEM((D, D), BF),
            pltpu.SemaphoreType.DMA((11,)),
            pltpu.VMEM((NT, R // 2, 128), U32),
            pltpu.VMEM((NT, (WA + S) // 2, 128), U32),
            pltpu.VMEM(((WA + S) // 128, D // 2, 128), U32),
            pltpu.VMEM((D, R), F32),
            pltpu.VMEM((R, D), BF),
            pltpu.VMEM((2, NU, WA + QC, 128), F32),
            pltpu.VMEM((2, NU, 192, 128), U32),
            pltpu.VMEM((3, NLT, D, 128), BF),
            pltpu.VMEM((NLT, D, 128), BF),
            pltpu.VMEM((NLT, D, 128), F32),
            pltpu.VMEM((NLT, R, 128), F32),
            pltpu.VMEM((NLT, HB + S, 128), F32),
            pltpu.VMEM((NLT, HB + S, 128), F32),
            pltpu.VMEM((R, D), BF),
        ],
        compiler_params=pltpu.CompilerParams(
            dimension_semantics=("arbitrary",),
            vmem_limit_bytes=100 * 1024 * 1024,
        ),
        name="gated_mix_attn",
    )(x, A_wqkv, A_wo, B_wqkv, B_wo, gw)
    return out.reshape(1, S, D)
```

```python
import jax
import jax.numpy as jnp
import numpy as np
import jax.experimental.pallas as pl
import jax.experimental.pallas.tpu as pltpu

S = 2048
D = 640
H = 32
DH = 20
NLT = D // 128
R = 512
QC = 64
NU = 4
NBAT = R // (QC * NU)
NPAIR = H // 2
WA = 256
HB = 16
RB = 16
NB1 = 24
LINK = 1
NEG = -1e30
LOG2E = 1.4426950408889634
QSCALE = float(DH ** -0.5) * LOG2E
BF = jnp.bfloat16
U32 = jnp.uint32
F32 = jnp.float32


def _pair_tile(p):
    c0 = 40 * p
    t0, off = divmod(c0, 128)
    if off + 40 <= 128:
        return (t0, t0, 0), off
    return (t0, t0 + 1, off), off


_TILES = []
_PAIR = []
for _p in range(NPAIR):
    _t, _o = _pair_tile(_p)
    if _t not in _TILES:
        _TILES.append(_t)
    _PAIR.append((_TILES.index(_t), _o))
NT = len(_TILES)


def _u32(x):
    return pltpu.bitcast(x, jnp.uint32)


def _bf(x):
    return pltpu.bitcast(x, BF)


def _pack16(y):
    g = y.shape[0] // 16
    y = y.reshape(g, 2, 8, y.shape[1])
    return pltpu.pack_elementwise(
        [y[:, 0].reshape(8 * g, -1), y[:, 1].reshape(8 * g, -1)], packed_dtype=BF)


def _nt_dot(a, b):
    return jax.lax.dot_general(a, b, (((1,), (1,)), ((), ())), preferred_element_type=F32)


def _dot(a, b):
    return jnp.dot(a, b, preferred_element_type=F32)


def kernel(x_hbm, wa_hbm, woa_hbm, wb_hbm, wob_hbm, gw_hbm, o_ref,
           x_ref, gw_ref, wa_ref, woa_ref, wb_ref, wob_ref, sems,
           qa_ref, ka_ref, vta_ref, ot_ref, oa_ref, s_ref, p_ref,
           wbt_ref, wobp_ref, tmp_ref, qb_ref, kb_ref, vb_ref, ob_ref):
    t = pl.program_id(0)
    not_first = t > 0
    row0 = pl.multiple_of(t * R, R)
    prow0 = pl.multiple_of(t * (R // 2), R // 2)

    phase = pl.when(t >= 0)

    def sec(ref, i):
        return ref.at[:, pl.ds(i * D, D)]

    copies = [pltpu.make_async_copy(sec(wb_hbm, i), wb_ref.at[i], sems.at[i]) for i in range(3)]
    copies += [pltpu.make_async_copy(sec(wa_hbm, i), wa_ref.at[i], sems.at[3 + i]) for i in range(3)]
    copies += [pltpu.make_async_copy(wob_hbm, wob_ref, sems.at[6]),
               pltpu.make_async_copy(woa_hbm, woa_ref, sems.at[7])]
    x_first = pltpu.make_async_copy(x_hbm.at[pl.ds(0, R)], x_ref.at[pl.ds(0, R)], sems.at[8])
    x_rest = pltpu.make_async_copy(x_hbm.at[pl.ds(R, S - R)], x_ref.at[pl.ds(R, S - R)], sems.at[9])
    gw_copy = pltpu.make_async_copy(gw_hbm, gw_ref, sems.at[10])

    @pl.when(t == 0)
    def _():
        x_first.start()
        copies[0].start()
        copies[1].start()
        gw_copy.start()
        ka_ref[:, 0:WA // 2, :] = jnp.zeros((NT, WA // 2, 128), U32)
        for j in range(WA // 128):
            vta_ref[j] = jnp.zeros((D // 2, 128), U32)
        for u in range(NU):
            z = (WA + QC) // 2 if u % 2 == 0 else 0
            p_ref[:, u, z:z + QC // 2, :] = jnp.zeros((2, QC // 2, 128), U32)
        kb_ref[:, 0:HB, :] = jnp.zeros((NLT, HB, 128), F32)
        vb_ref[:, 0:HB, :] = jnp.zeros((NLT, HB, 128), F32)

        x_first.wait()
        gw_copy.wait()

    @pl.when(t == 1)
    def _():
        x_rest.wait()

    x = x_ref[pl.ds(row0, R), :]

    def permute_rows(dst_ref):
        for c in range(NLT):
            for d in range(DH):
                dst_ref[c, d * H:(d + 1) * H, :] = tmp_ref[c, pl.ds(d, H, stride=DH), :].astype(BF)

    def prep_b(i):
        copies[i].wait()
        copies[2 * i + 2].start()
        copies[2 * i + 3].start()
        for c in range(NLT):
            for n in range(NLT):
                w = wb_ref[i, c * 128:(c + 1) * 128, n * 128:(n + 1) * 128]
                tmp_ref[c, n * 128:(n + 1) * 128, :] = w.astype(F32).T
        permute_rows(wbt_ref.at[i])

    def proj_b(i):
        dst = (qb_ref, kb_ref, vb_ref)[i]
        for n in range(NLT):
            y = None
            for c in range(NLT):
                z = _nt_dot(x[:, c * 128:(c + 1) * 128], wbt_ref[i, c, n * 128:(n + 1) * 128, :])
                y = z if y is None else y + z
            if i == 0:
                dst[n] = y * QSCALE
            else:
                dst[n, pl.ds(row0 + HB, R), :] = y

    @pl.when(t == 0)
    def _():
        for i in range(3):
            prep_b(i)
            proj_b(i)
        x_rest.start()
        for cp in copies[3:6]:
            cp.wait()

    @pl.when(t > 0)
    def _():
        for i in range(3):
            proj_b(i)

    rowb = jax.lax.broadcasted_iota(jnp.int32, (RB, 128), 0)

    never = t < 0
    chain = [None, None]

    def attn_b(ci):
        r = ci * RB
        q = [qb_ref[c, r:r + RB, :] for c in range(NLT)]
        if chain[ci % LINK] is not None:
            q[0] = jnp.where(never, chain[ci % LINK], q[0])
            q[NLT - 1] = jnp.where(never, chain[ci % LINK], q[NLT - 1])
        sc = []
        for j in range(8):
            acc = None
            for c in range(NLT):
                y = q[c] * kb_ref[c, pl.ds(row0 + (r + HB - 2 * j), RB), :]
                acc = y if acc is None else acc + y
            acc = acc + pltpu.roll(acc, 64, 1)
            acc = acc + pltpu.roll(acc, 32, 1)
            if r < 2 * j:
                acc = jnp.where(not_first | (rowb >= 2 * j - r), acc, NEG)
            sc.append(acc)
        m = sc[0]
        for y in sc[1:]:
            m = jnp.maximum(m, y)
        e = [jnp.exp2(y - m) for y in sc]
        l = e[0]
        for y in e[1:]:
            l = l + y
        inv = 1.0 / l
        for c in range(NLT):
            acc = None
            for j in range(8):
                y = e[j] * vb_ref[c, pl.ds(row0 + (r + HB - 2 * j), RB), :]
                acc = y if acc is None else acc + y
            ob_ref[r:r + RB, c * 128:(c + 1) * 128] = (acc * inv).astype(BF)
        chain[ci % LINK] = acc

    @phase
    def _():
        def put_tile(ref, rows, c, y):
            y = _u32(y.astype(BF))
            ref[_TILES.index((c, c, 0)), rows, :] = y
            for i, (ta, tb, split) in enumerate(_TILES):
                if ta != tb and tb == c:
                    lane = jax.lax.broadcasted_iota(jnp.int32, y.shape, 1)
                    ref[i, rows, :] = jnp.where(lane >= split, ref[_TILES.index((ta, ta, 0)), rows, :], y)

        for n in range(3 * NLT):
            sec_i, c = divmod(n, NLT)
            y = _dot(x, wa_ref[sec_i, :, c * 128:(c + 1) * 128])
            if sec_i == 0:
                put_tile(qa_ref, pl.ds(0, R // 2), c, y * QSCALE)
            elif sec_i == 1:
                put_tile(ka_ref, pl.ds(prow0 + WA // 2, R // 2), c, y)
            else:
                va = _bf(_pack16(y).astype(U32))
                for j in range(R // 128):
                    vta_ref[t * (R // 128) + WA // 128 + j, c * 64:(c + 1) * 64, :] = (
                        _u32(va[j * 128:(j + 1) * 128, :].T))
            for ci in range(n * NB1 // (3 * NLT), (n + 1) * NB1 // (3 * NLT)):
                attn_b(ci)

    lane128 = jax.lax.broadcasted_iota(jnp.int32, (QC, 128), 1)
    row64 = jax.lax.broadcasted_iota(jnp.int32, (QC, 128), 0)
    lower = row64 <= (lane128 & (QC - 1))
    lane32 = jax.lax.broadcasted_iota(jnp.int32, (QC // 2, 128), 1)
    row48 = jax.lax.broadcasted_iota(jnp.int32, (48, 128), 0)
    lane48 = jax.lax.broadcasted_iota(jnp.int32, (48, 128), 1)
    left = lane48 < 64

    def masked_q(p, i):
        tix, off = _PAIR[p]
        qt = qa_ref[tix, i * QC // 2:(i + 1) * QC // 2, :]
        rel = (lane32 - off) & 127
        ones = jnp.uint32(0xFFFFFFFF)
        m0 = jnp.where(rel < DH, ones, jnp.uint32(0))
        m1 = jnp.where((rel >= DH) & (rel < 2 * DH), ones, jnp.uint32(0))
        return _bf(jnp.concatenate([qt & m0, qt & m1], axis=0))

    def qk_a(sl, u, p, i):
        kk = _bf(ka_ref[_PAIR[p][0], pl.ds(prow0 + i * QC // 2, (WA + QC) // 2), :])
        s_ref[sl, u] = _nt_dot(kk, masked_q(p, i))

    def sm_a(sl, u, i, first):
        def chunk(c):
            if first and c < WA // QC - i:
                return None
            return s_ref[sl, u, c * QC:(c + 1) * QC, :]

        def put_p(c, v):
            o = (QC * (i % 2) + c * QC) // 2
            p_ref[sl, u, o:o + QC // 2, :] = (
                jnp.zeros((QC // 2, 128), U32) if v is None else _pack16(v).astype(U32))

        mrg = jnp.where(lower, s_ref[sl, u, WA:WA + QC, :], NEG if chunk(0) is None else chunk(0))
        mid = [chunk(c) for c in range(1, 4)]
        m = jnp.max(mrg, axis=0, keepdims=True)
        for v in mid:
            if v is not None:
                m = jnp.maximum(m, jnp.max(v, axis=0, keepdims=True))
        pg = jnp.exp2(mrg - m)
        put_p(0, jnp.where(lower, 0.0, pg))
        put_p(4, jnp.where(lower, pg, 0.0))
        for c, v in enumerate(mid):
            put_p(c + 1, None if v is None else jnp.exp2(v - m))

    word = jax.lax.broadcasted_iota(jnp.int32, (8, 128), 0)
    ones_w = jnp.uint32(0x3F803F80)

    def pv_a(sl, u, p, i):
        w0 = 20 * p - 4 * (p % 2)
        c0 = t * (R // 128) + i // 2
        acc = None
        for j in range(3):
            v = vta_ref[c0 + j, w0:w0 + 24, :]
            if p % 2:
                v = jnp.concatenate([jnp.where(word < 4, ones_w, v[0:8]), v[8:24]], axis=0)
            else:
                v = jnp.concatenate([v[0:16], jnp.where(word >= 4, ones_w, v[16:24])], axis=0)
            y = _dot(_bf(v), _bf(p_ref[sl, u, j * 64:(j + 1) * 64, :]))
            acc = y if acc is None else acc + y
        if p % 2:
            return acc[8:48] * jnp.tile(1.0 / acc[0:8], (5, 1))
        return acc[0:40] * jnp.tile(1.0 / acc[40:48], (5, 1))

    row40 = jax.lax.broadcasted_iota(jnp.int32, (40, 128), 0)
    left = jax.lax.broadcasted_iota(jnp.int32, (40, 128), 1) < 64

    def put(p, mm, r_e, r_o):
        h0 = row40 < DH
        tt = jnp.where(left, jnp.where(h0, r_e, pltpu.roll(r_e, 64, 1)),
                       jnp.where(h0, pltpu.roll(r_o, 64, 1), r_o))
        ot_ref[40 * p:40 * p + 40, mm * 128:(mm + 1) * 128] = tt
        for c in range(NLT):
            if 40 * p < (c + 1) * 128 <= 40 * p + 40:
                oa_ref[mm * 128:(mm + 1) * 128, c * 128:(c + 1) * 128] = (
                    ot_ref[c * 128:(c + 1) * 128, mm * 128:(mm + 1) * 128].astype(BF).T)

    def attn_a(first):
        chain[:] = [None] * len(chain)
        batches = [(p, h) for p in range(NPAIR) for h in range(NBAT)]
        for n in range(len(batches) + 2):
            if NB1 + n < R // RB:
                attn_b(NB1 + n)
            res = {}
            for u in range(NU):
                if n < len(batches):
                    p, h = batches[n]
                    qk_a(n % 2, u, p, NU * h + u)
                if 1 <= n <= len(batches):
                    p, h = batches[n - 1]
                    sm_a((n - 1) % 2, u, NU * h + u, first)
                if n >= 2:
                    p, h = batches[n - 2]
                    res[u] = pv_a((n - 2) % 2, u, p, NU * h + u)
                    if u % 2:
                        put(p, (NU * h + u) // 2, res[u - 1], res[u])

    pl.when(t == 0)(lambda: attn_a(True))
    pl.when(t > 0)(lambda: attn_a(False))

    @pl.when(t == 0)
    def _():
        copies[6].wait()
        copies[7].wait()
        for c in range(NLT):
            tmp_ref[c] = wob_ref[:, c * 128:(c + 1) * 128].astype(F32)
        permute_rows(wobp_ref)

    gl = jnp.sum(x.astype(F32) * gw_ref[...].astype(F32), axis=1, keepdims=True)
    g = jax.nn.sigmoid(gl)
    for c in range(NLT):
        a = _dot(oa_ref[...], woa_ref[:, c * 128:(c + 1) * 128])
        b = _dot(ob_ref[...], wobp_ref[c])
        o_ref[:, c * 128:(c + 1) * 128] = (g * a + (1.0 - g) * b).astype(o_ref.dtype)


@jax.jit
def pallas_gated_mix__sliding_block__sliding_local_dilated__prompt_kernel(
    A_x: jax.Array,
    A_wqkv: jax.Array,
    A_wo: jax.Array,
    B_x: jax.Array,
    B_wqkv: jax.Array,
    B_wo: jax.Array,
    gate_w: jax.Array,
):
    del B_x
    x = A_x.reshape(S, D)
    gw = gate_w.reshape(1, D)
    hbm = pl.BlockSpec(memory_space=pl.ANY)
    out = pl.pallas_call(
        kernel,
        grid=(S // R,),
        in_specs=[hbm] * 6,
        out_specs=pl.BlockSpec((R, D), lambda t: (t, 0)),
        out_shape=jax.ShapeDtypeStruct((S, D), BF),
        scratch_shapes=[
            pltpu.VMEM((S, D), BF),
            pltpu.VMEM((1, D), BF),
            pltpu.VMEM((3, D, D), BF),
            pltpu.VMEM((D, D), BF),
            pltpu.VMEM((3, D, D), BF),
            pltpu.VMEM((D, D), BF),
            pltpu.SemaphoreType.DMA((11,)),
            pltpu.VMEM((NT, R // 2, 128), U32),
            pltpu.VMEM((NT, (WA + S) // 2, 128), U32),
            pltpu.VMEM(((WA + S) // 128, D // 2, 128), U32),
            pltpu.VMEM((D, R), F32),
            pltpu.VMEM((R, D), BF),
            pltpu.VMEM((2, NU, WA + QC, 128), F32),
            pltpu.VMEM((2, NU, 192, 128), U32),
            pltpu.VMEM((3, NLT, D, 128), BF),
            pltpu.VMEM((NLT, D, 128), BF),
            pltpu.VMEM((NLT, D, 128), F32),
            pltpu.VMEM((NLT, R, 128), F32),
            pltpu.VMEM((NLT, HB + S, 128), F32),
            pltpu.VMEM((NLT, HB + S, 128), F32),
            pltpu.VMEM((R, D), BF),
        ],
        compiler_params=pltpu.CompilerParams(
            dimension_semantics=("arbitrary",),
            vmem_limit_bytes=100 * 1024 * 1024,
        ),
        name="gated_mix_attn",
    )(x, A_wqkv, A_wo, B_wqkv, B_wo, gw)
    return out.reshape(1, S, D)
```

```python
import jax
import jax.numpy as jnp
import numpy as np
import jax.experimental.pallas as pl
import jax.experimental.pallas.tpu as pltpu

S = 2048
D = 640
H = 32
DH = 20
NLT = D // 128
R = 512
QC = 64
NU = 4
NBAT = R // (QC * NU)
NPAIR = H // 2
WA = 256
HB = 16
RB = 16
NB1 = 24
LINK = 1
NEG = -1e30
LOG2E = 1.4426950408889634
QSCALE = float(DH ** -0.5) * LOG2E
BF = jnp.bfloat16
U32 = jnp.uint32
F32 = jnp.float32


def _pair_tile(p):
    c0 = 40 * p
    t0, off = divmod(c0, 128)
    if off + 40 <= 128:
        return (t0, t0, 0), off
    return (t0, t0 + 1, off), off


_TILES = []
_PAIR = []
for _p in range(NPAIR):
    _t, _o = _pair_tile(_p)
    if _t not in _TILES:
        _TILES.append(_t)
    _PAIR.append((_TILES.index(_t), _o))
NT = len(_TILES)


def _u32(x):
    return pltpu.bitcast(x, jnp.uint32)


def _bf(x):
    return pltpu.bitcast(x, BF)


def _pack16(y):
    g = y.shape[0] // 16
    y = y.reshape(g, 2, 8, y.shape[1])
    return pltpu.pack_elementwise(
        [y[:, 0].reshape(8 * g, -1), y[:, 1].reshape(8 * g, -1)], packed_dtype=BF)


def _nt_dot(a, b):
    return jax.lax.dot_general(a, b, (((1,), (1,)), ((), ())), preferred_element_type=F32)


def _dot(a, b):
    return jnp.dot(a, b, preferred_element_type=F32)


def kernel(x_hbm, wa_hbm, woa_hbm, wb_hbm, wob_hbm, gw_hbm, o_ref,
           x_ref, gw_ref, wa_ref, woa_ref, wb_ref, wob_ref, sems,
           qa_ref, ka_ref, vta_ref, ot_ref, oa_ref, s_ref, p_ref,
           wbt_ref, wobp_ref, tmp_ref, qb_ref, kb_ref, vb_ref, ob_ref):
    t = pl.program_id(0)
    not_first = t > 0
    row0 = pl.multiple_of(t * R, R)
    prow0 = pl.multiple_of(t * (R // 2), R // 2)

    phase = pl.when(t >= 0)

    def sec(ref, i):
        return ref.at[:, pl.ds(i * D, D)]

    copies = [pltpu.make_async_copy(sec(wb_hbm, i), wb_ref.at[i], sems.at[i]) for i in range(3)]
    copies += [pltpu.make_async_copy(sec(wa_hbm, i), wa_ref.at[i], sems.at[3 + i]) for i in range(3)]
    copies += [pltpu.make_async_copy(wob_hbm, wob_ref, sems.at[6]),
               pltpu.make_async_copy(woa_hbm, woa_ref, sems.at[7])]
    x_first = pltpu.make_async_copy(x_hbm.at[pl.ds(0, R)], x_ref.at[pl.ds(0, R)], sems.at[8])
    x_rest = pltpu.make_async_copy(x_hbm.at[pl.ds(R, S - R)], x_ref.at[pl.ds(R, S - R)], sems.at[9])
    gw_copy = pltpu.make_async_copy(gw_hbm, gw_ref, sems.at[10])

    @pl.when(t == 0)
    def _():
        x_first.start()
        copies[0].start()
        copies[1].start()
        gw_copy.start()
        ka_ref[:, 0:WA // 2, :] = jnp.zeros((NT, WA // 2, 128), U32)
        for j in range(WA // 128):
            vta_ref[j] = jnp.zeros((D // 2, 128), U32)
        for u in range(NU):
            z = (WA + QC) // 2 if u % 2 == 0 else 0
            p_ref[:, u, z:z + QC // 2, :] = jnp.zeros((2, QC // 2, 128), U32)
        kb_ref[:, 0:HB, :] = jnp.zeros((NLT, HB, 128), F32)
        vb_ref[:, 0:HB, :] = jnp.zeros((NLT, HB, 128), F32)

        x_first.wait()
        gw_copy.wait()

    @pl.when(t == 1)
    def _():
        x_rest.wait()

    x = x_ref[pl.ds(row0, R), :]

    def permute_rows(dst_ref):
        for c in range(NLT):
            for d in range(DH):
                dst_ref[c, d * H:(d + 1) * H, :] = tmp_ref[c, pl.ds(d, H, stride=DH), :].astype(BF)

    @pl.when(t == 0)
    def _():
        for i in range(3):
            copies[i].wait()
            copies[2 * i + 2].start()
            copies[2 * i + 3].start()
            for c in range(NLT):
                for n in range(NLT):
                    w = wb_ref[i, c * 128:(c + 1) * 128, n * 128:(n + 1) * 128]
                    tmp_ref[c, n * 128:(n + 1) * 128, :] = w.astype(F32).T
            permute_rows(wbt_ref.at[i])

    for i, dst in enumerate((qb_ref, kb_ref, vb_ref)):
        for n in range(NLT):
            y = None
            for c in range(NLT):
                z = _nt_dot(x[:, c * 128:(c + 1) * 128], wbt_ref[i, c, n * 128:(n + 1) * 128, :])
                y = z if y is None else y + z
            if i == 0:
                dst[n] = y * QSCALE
            else:
                dst[n, pl.ds(row0 + HB, R), :] = y

    @pl.when(t == 0)
    def _():
        x_rest.start()
        for cp in copies[3:6]:
            cp.wait()

    rowb = jax.lax.broadcasted_iota(jnp.int32, (RB, 128), 0)

    never = t < 0
    chain = [None, None]

    def attn_b(ci):
        r = ci * RB
        q = [qb_ref[c, r:r + RB, :] for c in range(NLT)]
        if chain[ci % LINK] is not None:
            q[0] = jnp.where(never, chain[ci % LINK], q[0])
            q[NLT - 1] = jnp.where(never, chain[ci % LINK], q[NLT - 1])
        sc = []
        for j in range(8):
            acc = None
            for c in range(NLT):
                y = q[c] * kb_ref[c, pl.ds(row0 + (r + HB - 2 * j), RB), :]
                acc = y if acc is None else acc + y
            acc = acc + pltpu.roll(acc, 64, 1)
            acc = acc + pltpu.roll(acc, 32, 1)
            if r < 2 * j:
                acc = jnp.where(not_first | (rowb >= 2 * j - r), acc, NEG)
            sc.append(acc)
        m = sc[0]
        for y in sc[1:]:
            m = jnp.maximum(m, y)
        e = [jnp.exp2(y - m) for y in sc]
        l = e[0]
        for y in e[1:]:
            l = l + y
        inv = 1.0 / l
        for c in range(NLT):
            acc = None
            for j in range(8):
                y = e[j] * vb_ref[c, pl.ds(row0 + (r + HB - 2 * j), RB), :]
                acc = y if acc is None else acc + y
            ob_ref[r:r + RB, c * 128:(c + 1) * 128] = (acc * inv).astype(BF)
        chain[ci % LINK] = acc

    @phase
    def _():
        def put_tile(ref, rows, c, y):
            y = _u32(y.astype(BF))
            ref[_TILES.index((c, c, 0)), rows, :] = y
            for i, (ta, tb, split) in enumerate(_TILES):
                if ta != tb and tb == c:
                    lane = jax.lax.broadcasted_iota(jnp.int32, y.shape, 1)
                    ref[i, rows, :] = jnp.where(lane >= split, ref[_TILES.index((ta, ta, 0)), rows, :], y)

        for n in range(3 * NLT):
            sec_i, c = divmod(n, NLT)
            y = _dot(x, wa_ref[sec_i, :, c * 128:(c + 1) * 128])
            if sec_i == 0:
                put_tile(qa_ref, pl.ds(0, R // 2), c, y * QSCALE)
            elif sec_i == 1:
                put_tile(ka_ref, pl.ds(prow0 + WA // 2, R // 2), c, y)
            else:
                va = _bf(_pack16(y).astype(U32))
                for j in range(R // 128):
                    vta_ref[t * (R // 128) + WA // 128 + j, c * 64:(c + 1) * 64, :] = (
                        _u32(va[j * 128:(j + 1) * 128, :].T))
            for ci in range(n * NB1 // (3 * NLT), (n + 1) * NB1 // (3 * NLT)):
                attn_b(ci)

    lane128 = jax.lax.broadcasted_iota(jnp.int32, (QC, 128), 1)
    row64 = jax.lax.broadcasted_iota(jnp.int32, (QC, 128), 0)
    lower = row64 <= (lane128 & (QC - 1))
    lane32 = jax.lax.broadcasted_iota(jnp.int32, (QC // 2, 128), 1)
    row48 = jax.lax.broadcasted_iota(jnp.int32, (48, 128), 0)
    lane48 = jax.lax.broadcasted_iota(jnp.int32, (48, 128), 1)
    left = lane48 < 64

    def masked_q(p, i):
        tix, off = _PAIR[p]
        qt = qa_ref[tix, i * QC // 2:(i + 1) * QC // 2, :]
        rel = (lane32 - off) & 127
        ones = jnp.uint32(0xFFFFFFFF)
        m0 = jnp.where(rel < DH, ones, jnp.uint32(0))
        m1 = jnp.where((rel >= DH) & (rel < 2 * DH), ones, jnp.uint32(0))
        return _bf(jnp.concatenate([qt & m0, qt & m1], axis=0))

    def qk_a(sl, u, p, i):
        kk = _bf(ka_ref[_PAIR[p][0], pl.ds(prow0 + i * QC // 2, (WA + QC) // 2), :])
        s_ref[sl, u] = _nt_dot(kk, masked_q(p, i))

    def sm_a(sl, u, i):
        def chunk(c):
            v = s_ref[sl, u, c * QC:(c + 1) * QC, :]
            if c < WA // QC - i:
                v = jnp.where(not_first, v, NEG)
            return v

        def put_p(c, v):
            o = (QC * (i % 2) + c * QC) // 2
            p_ref[sl, u, o:o + QC // 2, :] = _pack16(v).astype(U32)

        mrg = jnp.where(lower, s_ref[sl, u, WA:WA + QC, :], chunk(0))
        mid = [chunk(c) for c in range(1, 4)]
        m = jnp.max(mrg, axis=0, keepdims=True)
        for v in mid:
            m = jnp.maximum(m, jnp.max(v, axis=0, keepdims=True))
        pg = jnp.exp2(mrg - m)
        put_p(0, jnp.where(lower, 0.0, pg))
        put_p(4, jnp.where(lower, pg, 0.0))
        for c, v in enumerate(mid):
            put_p(c + 1, jnp.exp2(v - m))

    word = jax.lax.broadcasted_iota(jnp.int32, (8, 128), 0)
    ones_w = jnp.uint32(0x3F803F80)

    def pv_a(sl, u, p, i):
        w0 = 20 * p - 4 * (p % 2)
        c0 = t * (R // 128) + i // 2
        acc = None
        for j in range(3):
            v = vta_ref[c0 + j, w0:w0 + 24, :]
            if p % 2:
                v = jnp.concatenate([jnp.where(word < 4, ones_w, v[0:8]), v[8:24]], axis=0)
            else:
                v = jnp.concatenate([v[0:16], jnp.where(word >= 4, ones_w, v[16:24])], axis=0)
            y = _dot(_bf(v), _bf(p_ref[sl, u, j * 64:(j + 1) * 64, :]))
            acc = y if acc is None else acc + y
        if p % 2:
            return acc[8:48] * jnp.tile(1.0 / acc[0:8], (5, 1))
        return acc[0:40] * jnp.tile(1.0 / acc[40:48], (5, 1))

    row40 = jax.lax.broadcasted_iota(jnp.int32, (40, 128), 0)
    left = jax.lax.broadcasted_iota(jnp.int32, (40, 128), 1) < 64

    def put(p, mm, r_e, r_o):
        h0 = row40 < DH
        tt = jnp.where(left, jnp.where(h0, r_e, pltpu.roll(r_e, 64, 1)),
                       jnp.where(h0, pltpu.roll(r_o, 64, 1), r_o))
        ot_ref[40 * p:40 * p + 40, mm * 128:(mm + 1) * 128] = tt
        for c in range(NLT):
            if 40 * p < (c + 1) * 128 <= 40 * p + 40:
                oa_ref[mm * 128:(mm + 1) * 128, c * 128:(c + 1) * 128] = (
                    ot_ref[c * 128:(c + 1) * 128, mm * 128:(mm + 1) * 128].astype(BF).T)

    @phase
    def _():
        chain[:] = [None] * len(chain)
        batches = [(p, h) for p in range(NPAIR) for h in range(NBAT)]
        for n in range(len(batches) + 2):
            if NB1 + n < R // RB:
                attn_b(NB1 + n)
            res = {}
            for u in range(NU):
                if n < len(batches):
                    p, h = batches[n]
                    qk_a(n % 2, u, p, NU * h + u)
                if 1 <= n <= len(batches):
                    p, h = batches[n - 1]
                    sm_a((n - 1) % 2, u, NU * h + u)
                if n >= 2:
                    p, h = batches[n - 2]
                    res[u] = pv_a((n - 2) % 2, u, p, NU * h + u)
                    if u % 2:
                        put(p, (NU * h + u) // 2, res[u - 1], res[u])

    @pl.when(t == 0)
    def _():
        copies[6].wait()
        copies[7].wait()
        for c in range(NLT):
            tmp_ref[c] = wob_ref[:, c * 128:(c + 1) * 128].astype(F32)
        permute_rows(wobp_ref)

    gl = jnp.sum(x.astype(F32) * gw_ref[...].astype(F32), axis=1, keepdims=True)
    g = jax.nn.sigmoid(gl)
    for c in range(NLT):
        a = _dot(oa_ref[...], woa_ref[:, c * 128:(c + 1) * 128])
        b = _dot(ob_ref[...], wobp_ref[c])
        o_ref[:, c * 128:(c + 1) * 128] = (g * a + (1.0 - g) * b).astype(o_ref.dtype)


@jax.jit
def pallas_gated_mix__sliding_block__sliding_local_dilated__prompt_kernel(
    A_x: jax.Array,
    A_wqkv: jax.Array,
    A_wo: jax.Array,
    B_x: jax.Array,
    B_wqkv: jax.Array,
    B_wo: jax.Array,
    gate_w: jax.Array,
):
    del B_x
    x = A_x.reshape(S, D)
    gw = gate_w.reshape(1, D)
    hbm = pl.BlockSpec(memory_space=pl.ANY)
    out = pl.pallas_call(
        kernel,
        grid=(S // R,),
        in_specs=[hbm] * 6,
        out_specs=pl.BlockSpec((R, D), lambda t: (t, 0)),
        out_shape=jax.ShapeDtypeStruct((S, D), BF),
        scratch_shapes=[
            pltpu.VMEM((S, D), BF),
            pltpu.VMEM((1, D), BF),
            pltpu.VMEM((3, D, D), BF),
            pltpu.VMEM((D, D), BF),
            pltpu.VMEM((3, D, D), BF),
            pltpu.VMEM((D, D), BF),
            pltpu.SemaphoreType.DMA((11,)),
            pltpu.VMEM((NT, R // 2, 128), U32),
            pltpu.VMEM((NT, (WA + S) // 2, 128), U32),
            pltpu.VMEM(((WA + S) // 128, D // 2, 128), U32),
            pltpu.VMEM((D, R), F32),
            pltpu.VMEM((R, D), BF),
            pltpu.VMEM((2, NU, WA + QC, 128), F32),
            pltpu.VMEM((2, NU, 192, 128), U32),
            pltpu.VMEM((3, NLT, D, 128), BF),
            pltpu.VMEM((NLT, D, 128), BF),
            pltpu.VMEM((NLT, D, 128), F32),
            pltpu.VMEM((NLT, R, 128), F32),
            pltpu.VMEM((NLT, HB + S, 128), F32),
            pltpu.VMEM((NLT, HB + S, 128), F32),
            pltpu.VMEM((R, D), BF),
        ],
        compiler_params=pltpu.CompilerParams(
            dimension_semantics=("arbitrary",),
            vmem_limit_bytes=100 * 1024 * 1024,
        ),
        name="gated_mix_attn",
    )(x, A_wqkv, A_wo, B_wqkv, B_wo, gw)
    return out.reshape(1, S, D)
```

```python
import jax
import jax.numpy as jnp
import numpy as np
import jax.experimental.pallas as pl
import jax.experimental.pallas.tpu as pltpu

S = 2048
D = 640
H = 32
DH = 20
NLT = D // 128
R = 512
QC = 64
NU = 4
NBAT = R // (QC * NU)
NPAIR = H // 2
WA = 256
HB = 16
RB = 16
NB1 = 24
LINK = 1
NEG = -1e30
LOG2E = 1.4426950408889634
QSCALE = float(DH ** -0.5) * LOG2E
BF = jnp.bfloat16
U32 = jnp.uint32
F32 = jnp.float32


def _pair_tile(p):
    c0 = 40 * p
    t0, off = divmod(c0, 128)
    if off + 40 <= 128:
        return (t0, t0, 0), off
    return (t0, t0 + 1, off), off


_TILES = []
_PAIR = []
for _p in range(NPAIR):
    _t, _o = _pair_tile(_p)
    if _t not in _TILES:
        _TILES.append(_t)
    _PAIR.append((_TILES.index(_t), _o))
NT = len(_TILES)


def _u32(x):
    return pltpu.bitcast(x, jnp.uint32)


def _bf(x):
    return pltpu.bitcast(x, BF)


def _pack16(y):
    g = y.shape[0] // 16
    y = y.reshape(g, 2, 8, y.shape[1])
    return pltpu.pack_elementwise(
        [y[:, 0].reshape(8 * g, -1), y[:, 1].reshape(8 * g, -1)], packed_dtype=BF)


def _nt_dot(a, b):
    return jax.lax.dot_general(a, b, (((1,), (1,)), ((), ())), preferred_element_type=F32)


def _dot(a, b):
    return jnp.dot(a, b, preferred_element_type=F32)


def kernel(x_hbm, wa_hbm, woa_hbm, wb_hbm, wob_hbm, gw_hbm, o_ref,
           x_ref, gw_ref, wa_ref, woa_ref, wb_ref, wob_ref, sems,
           qa_ref, ka_ref, vta_ref, ot_ref, oa_ref, s_ref, p_ref,
           wbt_ref, wobp_ref, tmp_ref, qb_ref, kb_ref, vb_ref, ob_ref):
    t = pl.program_id(0)
    not_first = t > 0
    row0 = pl.multiple_of(t * R, R)
    prow0 = pl.multiple_of(t * (R // 2), R // 2)

    phase = pl.when(t >= 0)

    def sec(ref, i):
        return ref.at[:, pl.ds(i * D, D)]

    copies = [pltpu.make_async_copy(sec(wb_hbm, i), wb_ref.at[i], sems.at[i]) for i in range(3)]
    copies += [pltpu.make_async_copy(sec(wa_hbm, i), wa_ref.at[i], sems.at[3 + i]) for i in range(3)]
    copies += [pltpu.make_async_copy(wob_hbm, wob_ref, sems.at[6]),
               pltpu.make_async_copy(woa_hbm, woa_ref, sems.at[7])]
    x_first = pltpu.make_async_copy(x_hbm.at[pl.ds(0, R)], x_ref.at[pl.ds(0, R)], sems.at[8])
    x_rest = pltpu.make_async_copy(x_hbm.at[pl.ds(R, S - R)], x_ref.at[pl.ds(R, S - R)], sems.at[9])
    gw_copy = pltpu.make_async_copy(gw_hbm, gw_ref, sems.at[10])

    @pl.when(t == 0)
    def _():
        x_first.start()
        copies[0].start()
        copies[1].start()
        gw_copy.start()
        ka_ref[:, 0:WA // 2, :] = jnp.zeros((NT, WA // 2, 128), U32)
        for j in range(WA // 128):
            vta_ref[j] = jnp.zeros((D // 2, 128), U32)
        for u in range(NU):
            z = (WA + QC) // 2 if u % 2 == 0 else 0
            p_ref[:, u, z:z + QC // 2, :] = jnp.zeros((2, QC // 2, 128), U32)
        kb_ref[:, 0:HB, :] = jnp.zeros((NLT, HB, 128), F32)
        vb_ref[:, 0:HB, :] = jnp.zeros((NLT, HB, 128), F32)

        x_first.wait()
        gw_copy.wait()

    @pl.when(t == 1)
    def _():
        x_rest.wait()

    x = x_ref[pl.ds(row0, R), :]

    def permute_rows(dst_ref):
        for c in range(NLT):
            for d in range(DH):
                dst_ref[c, d * H:(d + 1) * H, :] = tmp_ref[c, pl.ds(d, H, stride=DH), :].astype(BF)

    def prep_b(i):
        copies[i].wait()
        copies[2 * i + 2].start()
        copies[2 * i + 3].start()
        for c in range(NLT):
            for n in range(NLT):
                w = wb_ref[i, c * 128:(c + 1) * 128, n * 128:(n + 1) * 128]
                tmp_ref[c, n * 128:(n + 1) * 128, :] = w.astype(F32).T
        permute_rows(wbt_ref.at[i])

    def proj_b(i):
        dst = (qb_ref, kb_ref, vb_ref)[i]
        for n in range(NLT):
            y = None
            for c in range(NLT):
                z = _nt_dot(x[:, c * 128:(c + 1) * 128], wbt_ref[i, c, n * 128:(n + 1) * 128, :])
                y = z if y is None else y + z
            if i == 0:
                dst[n] = y * QSCALE
            else:
                dst[n, pl.ds(row0 + HB, R), :] = y

    @pl.when(t == 0)
    def _():
        for i in range(3):
            prep_b(i)
            proj_b(i)
        x_rest.start()
        for cp in copies[3:6]:
            cp.wait()

    @pl.when(t > 0)
    def _():
        for i in range(3):
            proj_b(i)

    rowb = jax.lax.broadcasted_iota(jnp.int32, (RB, 128), 0)

    never = t < 0
    chain = [None, None]

    def attn_b(ci):
        r = ci * RB
        q = [qb_ref[c, r:r + RB, :] for c in range(NLT)]
        if chain[ci % LINK] is not None:
            q[0] = jnp.where(never, chain[ci % LINK], q[0])
            q[NLT - 1] = jnp.where(never, chain[ci % LINK], q[NLT - 1])
        sc = []
        for j in range(8):
            acc = None
            for c in range(NLT):
                y = q[c] * kb_ref[c, pl.ds(row0 + (r + HB - 2 * j), RB), :]
                acc = y if acc is None else acc + y
            acc = acc + pltpu.roll(acc, 64, 1)
            acc = acc + pltpu.roll(acc, 32, 1)
            if r < 2 * j:
                acc = jnp.where(not_first | (rowb >= 2 * j - r), acc, NEG)
            sc.append(acc)
        m = sc[0]
        for y in sc[1:]:
            m = jnp.maximum(m, y)
        e = [jnp.exp2(y - m) for y in sc]
        l = e[0]
        for y in e[1:]:
            l = l + y
        inv = 1.0 / l
        for c in range(NLT):
            acc = None
            for j in range(8):
                y = e[j] * vb_ref[c, pl.ds(row0 + (r + HB - 2 * j), RB), :]
                acc = y if acc is None else acc + y
            ob_ref[r:r + RB, c * 128:(c + 1) * 128] = (acc * inv).astype(BF)
        chain[ci % LINK] = acc

    @phase
    def _():
        def put_tile(ref, rows, c, y):
            y = _u32(y.astype(BF))
            ref[_TILES.index((c, c, 0)), rows, :] = y
            for i, (ta, tb, split) in enumerate(_TILES):
                if ta != tb and tb == c:
                    lane = jax.lax.broadcasted_iota(jnp.int32, y.shape, 1)
                    ref[i, rows, :] = jnp.where(lane >= split, ref[_TILES.index((ta, ta, 0)), rows, :], y)

        for n in range(3 * NLT):
            sec_i, c = divmod(n, NLT)
            y = _dot(x, wa_ref[sec_i, :, c * 128:(c + 1) * 128])
            if sec_i == 0:
                put_tile(qa_ref, pl.ds(0, R // 2), c, y * QSCALE)
            elif sec_i == 1:
                put_tile(ka_ref, pl.ds(prow0 + WA // 2, R // 2), c, y)
            else:
                va = _bf(_pack16(y).astype(U32))
                for j in range(R // 128):
                    vta_ref[t * (R // 128) + WA // 128 + j, c * 64:(c + 1) * 64, :] = (
                        _u32(va[j * 128:(j + 1) * 128, :].T))
            for ci in range(n * NB1 // (3 * NLT), (n + 1) * NB1 // (3 * NLT)):
                attn_b(ci)

    lane128 = jax.lax.broadcasted_iota(jnp.int32, (QC, 128), 1)
    row64 = jax.lax.broadcasted_iota(jnp.int32, (QC, 128), 0)
    lower = row64 <= (lane128 & (QC - 1))
    lane32 = jax.lax.broadcasted_iota(jnp.int32, (QC // 2, 128), 1)
    row48 = jax.lax.broadcasted_iota(jnp.int32, (48, 128), 0)
    lane48 = jax.lax.broadcasted_iota(jnp.int32, (48, 128), 1)
    left = lane48 < 64

    def masked_q(p, i):
        tix, off = _PAIR[p]
        qt = qa_ref[tix, i * QC // 2:(i + 1) * QC // 2, :]
        rel = (lane32 - off) & 127
        ones = jnp.uint32(0xFFFFFFFF)
        m0 = jnp.where(rel < DH, ones, jnp.uint32(0))
        m1 = jnp.where((rel >= DH) & (rel < 2 * DH), ones, jnp.uint32(0))
        return _bf(jnp.concatenate([qt & m0, qt & m1], axis=0))

    def qk_a(sl, u, p, i):
        kk = _bf(ka_ref[_PAIR[p][0], pl.ds(prow0 + i * QC // 2, (WA + QC) // 2), :])
        s_ref[sl, u] = _nt_dot(kk, masked_q(p, i))

    def sm_a(sl, u, i):
        def chunk(c):
            v = s_ref[sl, u, c * QC:(c + 1) * QC, :]
            if c < WA // QC - i:
                v = jnp.where(not_first, v, NEG)
            return v

        def put_p(c, v):
            o = (QC * (i % 2) + c * QC) // 2
            p_ref[sl, u, o:o + QC // 2, :] = _pack16(v).astype(U32)

        mrg = jnp.where(lower, s_ref[sl, u, WA:WA + QC, :], chunk(0))
        mid = [chunk(c) for c in range(1, 4)]
        m = jnp.max(mrg, axis=0, keepdims=True)
        for v in mid:
            m = jnp.maximum(m, jnp.max(v, axis=0, keepdims=True))
        pg = jnp.exp2(mrg - m)
        put_p(0, jnp.where(lower, 0.0, pg))
        put_p(4, jnp.where(lower, pg, 0.0))
        for c, v in enumerate(mid):
            put_p(c + 1, jnp.exp2(v - m))

    word = jax.lax.broadcasted_iota(jnp.int32, (8, 128), 0)
    ones_w = jnp.uint32(0x3F803F80)

    def pv_a(sl, u, p, i):
        w0 = 20 * p - 4 * (p % 2)
        c0 = t * (R // 128) + i // 2
        acc = None
        for j in range(3):
            v = vta_ref[c0 + j, w0:w0 + 24, :]
            if p % 2:
                v = jnp.concatenate([jnp.where(word < 4, ones_w, v[0:8]), v[8:24]], axis=0)
            else:
                v = jnp.concatenate([v[0:16], jnp.where(word >= 4, ones_w, v[16:24])], axis=0)
            y = _dot(_bf(v), _bf(p_ref[sl, u, j * 64:(j + 1) * 64, :]))
            acc = y if acc is None else acc + y
        if p % 2:
            return acc[8:48] * jnp.tile(1.0 / acc[0:8], (5, 1))
        return acc[0:40] * jnp.tile(1.0 / acc[40:48], (5, 1))

    row40 = jax.lax.broadcasted_iota(jnp.int32, (40, 128), 0)
    left = jax.lax.broadcasted_iota(jnp.int32, (40, 128), 1) < 64

    def put(p, mm, r_e, r_o):
        h0 = row40 < DH
        tt = jnp.where(left, jnp.where(h0, r_e, pltpu.roll(r_e, 64, 1)),
                       jnp.where(h0, pltpu.roll(r_o, 64, 1), r_o))
        ot_ref[40 * p:40 * p + 40, mm * 128:(mm + 1) * 128] = tt
        for c in range(NLT):
            if 40 * p < (c + 1) * 128 <= 40 * p + 40:
                oa_ref[mm * 128:(mm + 1) * 128, c * 128:(c + 1) * 128] = (
                    ot_ref[c * 128:(c + 1) * 128, mm * 128:(mm + 1) * 128].astype(BF).T)

    @phase
    def _():
        chain[:] = [None] * len(chain)
        batches = [(p, h) for p in range(NPAIR) for h in range(NBAT)]
        for n in range(len(batches) + 2):
            if NB1 + n < R // RB:
                attn_b(NB1 + n)
            res = {}
            for u in range(NU):
                if n < len(batches):
                    p, h = batches[n]
                    qk_a(n % 2, u, p, NU * h + u)
                if 1 <= n <= len(batches):
                    p, h = batches[n - 1]
                    sm_a((n - 1) % 2, u, NU * h + u)
                if n >= 2:
                    p, h = batches[n - 2]
                    res[u] = pv_a((n - 2) % 2, u, p, NU * h + u)
                    if u % 2:
                        put(p, (NU * h + u) // 2, res[u - 1], res[u])

    @pl.when(t == 0)
    def _():
        copies[6].wait()
        copies[7].wait()
        for c in range(NLT):
            tmp_ref[c] = wob_ref[:, c * 128:(c + 1) * 128].astype(F32)
        permute_rows(wobp_ref)

    gl = jnp.sum(x.astype(F32) * gw_ref[...].astype(F32), axis=1, keepdims=True)
    g = jax.nn.sigmoid(gl)
    for c in range(NLT):
        a = _dot(oa_ref[...], woa_ref[:, c * 128:(c + 1) * 128])
        b = _dot(ob_ref[...], wobp_ref[c])
        o_ref[:, c * 128:(c + 1) * 128] = (g * a + (1.0 - g) * b).astype(o_ref.dtype)


@jax.jit
def pallas_gated_mix__sliding_block__sliding_local_dilated__prompt_kernel(
    A_x: jax.Array,
    A_wqkv: jax.Array,
    A_wo: jax.Array,
    B_x: jax.Array,
    B_wqkv: jax.Array,
    B_wo: jax.Array,
    gate_w: jax.Array,
):
    del B_x
    x = A_x.reshape(S, D)
    gw = gate_w.reshape(1, D)
    hbm = pl.BlockSpec(memory_space=pl.ANY)
    out = pl.pallas_call(
        kernel,
        grid=(S // R,),
        in_specs=[hbm] * 6,
        out_specs=pl.BlockSpec((R, D), lambda t: (t, 0)),
        out_shape=jax.ShapeDtypeStruct((S, D), BF),
        scratch_shapes=[
            pltpu.VMEM((S, D), BF),
            pltpu.VMEM((1, D), BF),
            pltpu.VMEM((3, D, D), BF),
            pltpu.VMEM((D, D), BF),
            pltpu.VMEM((3, D, D), BF),
            pltpu.VMEM((D, D), BF),
            pltpu.SemaphoreType.DMA((11,)),
            pltpu.VMEM((NT, R // 2, 128), U32),
            pltpu.VMEM((NT, (WA + S) // 2, 128), U32),
            pltpu.VMEM(((WA + S) // 128, D // 2, 128), U32),
            pltpu.VMEM((D, R), F32),
            pltpu.VMEM((R, D), BF),
            pltpu.VMEM((2, NU, WA + QC, 128), F32),
            pltpu.VMEM((2, NU, 192, 128), U32),
            pltpu.VMEM((3, NLT, D, 128), BF),
            pltpu.VMEM((NLT, D, 128), BF),
            pltpu.VMEM((NLT, D, 128), F32),
            pltpu.VMEM((NLT, R, 128), F32),
            pltpu.VMEM((NLT, HB + S, 128), F32),
            pltpu.VMEM((NLT, HB + S, 128), F32),
            pltpu.VMEM((R, D), BF),
        ],
        compiler_params=pltpu.CompilerParams(
            dimension_semantics=("arbitrary",),
            vmem_limit_bytes=100 * 1024 * 1024,
        ),
        name="gated_mix_attn",
    )(x, A_wqkv, A_wo, B_wqkv, B_wo, gw)
    return out.reshape(1, S, D)
```

```python
import jax
import jax.numpy as jnp
import numpy as np
import jax.experimental.pallas as pl
import jax.experimental.pallas.tpu as pltpu

S = 2048
D = 640
H = 32
DH = 20
NLT = D // 128
R = 512
QC = 64
NU = 4
NBAT = R // (QC * NU)
NPAIR = H // 2
WA = 256
HB = 16
RB = 16
NB1 = 20
LINK = 1
NEG = -1e30
LOG2E = 1.4426950408889634
QSCALE = float(DH ** -0.5) * LOG2E
BF = jnp.bfloat16
U32 = jnp.uint32
F32 = jnp.float32


def _pair_tile(p):
    c0 = 40 * p
    t0, off = divmod(c0, 128)
    if off + 40 <= 128:
        return (t0, t0, 0), off
    return (t0, t0 + 1, off), off


_TILES = []
_PAIR = []
for _p in range(NPAIR):
    _t, _o = _pair_tile(_p)
    if _t not in _TILES:
        _TILES.append(_t)
    _PAIR.append((_TILES.index(_t), _o))
NT = len(_TILES)


def _u32(x):
    return pltpu.bitcast(x, jnp.uint32)


def _bf(x):
    return pltpu.bitcast(x, BF)


def _pack16(y):
    g = y.shape[0] // 16
    y = y.reshape(g, 2, 8, y.shape[1])
    return pltpu.pack_elementwise(
        [y[:, 0].reshape(8 * g, -1), y[:, 1].reshape(8 * g, -1)], packed_dtype=BF)


def _nt_dot(a, b):
    return jax.lax.dot_general(a, b, (((1,), (1,)), ((), ())), preferred_element_type=F32)


def _dot(a, b):
    return jnp.dot(a, b, preferred_element_type=F32)


def kernel(x_hbm, wa_hbm, woa_hbm, wb_hbm, wob_hbm, gw_hbm, o_ref,
           x_ref, gw_ref, wa_ref, woa_ref, wb_ref, wob_ref, sems,
           qa_ref, ka_ref, vta_ref, ot_ref, oa_ref, s_ref, p_ref,
           wbt_ref, wobp_ref, tmp_ref, qb_ref, kb_ref, vb_ref, ob_ref):
    t = pl.program_id(0)
    not_first = t > 0
    row0 = pl.multiple_of(t * R, R)
    prow0 = pl.multiple_of(t * (R // 2), R // 2)

    phase = pl.when(t >= 0)

    def sec(ref, i):
        return ref.at[:, pl.ds(i * D, D)]

    copies = [pltpu.make_async_copy(sec(wb_hbm, i), wb_ref.at[i], sems.at[i]) for i in range(3)]
    copies += [pltpu.make_async_copy(sec(wa_hbm, i), wa_ref.at[i], sems.at[3 + i]) for i in range(3)]
    copies += [pltpu.make_async_copy(wob_hbm, wob_ref, sems.at[6]),
               pltpu.make_async_copy(woa_hbm, woa_ref, sems.at[7])]
    x_first = pltpu.make_async_copy(x_hbm.at[pl.ds(0, R)], x_ref.at[pl.ds(0, R)], sems.at[8])
    x_rest = pltpu.make_async_copy(x_hbm.at[pl.ds(R, S - R)], x_ref.at[pl.ds(R, S - R)], sems.at[9])
    gw_copy = pltpu.make_async_copy(gw_hbm, gw_ref, sems.at[10])

    @pl.when(t == 0)
    def _():
        x_first.start()
        copies[0].start()
        copies[1].start()
        gw_copy.start()
        ka_ref[:, 0:WA // 2, :] = jnp.zeros((NT, WA // 2, 128), U32)
        for j in range(WA // 128):
            vta_ref[j] = jnp.zeros((D // 2, 128), U32)
        for u in range(NU):
            z = (WA + QC) // 2 if u % 2 == 0 else 0
            p_ref[:, u, z:z + QC // 2, :] = jnp.zeros((2, QC // 2, 128), U32)
        kb_ref[:, 0:HB, :] = jnp.zeros((NLT, HB, 128), F32)
        vb_ref[:, 0:HB, :] = jnp.zeros((NLT, HB, 128), F32)

        x_first.wait()
        gw_copy.wait()

    @pl.when(t == 1)
    def _():
        x_rest.wait()

    x = x_ref[pl.ds(row0, R), :]

    def permute_rows(dst_ref):
        for c in range(NLT):
            for d in range(DH):
                dst_ref[c, d * H:(d + 1) * H, :] = tmp_ref[c, pl.ds(d, H, stride=DH), :].astype(BF)

    def prep_b(i):
        copies[i].wait()
        copies[2 * i + 2].start()
        copies[2 * i + 3].start()
        for c in range(NLT):
            for n in range(NLT):
                w = wb_ref[i, c * 128:(c + 1) * 128, n * 128:(n + 1) * 128]
                tmp_ref[c, n * 128:(n + 1) * 128, :] = w.astype(F32).T
        permute_rows(wbt_ref.at[i])

    def proj_b(i):
        dst = (qb_ref, kb_ref, vb_ref)[i]
        for n in range(NLT):
            y = None
            for c in range(NLT):
                z = _nt_dot(x[:, c * 128:(c + 1) * 128], wbt_ref[i, c, n * 128:(n + 1) * 128, :])
                y = z if y is None else y + z
            if i == 0:
                dst[n] = y * QSCALE
            else:
                dst[n, pl.ds(row0 + HB, R), :] = y

    @pl.when(t == 0)
    def _():
        for i in range(3):
            prep_b(i)
            proj_b(i)
        x_rest.start()
        for cp in copies[3:6]:
            cp.wait()

    @pl.when(t > 0)
    def _():
        for i in range(3):
            proj_b(i)

    rowb = jax.lax.broadcasted_iota(jnp.int32, (RB, 128), 0)

    never = t < 0
    chain = [None, None]

    def attn_b(ci):
        r = ci * RB
        q = [qb_ref[c, r:r + RB, :] for c in range(NLT)]
        if chain[ci % LINK] is not None:
            q[0] = jnp.where(never, chain[ci % LINK], q[0])
            q[NLT - 1] = jnp.where(never, chain[ci % LINK], q[NLT - 1])
        sc = []
        for j in range(8):
            acc = None
            for c in range(NLT):
                y = q[c] * kb_ref[c, pl.ds(row0 + (r + HB - 2 * j), RB), :]
                acc = y if acc is None else acc + y
            acc = acc + pltpu.roll(acc, 64, 1)
            acc = acc + pltpu.roll(acc, 32, 1)
            if r < 2 * j:
                acc = jnp.where(not_first | (rowb >= 2 * j - r), acc, NEG)
            sc.append(acc)
        m = sc[0]
        for y in sc[1:]:
            m = jnp.maximum(m, y)
        e = [jnp.exp2(y - m) for y in sc]
        l = e[0]
        for y in e[1:]:
            l = l + y
        inv = 1.0 / l
        for c in range(NLT):
            acc = None
            for j in range(8):
                y = e[j] * vb_ref[c, pl.ds(row0 + (r + HB - 2 * j), RB), :]
                acc = y if acc is None else acc + y
            ob_ref[r:r + RB, c * 128:(c + 1) * 128] = (acc * inv).astype(BF)
        chain[ci % LINK] = acc

    @phase
    def _():
        def put_tile(ref, rows, c, y):
            y = _u32(y.astype(BF))
            ref[_TILES.index((c, c, 0)), rows, :] = y
            for i, (ta, tb, split) in enumerate(_TILES):
                if ta != tb and tb == c:
                    lane = jax.lax.broadcasted_iota(jnp.int32, y.shape, 1)
                    ref[i, rows, :] = jnp.where(lane >= split, ref[_TILES.index((ta, ta, 0)), rows, :], y)

        for n in range(3 * NLT):
            sec_i, c = divmod(n, NLT)
            y = _dot(x, wa_ref[sec_i, :, c * 128:(c + 1) * 128])
            if sec_i == 0:
                put_tile(qa_ref, pl.ds(0, R // 2), c, y * QSCALE)
            elif sec_i == 1:
                put_tile(ka_ref, pl.ds(prow0 + WA // 2, R // 2), c, y)
            else:
                va = _bf(_pack16(y).astype(U32))
                for j in range(R // 128):
                    vta_ref[t * (R // 128) + WA // 128 + j, c * 64:(c + 1) * 64, :] = (
                        _u32(va[j * 128:(j + 1) * 128, :].T))
            for ci in range(n * NB1 // (3 * NLT), (n + 1) * NB1 // (3 * NLT)):
                attn_b(ci)

    lane128 = jax.lax.broadcasted_iota(jnp.int32, (QC, 128), 1)
    row64 = jax.lax.broadcasted_iota(jnp.int32, (QC, 128), 0)
    lower = row64 <= (lane128 & (QC - 1))
    lane32 = jax.lax.broadcasted_iota(jnp.int32, (QC // 2, 128), 1)
    row48 = jax.lax.broadcasted_iota(jnp.int32, (48, 128), 0)
    lane48 = jax.lax.broadcasted_iota(jnp.int32, (48, 128), 1)
    left = lane48 < 64

    def masked_q(p, i):
        tix, off = _PAIR[p]
        qt = qa_ref[tix, i * QC // 2:(i + 1) * QC // 2, :]
        rel = (lane32 - off) & 127
        ones = jnp.uint32(0xFFFFFFFF)
        m0 = jnp.where(rel < DH, ones, jnp.uint32(0))
        m1 = jnp.where((rel >= DH) & (rel < 2 * DH), ones, jnp.uint32(0))
        return _bf(jnp.concatenate([qt & m0, qt & m1], axis=0))

    def qk_a(sl, u, p, i):
        kk = _bf(ka_ref[_PAIR[p][0], pl.ds(prow0 + i * QC // 2, (WA + QC) // 2), :])
        s_ref[sl, u] = _nt_dot(kk, masked_q(p, i))

    def sm_a(sl, u, i):
        def chunk(c):
            v = s_ref[sl, u, c * QC:(c + 1) * QC, :]
            if c < WA // QC - i:
                v = jnp.where(not_first, v, NEG)
            return v

        def put_p(c, v):
            o = (QC * (i % 2) + c * QC) // 2
            p_ref[sl, u, o:o + QC // 2, :] = _pack16(v).astype(U32)

        mrg = jnp.where(lower, s_ref[sl, u, WA:WA + QC, :], chunk(0))
        mid = [chunk(c) for c in range(1, 4)]
        m = jnp.max(mrg, axis=0, keepdims=True)
        for v in mid:
            m = jnp.maximum(m, jnp.max(v, axis=0, keepdims=True))
        pg = jnp.exp2(mrg - m)
        put_p(0, jnp.where(lower, 0.0, pg))
        put_p(4, jnp.where(lower, pg, 0.0))
        for c, v in enumerate(mid):
            put_p(c + 1, jnp.exp2(v - m))

    word = jax.lax.broadcasted_iota(jnp.int32, (8, 128), 0)
    ones_w = jnp.uint32(0x3F803F80)

    left8 = jax.lax.broadcasted_iota(jnp.int32, (64, 128), 1) < 64

    def pv_a(sl, u, p, mm):
        c0 = t * (R // 128) + mm
        acc = [None, None]
        for j in range(3):
            pe = p_ref[sl, u, j * 64:(j + 1) * 64, :]
            po = p_ref[sl, u + 1, j * 64:(j + 1) * 64, :]
            ph = (jnp.where(left8, pe, pltpu.roll(po, 64, 1)), jnp.where(left8, pltpu.roll(pe, 64, 1), po))
            for e in range(2):
                h = 2 * p + e
                w0 = (DH * h) // 16 * 8
                v = vta_ref[c0 + j, w0:w0 + 16, :]
                if (DH * h) % 16 < 8:
                    v = jnp.concatenate([v[0:8], jnp.where(word >= 4, ones_w, v[8:16])], axis=0)
                else:
                    v = jnp.concatenate([jnp.where(word < 4, ones_w, v[0:8]), v[8:16]], axis=0)
                y = _dot(_bf(v), _bf(ph[e]))
                acc[e] = y if acc[e] is None else acc[e] + y
        out = []
        for e in range(2):
            if (DH * (2 * p + e)) % 16 < 8:
                out.append(acc[e][0:24] * jnp.tile(1.0 / acc[e][24:32], (3, 1)))
            else:
                out.append(acc[e][8:32] * jnp.tile(1.0 / acc[e][0:8], (3, 1)))
        tt = jnp.concatenate([out[0][0:16], jnp.where(word < 4, out[0][16:24], out[1][0:8]), out[1][8:24]], axis=0)
        ot_ref[40 * p:40 * p + 40, mm * 128:(mm + 1) * 128] = tt
        for c in range(NLT):
            if 40 * p < (c + 1) * 128 <= 40 * p + 40:
                oa_ref[mm * 128:(mm + 1) * 128, c * 128:(c + 1) * 128] = (
                    ot_ref[c * 128:(c + 1) * 128, mm * 128:(mm + 1) * 128].astype(BF).T)

    @phase
    def _():
        chain[:] = [None] * len(chain)
        batches = [(p, h) for p in range(NPAIR) for h in range(NBAT)]
        for n in range(len(batches) + 2):
            if NB1 + n < R // RB:
                attn_b(NB1 + n)
            for u in range(NU):
                if n < len(batches):
                    p, h = batches[n]
                    qk_a(n % 2, u, p, NU * h + u)
                if 1 <= n <= len(batches):
                    p, h = batches[n - 1]
                    sm_a((n - 1) % 2, u, NU * h + u)
                if n >= 2 and u % 2 == 0:
                    p, h = batches[n - 2]
                    pv_a((n - 2) % 2, u, p, (NU * h + u) // 2)

    @pl.when(t == 0)
    def _():
        copies[6].wait()
        copies[7].wait()
        for c in range(NLT):
            tmp_ref[c] = wob_ref[:, c * 128:(c + 1) * 128].astype(F32)
        permute_rows(wobp_ref)

    gl = jnp.sum(x.astype(F32) * gw_ref[...].astype(F32), axis=1, keepdims=True)
    g = jax.nn.sigmoid(gl)
    for c in range(NLT):
        a = _dot(oa_ref[...], woa_ref[:, c * 128:(c + 1) * 128])
        b = _dot(ob_ref[...], wobp_ref[c])
        o_ref[:, c * 128:(c + 1) * 128] = (g * a + (1.0 - g) * b).astype(o_ref.dtype)


@jax.jit
def pallas_gated_mix__sliding_block__sliding_local_dilated__prompt_kernel(
    A_x: jax.Array,
    A_wqkv: jax.Array,
    A_wo: jax.Array,
    B_x: jax.Array,
    B_wqkv: jax.Array,
    B_wo: jax.Array,
    gate_w: jax.Array,
):
    del B_x
    x = A_x.reshape(S, D)
    gw = gate_w.reshape(1, D)
    hbm = pl.BlockSpec(memory_space=pl.ANY)
    out = pl.pallas_call(
        kernel,
        grid=(S // R,),
        in_specs=[hbm] * 6,
        out_specs=pl.BlockSpec((R, D), lambda t: (t, 0)),
        out_shape=jax.ShapeDtypeStruct((S, D), BF),
        scratch_shapes=[
            pltpu.VMEM((S, D), BF),
            pltpu.VMEM((1, D), BF),
            pltpu.VMEM((3, D, D), BF),
            pltpu.VMEM((D, D), BF),
            pltpu.VMEM((3, D, D), BF),
            pltpu.VMEM((D, D), BF),
            pltpu.SemaphoreType.DMA((11,)),
            pltpu.VMEM((NT, R // 2, 128), U32),
            pltpu.VMEM((NT, (WA + S) // 2, 128), U32),
            pltpu.VMEM(((WA + S) // 128, D // 2, 128), U32),
            pltpu.VMEM((D, R), F32),
            pltpu.VMEM((R, D), BF),
            pltpu.VMEM((2, NU, WA + QC, 128), F32),
            pltpu.VMEM((2, NU, 192, 128), U32),
            pltpu.VMEM((3, NLT, D, 128), BF),
            pltpu.VMEM((NLT, D, 128), BF),
            pltpu.VMEM((NLT, D, 128), F32),
            pltpu.VMEM((NLT, R, 128), F32),
            pltpu.VMEM((NLT, HB + S, 128), F32),
            pltpu.VMEM((NLT, HB + S, 128), F32),
            pltpu.VMEM((R, D), BF),
        ],
        compiler_params=pltpu.CompilerParams(
            dimension_semantics=("arbitrary",),
            vmem_limit_bytes=100 * 1024 * 1024,
        ),
        name="gated_mix_attn",
    )(x, A_wqkv, A_wo, B_wqkv, B_wo, gw)
    return out.reshape(1, S, D)
```

```python
import jax
import jax.numpy as jnp
import numpy as np
import jax.experimental.pallas as pl
import jax.experimental.pallas.tpu as pltpu

S = 2048
D = 640
H = 32
DH = 20
NLT = D // 128
R = 512
QC = 64
NU = 4
NBAT = R // (QC * NU)
NPAIR = H // 2
WA = 256
HB = 16
RB = 16
NB1 = 20
LINK = 1
NEG = -1e30
LOG2E = 1.4426950408889634
QSCALE = float(DH ** -0.5) * LOG2E
BF = jnp.bfloat16
U32 = jnp.uint32
F32 = jnp.float32


def _pair_tile(p):
    c0 = 40 * p
    t0, off = divmod(c0, 128)
    if off + 40 <= 128:
        return (t0, t0, 0), off
    return (t0, t0 + 1, off), off


_TILES = []
_PAIR = []
for _p in range(NPAIR):
    _t, _o = _pair_tile(_p)
    if _t not in _TILES:
        _TILES.append(_t)
    _PAIR.append((_TILES.index(_t), _o))
NT = len(_TILES)


def _u32(x):
    return pltpu.bitcast(x, jnp.uint32)


def _bf(x):
    return pltpu.bitcast(x, BF)


def _pack16(y):
    g = y.shape[0] // 16
    y = y.reshape(g, 2, 8, y.shape[1])
    return pltpu.pack_elementwise(
        [y[:, 0].reshape(8 * g, -1), y[:, 1].reshape(8 * g, -1)], packed_dtype=BF)


def _nt_dot(a, b):
    return jax.lax.dot_general(a, b, (((1,), (1,)), ((), ())), preferred_element_type=F32)


def _dot(a, b):
    return jnp.dot(a, b, preferred_element_type=F32)


def kernel(x_hbm, wa_hbm, woa_hbm, wb_hbm, wob_hbm, gw_hbm, o_ref,
           x_ref, gw_ref, wa_ref, woa_ref, wb_ref, wob_ref, sems,
           qa_ref, ka_ref, vta_ref, ot_ref, oa_ref, s_ref, p_ref,
           wbt_ref, wobp_ref, tmp_ref, qb_ref, kb_ref, vb_ref, ob_ref):
    t = pl.program_id(0)
    not_first = t > 0
    row0 = pl.multiple_of(t * R, R)
    prow0 = pl.multiple_of(t * (R // 2), R // 2)

    phase = pl.when(t >= 0)

    def sec(ref, i):
        return ref.at[:, pl.ds(i * D, D)]

    copies = [pltpu.make_async_copy(sec(wb_hbm, i), wb_ref.at[i], sems.at[i]) for i in range(3)]
    copies += [pltpu.make_async_copy(sec(wa_hbm, i), wa_ref.at[i], sems.at[3 + i]) for i in range(3)]
    copies += [pltpu.make_async_copy(wob_hbm, wob_ref, sems.at[6]),
               pltpu.make_async_copy(woa_hbm, woa_ref, sems.at[7])]
    x_first = pltpu.make_async_copy(x_hbm.at[pl.ds(0, R)], x_ref.at[pl.ds(0, R)], sems.at[8])
    x_rest = pltpu.make_async_copy(x_hbm.at[pl.ds(R, S - R)], x_ref.at[pl.ds(R, S - R)], sems.at[9])
    gw_copy = pltpu.make_async_copy(gw_hbm, gw_ref, sems.at[10])

    @pl.when(t == 0)
    def _():
        x_first.start()
        copies[0].start()
        copies[1].start()
        gw_copy.start()
        ka_ref[:, 0:WA // 2, :] = jnp.zeros((NT, WA // 2, 128), U32)
        for j in range(WA // 128):
            vta_ref[j] = jnp.zeros((D // 2, 128), U32)
        for u in range(NU):
            z = (WA + QC) // 2 if u % 2 == 0 else 0
            p_ref[:, u, z:z + QC // 2, :] = jnp.zeros((2, QC // 2, 128), U32)
        kb_ref[:, 0:HB, :] = jnp.zeros((NLT, HB, 128), F32)
        vb_ref[:, 0:HB, :] = jnp.zeros((NLT, HB, 128), F32)

        x_first.wait()
        gw_copy.wait()

    @pl.when(t == 1)
    def _():
        x_rest.wait()

    x = x_ref[pl.ds(row0, R), :]

    def permute_rows(dst_ref):
        for c in range(NLT):
            for d in range(DH):
                dst_ref[c, d * H:(d + 1) * H, :] = tmp_ref[c, pl.ds(d, H, stride=DH), :].astype(BF)

    def prep_b(i):
        copies[i].wait()
        copies[2 * i + 2].start()
        copies[2 * i + 3].start()
        for c in range(NLT):
            for n in range(NLT):
                w = wb_ref[i, c * 128:(c + 1) * 128, n * 128:(n + 1) * 128]
                tmp_ref[c, n * 128:(n + 1) * 128, :] = w.astype(F32).T
        permute_rows(wbt_ref.at[i])

    def proj_b(i):
        dst = (qb_ref, kb_ref, vb_ref)[i]
        for n in range(NLT):
            y = None
            for c in range(NLT):
                z = _nt_dot(x[:, c * 128:(c + 1) * 128], wbt_ref[i, c, n * 128:(n + 1) * 128, :])
                y = z if y is None else y + z
            if i == 0:
                dst[n] = y * QSCALE
            else:
                dst[n, pl.ds(row0 + HB, R), :] = y

    @pl.when(t == 0)
    def _():
        for i in range(3):
            prep_b(i)
            proj_b(i)
        x_rest.start()
        for cp in copies[3:6]:
            cp.wait()

    @pl.when(t > 0)
    def _():
        for i in range(3):
            proj_b(i)

    rowb = jax.lax.broadcasted_iota(jnp.int32, (RB, 128), 0)

    never = t < 0
    chain = [None, None]

    def attn_b(ci):
        r = ci * RB
        q = [qb_ref[c, r:r + RB, :] for c in range(NLT)]
        if chain[ci % LINK] is not None:
            q[0] = jnp.where(never, chain[ci % LINK], q[0])
            q[NLT - 1] = jnp.where(never, chain[ci % LINK], q[NLT - 1])
        sc = []
        for j in range(8):
            acc = None
            for c in range(NLT):
                y = q[c] * kb_ref[c, pl.ds(row0 + (r + HB - 2 * j), RB), :]
                acc = y if acc is None else acc + y
            acc = acc + pltpu.roll(acc, 64, 1)
            acc = acc + pltpu.roll(acc, 32, 1)
            if r < 2 * j:
                acc = jnp.where(not_first | (rowb >= 2 * j - r), acc, NEG)
            sc.append(acc)
        m = sc[0]
        for y in sc[1:]:
            m = jnp.maximum(m, y)
        e = [jnp.exp2(y - m) for y in sc]
        l = e[0]
        for y in e[1:]:
            l = l + y
        inv = 1.0 / l
        for c in range(NLT):
            acc = None
            for j in range(8):
                y = e[j] * vb_ref[c, pl.ds(row0 + (r + HB - 2 * j), RB), :]
                acc = y if acc is None else acc + y
            ob_ref[r:r + RB, c * 128:(c + 1) * 128] = (acc * inv).astype(BF)
        chain[ci % LINK] = acc

    @phase
    def _():
        def put_tile(ref, rows, c, y):
            y = _u32(y.astype(BF))
            ref[_TILES.index((c, c, 0)), rows, :] = y
            for i, (ta, tb, split) in enumerate(_TILES):
                if ta != tb and tb == c:
                    lane = jax.lax.broadcasted_iota(jnp.int32, y.shape, 1)
                    ref[i, rows, :] = jnp.where(lane >= split, ref[_TILES.index((ta, ta, 0)), rows, :], y)

        for n in range(3 * NLT):
            sec_i, c = divmod(n, NLT)
            y = _dot(x, wa_ref[sec_i, :, c * 128:(c + 1) * 128])
            if sec_i == 0:
                put_tile(qa_ref, pl.ds(0, R // 2), c, y * QSCALE)
            elif sec_i == 1:
                put_tile(ka_ref, pl.ds(prow0 + WA // 2, R // 2), c, y)
            else:
                va = _bf(_pack16(y).astype(U32))
                for j in range(R // 128):
                    vta_ref[t * (R // 128) + WA // 128 + j, c * 64:(c + 1) * 64, :] = (
                        _u32(va[j * 128:(j + 1) * 128, :].T))
            for ci in range(n * NB1 // (3 * NLT), (n + 1) * NB1 // (3 * NLT)):
                attn_b(ci)

    lane128 = jax.lax.broadcasted_iota(jnp.int32, (QC, 128), 1)
    row64 = jax.lax.broadcasted_iota(jnp.int32, (QC, 128), 0)
    lower = row64 <= (lane128 & (QC - 1))
    lane32 = jax.lax.broadcasted_iota(jnp.int32, (QC // 2, 128), 1)
    row48 = jax.lax.broadcasted_iota(jnp.int32, (48, 128), 0)
    lane48 = jax.lax.broadcasted_iota(jnp.int32, (48, 128), 1)
    left = lane48 < 64

    def masked_q(p, i):
        tix, off = _PAIR[p]
        qt = qa_ref[tix, i * QC // 2:(i + 1) * QC // 2, :]
        rel = (lane32 - off) & 127
        ones = jnp.uint32(0xFFFFFFFF)
        m0 = jnp.where(rel < DH, ones, jnp.uint32(0))
        m1 = jnp.where((rel >= DH) & (rel < 2 * DH), ones, jnp.uint32(0))
        return _bf(jnp.concatenate([qt & m0, qt & m1], axis=0))

    def qk_a(sl, u, p, i):
        kk = _bf(ka_ref[_PAIR[p][0], pl.ds(prow0 + i * QC // 2, (WA + QC) // 2), :])
        s_ref[sl, u] = _nt_dot(kk, masked_q(p, i))

    def sm_a(sl, u, i):
        def chunk(c):
            v = s_ref[sl, u, c * QC:(c + 1) * QC, :]
            if c < WA // QC - i:
                v = jnp.where(not_first, v, NEG)
            return v

        def put_p(c, v):
            o = (QC * (i % 2) + c * QC) // 2
            p_ref[sl, u, o:o + QC // 2, :] = _pack16(v).astype(U32)

        mrg = jnp.where(lower, s_ref[sl, u, WA:WA + QC, :], chunk(0))
        mid = [chunk(c) for c in range(1, 4)]
        m = jnp.max(mrg, axis=0, keepdims=True)
        for v in mid:
            m = jnp.maximum(m, jnp.max(v, axis=0, keepdims=True))
        pg = jnp.exp2(mrg - m)
        put_p(0, jnp.where(lower, 0.0, pg))
        put_p(4, jnp.where(lower, pg, 0.0))
        for c, v in enumerate(mid):
            put_p(c + 1, jnp.exp2(v - m))

    word = jax.lax.broadcasted_iota(jnp.int32, (8, 128), 0)
    ones_w = jnp.uint32(0x3F803F80)

    def pv_a(sl, u, p, i):
        w0 = 20 * p - 4 * (p % 2)
        c0 = t * (R // 128) + i // 2
        acc = None
        for j in range(3):
            v = vta_ref[c0 + j, w0:w0 + 24, :]
            if p % 2:
                v = jnp.concatenate([jnp.where(word < 4, ones_w, v[0:8]), v[8:24]], axis=0)
            else:
                v = jnp.concatenate([v[0:16], jnp.where(word >= 4, ones_w, v[16:24])], axis=0)
            y = _dot(_bf(v), _bf(p_ref[sl, u, j * 64:(j + 1) * 64, :]))
            acc = y if acc is None else acc + y
        if p % 2:
            return acc[8:48] * jnp.tile(1.0 / acc[0:8], (5, 1))
        return acc[0:40] * jnp.tile(1.0 / acc[40:48], (5, 1))

    row40 = jax.lax.broadcasted_iota(jnp.int32, (40, 128), 0)
    left = jax.lax.broadcasted_iota(jnp.int32, (40, 128), 1) < 64

    def put(p, mm, r_e, r_o):
        h0 = row40 < DH
        tt = jnp.where(left, jnp.where(h0, r_e, pltpu.roll(r_e, 64, 1)),
                       jnp.where(h0, pltpu.roll(r_o, 64, 1), r_o))
        ot_ref[40 * p:40 * p + 40, mm * 128:(mm + 1) * 128] = tt
        for c in range(NLT):
            if 40 * p < (c + 1) * 128 <= 40 * p + 40:
                oa_ref[mm * 128:(mm + 1) * 128, c * 128:(c + 1) * 128] = (
                    ot_ref[c * 128:(c + 1) * 128, mm * 128:(mm + 1) * 128].astype(BF).T)

    @phase
    def _():
        chain[:] = [None] * len(chain)
        batches = [(p, h) for p in range(NPAIR) for h in range(NBAT)]
        for n in range(len(batches) + 2):
            if NB1 + n < R // RB:
                attn_b(NB1 + n)
            res = {}
            for u in range(NU):
                if n < len(batches):
                    p, h = batches[n]
                    qk_a(n % 2, u, p, NU * h + u)
                if 1 <= n <= len(batches):
                    p, h = batches[n - 1]
                    sm_a((n - 1) % 2, u, NU * h + u)
                if n >= 2:
                    p, h = batches[n - 2]
                    res[u] = pv_a((n - 2) % 2, u, p, NU * h + u)
                    if u % 2:
                        put(p, (NU * h + u) // 2, res[u - 1], res[u])

    @pl.when(t == 0)
    def _():
        copies[6].wait()
        copies[7].wait()
        for c in range(NLT):
            tmp_ref[c] = wob_ref[:, c * 128:(c + 1) * 128].astype(F32)
        permute_rows(wobp_ref)

    gl = jnp.sum(x.astype(F32) * gw_ref[...].astype(F32), axis=1, keepdims=True)
    g = jax.nn.sigmoid(gl)
    for c in range(NLT):
        a = _dot(oa_ref[...], woa_ref[:, c * 128:(c + 1) * 128])
        b = _dot(ob_ref[...], wobp_ref[c])
        o_ref[:, c * 128:(c + 1) * 128] = (g * a + (1.0 - g) * b).astype(o_ref.dtype)


@jax.jit
def pallas_gated_mix__sliding_block__sliding_local_dilated__prompt_kernel(
    A_x: jax.Array,
    A_wqkv: jax.Array,
    A_wo: jax.Array,
    B_x: jax.Array,
    B_wqkv: jax.Array,
    B_wo: jax.Array,
    gate_w: jax.Array,
):
    del B_x
    x = A_x.reshape(S, D)
    gw = gate_w.reshape(1, D)
    hbm = pl.BlockSpec(memory_space=pl.ANY)
    out = pl.pallas_call(
        kernel,
        grid=(S // R,),
        in_specs=[hbm] * 6,
        out_specs=pl.BlockSpec((R, D), lambda t: (t, 0)),
        out_shape=jax.ShapeDtypeStruct((S, D), BF),
        scratch_shapes=[
            pltpu.VMEM((S, D), BF),
            pltpu.VMEM((1, D), BF),
            pltpu.VMEM((3, D, D), BF),
            pltpu.VMEM((D, D), BF),
            pltpu.VMEM((3, D, D), BF),
            pltpu.VMEM((D, D), BF),
            pltpu.SemaphoreType.DMA((11,)),
            pltpu.VMEM((NT, R // 2, 128), U32),
            pltpu.VMEM((NT, (WA + S) // 2, 128), U32),
            pltpu.VMEM(((WA + S) // 128, D // 2, 128), U32),
            pltpu.VMEM((D, R), F32),
            pltpu.VMEM((R, D), BF),
            pltpu.VMEM((2, NU, WA + QC, 128), F32),
            pltpu.VMEM((2, NU, 192, 128), U32),
            pltpu.VMEM((3, NLT, D, 128), BF),
            pltpu.VMEM((NLT, D, 128), BF),
            pltpu.VMEM((NLT, D, 128), F32),
            pltpu.VMEM((NLT, R, 128), F32),
            pltpu.VMEM((NLT, HB + S, 128), F32),
            pltpu.VMEM((NLT, HB + S, 128), F32),
            pltpu.VMEM((R, D), BF),
        ],
        compiler_params=pltpu.CompilerParams(
            dimension_semantics=("arbitrary",),
            vmem_limit_bytes=100 * 1024 * 1024,
        ),
        name="gated_mix_attn",
    )(x, A_wqkv, A_wo, B_wqkv, B_wo, gw)
    return out.reshape(1, S, D)
```

```python
import jax
import jax.numpy as jnp
import numpy as np
import jax.experimental.pallas as pl
import jax.experimental.pallas.tpu as pltpu

S = 2048
D = 640
H = 32
DH = 20
NLT = D // 128
R = 512
QC = 64
NU = 4
NBAT = R // (QC * NU)
NPAIR = H // 2
WA = 256
HB = 16
RB = 16
NB1 = 20
LINK = 1
NEG = -1e30
LOG2E = 1.4426950408889634
QSCALE = float(DH ** -0.5) * LOG2E
BF = jnp.bfloat16
U32 = jnp.uint32
F32 = jnp.float32


def _pair_tile(p):
    c0 = 40 * p
    t0, off = divmod(c0, 128)
    if off + 40 <= 128:
        return (t0, t0, 0), off
    return (t0, t0 + 1, off), off


_TILES = []
_PAIR = []
for _p in range(NPAIR):
    _t, _o = _pair_tile(_p)
    if _t not in _TILES:
        _TILES.append(_t)
    _PAIR.append((_TILES.index(_t), _o))
NT = len(_TILES)


def _u32(x):
    return pltpu.bitcast(x, jnp.uint32)


def _bf(x):
    return pltpu.bitcast(x, BF)


def _pack16(y):
    g = y.shape[0] // 16
    y = y.reshape(g, 2, 8, y.shape[1])
    return pltpu.pack_elementwise(
        [y[:, 0].reshape(8 * g, -1), y[:, 1].reshape(8 * g, -1)], packed_dtype=BF)


def _nt_dot(a, b):
    return jax.lax.dot_general(a, b, (((1,), (1,)), ((), ())), preferred_element_type=F32)


def _dot(a, b):
    return jnp.dot(a, b, preferred_element_type=F32)


def kernel(*refs):
    jax.lax.fori_loop(0, S // R, lambda t, c: (step(t, *refs), c)[1], 0)


def step(t, x_hbm, wa_hbm, woa_hbm, wb_hbm, wob_hbm, gw_hbm, o_hbm,
         o_ref, osems, x_ref, gw_ref, wa_ref, woa_ref, wb_ref, wob_ref, sems,
           qa_ref, ka_ref, vta_ref, ot_ref, oa_ref, s_ref, p_ref,
           wbt_ref, wobp_ref, tmp_ref, qb_ref, kb_ref, vb_ref, ob_ref):
    not_first = t > 0
    row0 = pl.multiple_of(t * R, R)
    prow0 = pl.multiple_of(t * (R // 2), R // 2)

    phase = pl.when(t >= 0)

    def sec(ref, i):
        return ref.at[:, pl.ds(i * D, D)]

    copies = [pltpu.make_async_copy(sec(wb_hbm, i), wb_ref.at[i], sems.at[i]) for i in range(3)]
    copies += [pltpu.make_async_copy(sec(wa_hbm, i), wa_ref.at[i], sems.at[3 + i]) for i in range(3)]
    copies += [pltpu.make_async_copy(wob_hbm, wob_ref, sems.at[6]),
               pltpu.make_async_copy(woa_hbm, woa_ref, sems.at[7])]
    x_first = pltpu.make_async_copy(x_hbm.at[pl.ds(0, R)], x_ref.at[pl.ds(0, R)], sems.at[8])
    x_rest = pltpu.make_async_copy(x_hbm.at[pl.ds(R, S - R)], x_ref.at[pl.ds(R, S - R)], sems.at[9])
    gw_copy = pltpu.make_async_copy(gw_hbm, gw_ref, sems.at[10])

    @pl.when(t == 0)
    def _():
        copies[0].start()
        x_first.start()
        gw_copy.start()
        ka_ref[:, 0:WA // 2, :] = jnp.zeros((NT, WA // 2, 128), U32)
        for j in range(WA // 128):
            vta_ref[j] = jnp.zeros((D // 2, 128), U32)
        for u in range(NU):
            z = (WA + QC) // 2 if u % 2 == 0 else 0
            p_ref[:, u, z:z + QC // 2, :] = jnp.zeros((2, QC // 2, 128), U32)
        kb_ref[:, 0:HB, :] = jnp.zeros((NLT, HB, 128), F32)
        vb_ref[:, 0:HB, :] = jnp.zeros((NLT, HB, 128), F32)


    @pl.when(t == 1)
    def _():
        x_rest.wait()


    def permute_rows(dst_ref):
        for c in range(NLT):
            for d in range(DH):
                dst_ref[c, d * H:(d + 1) * H, :] = tmp_ref[c, pl.ds(d, H, stride=DH), :].astype(BF)

    def prep_b(i):
        copies[i].wait()
        for j in ((1,), (2, 3), (4, 5, 6, 7))[i]:
            copies[j].start()
        for c in range(NLT):
            for n in range(NLT):
                w = wb_ref[i, c * 128:(c + 1) * 128, n * 128:(n + 1) * 128]
                tmp_ref[c, n * 128:(n + 1) * 128, :] = w.astype(F32).T
        permute_rows(wbt_ref.at[i])
        if i == 0:
            x_first.wait()
            gw_copy.wait()

    def proj_b(i):
        dst = (qb_ref, kb_ref, vb_ref)[i]
        x = x_ref[pl.ds(row0, R), :]
        for n in range(NLT):
            y = None
            for c in range(NLT):
                z = _nt_dot(x[:, c * 128:(c + 1) * 128], wbt_ref[i, c, n * 128:(n + 1) * 128, :])
                y = z if y is None else y + z
            if i == 0:
                dst[n] = y * QSCALE
            else:
                dst[n, pl.ds(row0 + HB, R), :] = y

    @pl.when(t == 0)
    def _():
        for i in range(3):
            prep_b(i)
            proj_b(i)
        x_rest.start()
        for cp in copies[3:6]:
            cp.wait()

    @pl.when(t > 0)
    def _():
        for i in range(3):
            proj_b(i)

    rowb = jax.lax.broadcasted_iota(jnp.int32, (RB, 128), 0)

    never = t < 0
    chain = [None, None]

    def attn_b(ci):
        r = ci * RB
        q = [qb_ref[c, r:r + RB, :] for c in range(NLT)]
        if chain[ci % LINK] is not None:
            q[0] = jnp.where(never, chain[ci % LINK], q[0])
            q[NLT - 1] = jnp.where(never, chain[ci % LINK], q[NLT - 1])
        sc = []
        for j in range(8):
            acc = None
            for c in range(NLT):
                y = q[c] * kb_ref[c, pl.ds(row0 + (r + HB - 2 * j), RB), :]
                acc = y if acc is None else acc + y
            acc = acc + pltpu.roll(acc, 64, 1)
            acc = acc + pltpu.roll(acc, 32, 1)
            if r < 2 * j:
                acc = jnp.where(not_first | (rowb >= 2 * j - r), acc, NEG)
            sc.append(acc)
        m = sc[0]
        for y in sc[1:]:
            m = jnp.maximum(m, y)
        e = [jnp.exp2(y - m) for y in sc]
        l = e[0]
        for y in e[1:]:
            l = l + y
        inv = 1.0 / l
        for c in range(NLT):
            acc = None
            for j in range(8):
                y = e[j] * vb_ref[c, pl.ds(row0 + (r + HB - 2 * j), RB), :]
                acc = y if acc is None else acc + y
            ob_ref[r:r + RB, c * 128:(c + 1) * 128] = (acc * inv).astype(BF)
        chain[ci % LINK] = acc

    @phase
    def _():
        x = x_ref[pl.ds(row0, R), :]

        def put_tile(ref, rows, c, y):
            y = _u32(y.astype(BF))
            ref[_TILES.index((c, c, 0)), rows, :] = y
            for i, (ta, tb, split) in enumerate(_TILES):
                if ta != tb and tb == c:
                    lane = jax.lax.broadcasted_iota(jnp.int32, y.shape, 1)
                    ref[i, rows, :] = jnp.where(lane >= split, ref[_TILES.index((ta, ta, 0)), rows, :], y)

        for n in range(3 * NLT):
            sec_i, c = divmod(n, NLT)
            y = _dot(x, wa_ref[sec_i, :, c * 128:(c + 1) * 128])
            if sec_i == 0:
                put_tile(qa_ref, pl.ds(0, R // 2), c, y * QSCALE)
            elif sec_i == 1:
                put_tile(ka_ref, pl.ds(prow0 + WA // 2, R // 2), c, y)
            else:
                va = _bf(_pack16(y).astype(U32))
                for j in range(R // 128):
                    vta_ref[t * (R // 128) + WA // 128 + j, c * 64:(c + 1) * 64, :] = (
                        _u32(va[j * 128:(j + 1) * 128, :].T))
            for ci in range(n * NB1 // (3 * NLT), (n + 1) * NB1 // (3 * NLT)):
                attn_b(ci)

    lane128 = jax.lax.broadcasted_iota(jnp.int32, (QC, 128), 1)
    row64 = jax.lax.broadcasted_iota(jnp.int32, (QC, 128), 0)
    lower = row64 <= (lane128 & (QC - 1))
    lane32 = jax.lax.broadcasted_iota(jnp.int32, (QC // 2, 128), 1)
    row48 = jax.lax.broadcasted_iota(jnp.int32, (48, 128), 0)
    lane48 = jax.lax.broadcasted_iota(jnp.int32, (48, 128), 1)
    left = lane48 < 64

    def masked_q(p, i):
        tix, off = _PAIR[p]
        qt = qa_ref[tix, i * QC // 2:(i + 1) * QC // 2, :]
        rel = (lane32 - off) & 127
        ones = jnp.uint32(0xFFFFFFFF)
        m0 = jnp.where(rel < DH, ones, jnp.uint32(0))
        m1 = jnp.where((rel >= DH) & (rel < 2 * DH), ones, jnp.uint32(0))
        return _bf(jnp.concatenate([qt & m0, qt & m1], axis=0))

    def qk_a(sl, u, p, i):
        kk = _bf(ka_ref[_PAIR[p][0], pl.ds(prow0 + i * QC // 2, (WA + QC) // 2), :])
        s_ref[sl, u] = _nt_dot(kk, masked_q(p, i))

    def sm_a(sl, u, i):
        def chunk(c):
            v = s_ref[sl, u, c * QC:(c + 1) * QC, :]
            if c < WA // QC - i:
                v = jnp.where(not_first, v, NEG)
            return v

        def put_p(c, v):
            o = (QC * (i % 2) + c * QC) // 2
            p_ref[sl, u, o:o + QC // 2, :] = _pack16(v).astype(U32)

        mrg = jnp.where(lower, s_ref[sl, u, WA:WA + QC, :], chunk(0))
        mid = [chunk(c) for c in range(1, 4)]
        m = jnp.max(mrg, axis=0, keepdims=True)
        for v in mid:
            m = jnp.maximum(m, jnp.max(v, axis=0, keepdims=True))
        pg = jnp.exp2(mrg - m)
        put_p(0, jnp.where(lower, 0.0, pg))
        put_p(4, jnp.where(lower, pg, 0.0))
        for c, v in enumerate(mid):
            put_p(c + 1, jnp.exp2(v - m))

    word = jax.lax.broadcasted_iota(jnp.int32, (8, 128), 0)
    ones_w = jnp.uint32(0x3F803F80)

    def pv_a(sl, u, p, i):
        w0 = 20 * p - 4 * (p % 2)
        c0 = t * (R // 128) + i // 2
        acc = None
        for j in range(3):
            v = vta_ref[c0 + j, w0:w0 + 24, :]
            if p % 2:
                v = jnp.concatenate([jnp.where(word < 4, ones_w, v[0:8]), v[8:24]], axis=0)
            else:
                v = jnp.concatenate([v[0:16], jnp.where(word >= 4, ones_w, v[16:24])], axis=0)
            y = _dot(_bf(v), _bf(p_ref[sl, u, j * 64:(j + 1) * 64, :]))
            acc = y if acc is None else acc + y
        if p % 2:
            return acc[8:48] * jnp.tile(1.0 / acc[0:8], (5, 1))
        return acc[0:40] * jnp.tile(1.0 / acc[40:48], (5, 1))

    row40 = jax.lax.broadcasted_iota(jnp.int32, (40, 128), 0)
    left = jax.lax.broadcasted_iota(jnp.int32, (40, 128), 1) < 64

    def put(p, mm, r_e, r_o):
        h0 = row40 < DH
        tt = jnp.where(left, jnp.where(h0, r_e, pltpu.roll(r_e, 64, 1)),
                       jnp.where(h0, pltpu.roll(r_o, 64, 1), r_o))
        ot_ref[40 * p:40 * p + 40, mm * 128:(mm + 1) * 128] = tt
        for c in range(NLT):
            if 40 * p < (c + 1) * 128 <= 40 * p + 40:
                oa_ref[mm * 128:(mm + 1) * 128, c * 128:(c + 1) * 128] = (
                    ot_ref[c * 128:(c + 1) * 128, mm * 128:(mm + 1) * 128].astype(BF).T)

    @phase
    def _():
        chain[:] = [None] * len(chain)
        batches = [(p, h) for p in range(NPAIR) for h in range(NBAT)]
        for n in range(len(batches) + 2):
            if NB1 + n < R // RB:
                attn_b(NB1 + n)
            res = {}
            for u in range(NU):
                if n < len(batches):
                    p, h = batches[n]
                    qk_a(n % 2, u, p, NU * h + u)
                if 1 <= n <= len(batches):
                    p, h = batches[n - 1]
                    sm_a((n - 1) % 2, u, NU * h + u)
                if n >= 2:
                    p, h = batches[n - 2]
                    res[u] = pv_a((n - 2) % 2, u, p, NU * h + u)
                    if u % 2:
                        put(p, (NU * h + u) // 2, res[u - 1], res[u])

    @pl.when(t == 0)
    def _():
        copies[6].wait()
        copies[7].wait()
        for c in range(NLT):
            tmp_ref[c] = wob_ref[:, c * 128:(c + 1) * 128].astype(F32)
        permute_rows(wobp_ref)

    x = x_ref[pl.ds(row0, R), :]
    gl = jnp.sum(x.astype(F32) * gw_ref[...].astype(F32), axis=1, keepdims=True)
    g = jax.nn.sigmoid(gl)
    slot = t % 2
    parts = ((0, 384), (384, 256))

    def out_copy(tt, sl, k):
        c0, cn = parts[k]
        return pltpu.make_async_copy(o_ref.at[sl, :, pl.ds(c0, cn)],
                                     o_hbm.at[pl.ds(tt * R, R), pl.ds(c0, cn)], osems.at[sl, k])

    @pl.when(t >= 2)
    def _():
        for k in range(2):
            out_copy(t - 2, slot, k).wait()

    for c in range(NLT):
        a = _dot(oa_ref[...], woa_ref[:, c * 128:(c + 1) * 128])
        b = _dot(ob_ref[...], wobp_ref[c])
        o_ref[slot, :, c * 128:(c + 1) * 128] = (g * a + (1.0 - g) * b).astype(o_ref.dtype)
        if c == 2:
            out_copy(t, slot, 0).start()
    out_copy(t, slot, 1).start()

    @pl.when(t == S // R - 1)
    def _():
        for k in range(2):
            out_copy(t - 1, 1 - slot, k).wait()
            out_copy(t, slot, k).wait()


@jax.jit
def pallas_gated_mix__sliding_block__sliding_local_dilated__prompt_kernel(
    A_x: jax.Array,
    A_wqkv: jax.Array,
    A_wo: jax.Array,
    B_x: jax.Array,
    B_wqkv: jax.Array,
    B_wo: jax.Array,
    gate_w: jax.Array,
):
    del B_x
    x = A_x.reshape(S, D)
    gw = gate_w.reshape(1, D)
    hbm = pl.BlockSpec(memory_space=pl.ANY)
    out = pl.pallas_call(
        kernel,
        in_specs=[hbm] * 6,
        out_specs=hbm,
        out_shape=jax.ShapeDtypeStruct((S, D), BF),
        scratch_shapes=[
            pltpu.VMEM((2, R, D), BF),
            pltpu.SemaphoreType.DMA((2, 2)),
            pltpu.VMEM((S, D), BF),
            pltpu.VMEM((1, D), BF),
            pltpu.VMEM((3, D, D), BF),
            pltpu.VMEM((D, D), BF),
            pltpu.VMEM((3, D, D), BF),
            pltpu.VMEM((D, D), BF),
            pltpu.SemaphoreType.DMA((11,)),
            pltpu.VMEM((NT, R // 2, 128), U32),
            pltpu.VMEM((NT, (WA + S) // 2, 128), U32),
            pltpu.VMEM(((WA + S) // 128, D // 2, 128), U32),
            pltpu.VMEM((D, R), F32),
            pltpu.VMEM((R, D), BF),
            pltpu.VMEM((2, NU, WA + QC, 128), F32),
            pltpu.VMEM((2, NU, 192, 128), U32),
            pltpu.VMEM((3, NLT, D, 128), BF),
            pltpu.VMEM((NLT, D, 128), BF),
            pltpu.VMEM((NLT, D, 128), F32),
            pltpu.VMEM((NLT, R, 128), F32),
            pltpu.VMEM((NLT, HB + S, 128), F32),
            pltpu.VMEM((NLT, HB + S, 128), F32),
            pltpu.VMEM((R, D), BF),
        ],
        compiler_params=pltpu.CompilerParams(
            vmem_limit_bytes=100 * 1024 * 1024,
        ),
        name="gated_mix_attn",
    )(x, A_wqkv, A_wo, B_wqkv, B_wo, gw)
    return out.reshape(1, S, D)
```

```python
import jax
import jax.numpy as jnp
import jax.experimental.pallas as pl
import jax.experimental.pallas.tpu as pltpu

S = 2048
D = 640
H = 32
DH = 20
NLT = D // 128
R = 512
QC = 64
NU = 4
NBAT = R // (QC * NU)
NPAIR = H // 2
WA = 256
HB = 16
RB = 16
NB1 = 22
LINK = 1
NEG = -1e30
LOG2E = 1.4426950408889634
QSCALE = float(DH ** -0.5) * LOG2E
BF = jnp.bfloat16
U32 = jnp.uint32
F32 = jnp.float32


def _pair_tile(p):
    c0 = 40 * p
    t0, off = divmod(c0, 128)
    if off + 40 <= 128:
        return (t0, t0, 0), off
    return (t0, t0 + 1, off), off


_TILES = []
_PAIR = []
for _p in range(NPAIR):
    _t, _o = _pair_tile(_p)
    if _t not in _TILES:
        _TILES.append(_t)
    _PAIR.append((_TILES.index(_t), _o))
NT = len(_TILES)


def _u32(x):
    return pltpu.bitcast(x, jnp.uint32)


def _bf(x):
    return pltpu.bitcast(x, BF)


def _pack16(y):
    g = y.shape[0] // 16
    y = y.reshape(g, 2, 8, y.shape[1])
    return pltpu.pack_elementwise(
        [y[:, 0].reshape(8 * g, -1), y[:, 1].reshape(8 * g, -1)], packed_dtype=BF)


def _nt_dot(a, b):
    return jax.lax.dot_general(a, b, (((1,), (1,)), ((), ())), preferred_element_type=F32)


def _dot(a, b):
    return jnp.dot(a, b, preferred_element_type=F32)


def kernel(*refs):
    jax.lax.fori_loop(0, S // R, lambda t, c: (step(t, *refs), c)[1], 0)


def step(t, x_hbm, wa_hbm, woa_hbm, wb_hbm, wob_hbm, gw_hbm, o_hbm,
         o_ref, osems, x_ref, gw_ref, wa_ref, woa_ref, wb_ref, wob_ref, sems,
         qa_ref, ka_ref, vta_ref, ot_ref, oa_ref, s_ref, p_ref,
         wbt_ref, wobp_ref, tmp_ref, qb_ref, kb_ref, vb_ref, ob_ref):
    not_first = t > 0
    row0 = pl.multiple_of(t * R, R)
    prow0 = pl.multiple_of(t * (R // 2), R // 2)

    phase = pl.when(t >= 0)

    def sec(ref, i):
        return ref.at[:, pl.ds(i * D, D)]

    copies = [pltpu.make_async_copy(sec(wb_hbm, i), wb_ref.at[i], sems.at[i]) for i in range(3)]
    copies += [pltpu.make_async_copy(sec(wa_hbm, i), wa_ref.at[i], sems.at[3 + i]) for i in range(3)]
    copies += [pltpu.make_async_copy(wob_hbm, wob_ref, sems.at[6]),
               pltpu.make_async_copy(woa_hbm, woa_ref, sems.at[7])]
    x_first = pltpu.make_async_copy(x_hbm.at[pl.ds(0, R)], x_ref.at[pl.ds(0, R)], sems.at[8])
    x_rest = pltpu.make_async_copy(x_hbm.at[pl.ds(R, S - R)], x_ref.at[pl.ds(R, S - R)], sems.at[9])
    gw_copy = pltpu.make_async_copy(gw_hbm, gw_ref, sems.at[10])

    @pl.when(t == 0)
    def _():
        copies[0].start()
        x_first.start()
        gw_copy.start()
        ka_ref[:, 0:WA // 2, :] = jnp.zeros((NT, WA // 2, 128), U32)
        for j in range(WA // 128):
            vta_ref[j] = jnp.zeros((D // 2, 128), U32)
        for u in range(NU):
            z = (WA + QC) // 2 if u % 2 == 0 else 0
            p_ref[:, u, z:z + QC // 2, :] = jnp.zeros((2, QC // 2, 128), U32)
        kb_ref[:, 0:HB, :] = jnp.zeros((NLT, HB, 128), F32)
        vb_ref[:, 0:HB, :] = jnp.zeros((NLT, HB, 128), F32)

    @pl.when(t == 1)
    def _():
        x_rest.wait()

    def permute_rows(dst_ref):
        for c in range(NLT):
            for d in range(DH):
                dst_ref[c, d * H:(d + 1) * H, :] = tmp_ref[c, pl.ds(d, H, stride=DH), :].astype(BF)

    def prep_b(i):
        copies[i].wait()
        for j in ((1,), (2, 3), (4, 5, 6, 7))[i]:
            copies[j].start()
        for c in range(NLT):
            for n in range(NLT):
                w = wb_ref[i, c * 128:(c + 1) * 128, n * 128:(n + 1) * 128]
                tmp_ref[c, n * 128:(n + 1) * 128, :] = w.astype(F32).T
        permute_rows(wbt_ref.at[i])
        if i == 0:
            x_first.wait()
            gw_copy.wait()

    def proj_b(i):
        dst = (qb_ref, kb_ref, vb_ref)[i]
        x = x_ref[pl.ds(row0, R), :]
        for n in range(NLT):
            y = None
            for c in range(NLT):
                z = _nt_dot(x[:, c * 128:(c + 1) * 128], wbt_ref[i, c, n * 128:(n + 1) * 128, :])
                y = z if y is None else y + z
            if i == 0:
                dst[n] = y * QSCALE
            else:
                dst[n, pl.ds(row0 + HB, R), :] = y

    @pl.when(t == 0)
    def _():
        for i in range(3):
            prep_b(i)
            proj_b(i)
        x_rest.start()
        for cp in copies[3:6]:
            cp.wait()

    @pl.when(t > 0)
    def _():
        for i in range(3):
            proj_b(i)

    rowb = jax.lax.broadcasted_iota(jnp.int32, (RB, 128), 0)

    never = t < 0
    chain = [None, None]

    def attn_b(ci):
        r = ci * RB
        q = [qb_ref[c, r:r + RB, :] for c in range(NLT)]
        if chain[ci % LINK] is not None:
            q[0] = jnp.where(never, chain[ci % LINK], q[0])
            q[NLT - 1] = jnp.where(never, chain[ci % LINK], q[NLT - 1])
        sc = []
        for j in range(8):
            acc = None
            for c in range(NLT):
                y = q[c] * kb_ref[c, pl.ds(row0 + (r + HB - 2 * j), RB), :]
                acc = y if acc is None else acc + y
            acc = acc + pltpu.roll(acc, 64, 1)
            acc = acc + pltpu.roll(acc, 32, 1)
            if r < 2 * j:
                acc = jnp.where(not_first | (rowb >= 2 * j - r), acc, NEG)
            sc.append(acc)
        m = sc[0]
        for y in sc[1:]:
            m = jnp.maximum(m, y)
        e = [jnp.exp2(y - m) for y in sc]
        l = e[0]
        for y in e[1:]:
            l = l + y
        inv = 1.0 / l
        for c in range(NLT):
            acc = None
            for j in range(8):
                y = e[j] * vb_ref[c, pl.ds(row0 + (r + HB - 2 * j), RB), :]
                acc = y if acc is None else acc + y
            ob_ref[r:r + RB, c * 128:(c + 1) * 128] = (acc * inv).astype(BF)
        chain[ci % LINK] = acc

    @phase
    def _():
        x = x_ref[pl.ds(row0, R), :]

        def put_tile(ref, rows, c, y):
            y = _u32(y.astype(BF))
            ref[_TILES.index((c, c, 0)), rows, :] = y
            for i, (ta, tb, split) in enumerate(_TILES):
                if ta != tb and tb == c:
                    lane = jax.lax.broadcasted_iota(jnp.int32, y.shape, 1)
                    ref[i, rows, :] = jnp.where(lane >= split, ref[_TILES.index((ta, ta, 0)), rows, :], y)

        for n in range(3 * NLT):
            sec_i, c = divmod(n, NLT)
            y = _dot(x, wa_ref[sec_i, :, c * 128:(c + 1) * 128])
            if sec_i == 0:
                put_tile(qa_ref, pl.ds(0, R // 2), c, y * QSCALE)
            elif sec_i == 1:
                put_tile(ka_ref, pl.ds(prow0 + WA // 2, R // 2), c, y)
            else:
                va = _bf(_pack16(y).astype(U32))
                for j in range(R // 128):
                    vta_ref[t * (R // 128) + WA // 128 + j, c * 64:(c + 1) * 64, :] = (
                        _u32(va[j * 128:(j + 1) * 128, :].T))
            for ci in range(n * NB1 // (3 * NLT), (n + 1) * NB1 // (3 * NLT)):
                attn_b(ci)

    lane128 = jax.lax.broadcasted_iota(jnp.int32, (QC, 128), 1)
    row64 = jax.lax.broadcasted_iota(jnp.int32, (QC, 128), 0)
    lower = row64 <= (lane128 & (QC - 1))
    lane32 = jax.lax.broadcasted_iota(jnp.int32, (QC // 2, 128), 1)
    row48 = jax.lax.broadcasted_iota(jnp.int32, (48, 128), 0)
    lane48 = jax.lax.broadcasted_iota(jnp.int32, (48, 128), 1)
    left = lane48 < 64

    def masked_q(p, i):
        tix, off = _PAIR[p]
        qt = qa_ref[tix, i * QC // 2:(i + 1) * QC // 2, :]
        rel = (lane32 - off) & 127
        ones = jnp.uint32(0xFFFFFFFF)
        m0 = jnp.where(rel < DH, ones, jnp.uint32(0))
        m1 = jnp.where((rel >= DH) & (rel < 2 * DH), ones, jnp.uint32(0))
        return _bf(jnp.concatenate([qt & m0, qt & m1], axis=0))

    def qk_a(sl, u, p, i):
        kk = _bf(ka_ref[_PAIR[p][0], pl.ds(prow0 + i * QC // 2, (WA + QC) // 2), :])
        s_ref[sl, u] = _nt_dot(kk, masked_q(p, i))

    def sm_a(sl, u, i):
        def chunk(c):
            v = s_ref[sl, u, c * QC:(c + 1) * QC, :]
            if c < WA // QC - i:
                v = jnp.where(not_first, v, NEG)
            return v

        def put_p(c, v):
            o = (QC * (i % 2) + c * QC) // 2
            p_ref[sl, u, o:o + QC // 2, :] = _pack16(v).astype(U32)

        mrg = jnp.where(lower, s_ref[sl, u, WA:WA + QC, :], chunk(0))
        mid = [chunk(c) for c in range(1, 4)]
        m = jnp.max(mrg, axis=0, keepdims=True)
        for v in mid:
            m = jnp.maximum(m, jnp.max(v, axis=0, keepdims=True))
        pg = jnp.exp2(mrg - m)
        put_p(0, jnp.where(lower, 0.0, pg))
        put_p(4, jnp.where(lower, pg, 0.0))
        for c, v in enumerate(mid):
            put_p(c + 1, jnp.exp2(v - m))

    word = jax.lax.broadcasted_iota(jnp.int32, (8, 128), 0)
    ones_w = jnp.uint32(0x3F803F80)

    def pv_a(sl, u, p, i):
        w0 = 20 * p - 4 * (p % 2)
        c0 = t * (R // 128) + i // 2
        acc = None
        for j in range(3):
            v = vta_ref[c0 + j, w0:w0 + 24, :]
            if p % 2:
                v = jnp.concatenate([jnp.where(word < 4, ones_w, v[0:8]), v[8:24]], axis=0)
            else:
                v = jnp.concatenate([v[0:16], jnp.where(word >= 4, ones_w, v[16:24])], axis=0)
            y = _dot(_bf(v), _bf(p_ref[sl, u, j * 64:(j + 1) * 64, :]))
            acc = y if acc is None else acc + y
        if p % 2:
            return acc[8:48] * jnp.tile(1.0 / acc[0:8], (5, 1))
        return acc[0:40] * jnp.tile(1.0 / acc[40:48], (5, 1))

    row40 = jax.lax.broadcasted_iota(jnp.int32, (40, 128), 0)
    left = jax.lax.broadcasted_iota(jnp.int32, (40, 128), 1) < 64

    def put(p, mm, r_e, r_o):
        h0 = row40 < DH
        tt = jnp.where(left, jnp.where(h0, r_e, pltpu.roll(r_e, 64, 1)),
                       jnp.where(h0, pltpu.roll(r_o, 64, 1), r_o))
        ot_ref[40 * p:40 * p + 40, mm * 128:(mm + 1) * 128] = tt
        for c in range(NLT):
            if 40 * p < (c + 1) * 128 <= 40 * p + 40:
                oa_ref[mm * 128:(mm + 1) * 128, c * 128:(c + 1) * 128] = (
                    ot_ref[c * 128:(c + 1) * 128, mm * 128:(mm + 1) * 128].astype(BF).T)

    @phase
    def _():
        chain[:] = [None] * len(chain)
        batches = [(p, h) for p in range(NPAIR) for h in range(NBAT)]
        for n in range(len(batches) + 2):
            if NB1 + n < R // RB:
                attn_b(NB1 + n)
            res = {}
            for u in range(NU):
                if n < len(batches):
                    p, h = batches[n]
                    qk_a(n % 2, u, p, NU * h + u)
                if 1 <= n <= len(batches):
                    p, h = batches[n - 1]
                    sm_a((n - 1) % 2, u, NU * h + u)
                if n >= 2:
                    p, h = batches[n - 2]
                    res[u] = pv_a((n - 2) % 2, u, p, NU * h + u)
                    if u % 2:
                        put(p, (NU * h + u) // 2, res[u - 1], res[u])

    @pl.when(t == 0)
    def _():
        copies[6].wait()
        copies[7].wait()
        for c in range(NLT):
            tmp_ref[c] = wob_ref[:, c * 128:(c + 1) * 128].astype(F32)
        permute_rows(wobp_ref)

    x = x_ref[pl.ds(row0, R), :]
    gl = jnp.sum(x.astype(F32) * gw_ref[...].astype(F32), axis=1, keepdims=True)
    g = jax.nn.sigmoid(gl)
    slot = t % 2
    parts = ((0, 384), (384, 256))

    def out_copy(tt, sl, k):
        c0, cn = parts[k]
        return pltpu.make_async_copy(o_ref.at[sl, :, pl.ds(c0, cn)],
                                     o_hbm.at[pl.ds(tt * R, R), pl.ds(c0, cn)], osems.at[sl, k])

    @pl.when(t >= 2)
    def _():
        for k in range(2):
            out_copy(t - 2, slot, k).wait()

    for c in range(NLT):
        a = _dot(oa_ref[...], woa_ref[:, c * 128:(c + 1) * 128])
        b = _dot(ob_ref[...], wobp_ref[c])
        o_ref[slot, :, c * 128:(c + 1) * 128] = (g * a + (1.0 - g) * b).astype(o_ref.dtype)
        if c == 2:
            out_copy(t, slot, 0).start()
    out_copy(t, slot, 1).start()

    @pl.when(t == S // R - 1)
    def _():
        for k in range(2):
            out_copy(t - 1, 1 - slot, k).wait()
            out_copy(t, slot, k).wait()


@jax.jit
def pallas_gated_mix__sliding_block__sliding_local_dilated__prompt_kernel(
    A_x: jax.Array,
    A_wqkv: jax.Array,
    A_wo: jax.Array,
    B_x: jax.Array,
    B_wqkv: jax.Array,
    B_wo: jax.Array,
    gate_w: jax.Array,
):
    del B_x
    x = A_x.reshape(S, D)
    gw = gate_w.reshape(1, D)
    hbm = pl.BlockSpec(memory_space=pl.ANY)
    out = pl.pallas_call(
        kernel,
        in_specs=[hbm] * 6,
        out_specs=hbm,
        out_shape=jax.ShapeDtypeStruct((S, D), BF),
        scratch_shapes=[
            pltpu.VMEM((2, R, D), BF),
            pltpu.SemaphoreType.DMA((2, 2)),
            pltpu.VMEM((S, D), BF),
            pltpu.VMEM((1, D), BF),
            pltpu.VMEM((3, D, D), BF),
            pltpu.VMEM((D, D), BF),
            pltpu.VMEM((3, D, D), BF),
            pltpu.VMEM((D, D), BF),
            pltpu.SemaphoreType.DMA((11,)),
            pltpu.VMEM((NT, R // 2, 128), U32),
            pltpu.VMEM((NT, (WA + S) // 2, 128), U32),
            pltpu.VMEM(((WA + S) // 128, D // 2, 128), U32),
            pltpu.VMEM((D, R), F32),
            pltpu.VMEM((R, D), BF),
            pltpu.VMEM((2, NU, WA + QC, 128), F32),
            pltpu.VMEM((2, NU, 192, 128), U32),
            pltpu.VMEM((3, NLT, D, 128), BF),
            pltpu.VMEM((NLT, D, 128), BF),
            pltpu.VMEM((NLT, D, 128), F32),
            pltpu.VMEM((NLT, R, 128), F32),
            pltpu.VMEM((NLT, HB + S, 128), F32),
            pltpu.VMEM((NLT, HB + S, 128), F32),
            pltpu.VMEM((R, D), BF),
        ],
        compiler_params=pltpu.CompilerParams(
            vmem_limit_bytes=100 * 1024 * 1024,
        ),
        name="gated_mix_attn",
    )(x, A_wqkv, A_wo, B_wqkv, B_wo, gw)
    return out.reshape(1, S, D)
```

```python
import jax
import jax.numpy as jnp
import jax.experimental.pallas as pl
import jax.experimental.pallas.tpu as pltpu

S = 2048
D = 640
H = 32
DH = 20
NLT = D // 128
R = 512
QC = 64
NU = 4
NBAT = R // (QC * NU)
NPAIR = H // 2
WA = 256
HB = 16
RB = 16
NB1 = 24
BSTR = 3
LINK = 1
NEG = -1e30
LOG2E = 1.4426950408889634
QSCALE = float(DH ** -0.5) * LOG2E
BF = jnp.bfloat16
U32 = jnp.uint32
F32 = jnp.float32


def _pair_tile(p):
    c0 = 40 * p
    t0, off = divmod(c0, 128)
    if off + 40 <= 128:
        return (t0, t0, 0), off
    return (t0, t0 + 1, off), off


_TILES = []
_PAIR = []
for _p in range(NPAIR):
    _t, _o = _pair_tile(_p)
    if _t not in _TILES:
        _TILES.append(_t)
    _PAIR.append((_TILES.index(_t), _o))
NT = len(_TILES)


def _u32(x):
    return pltpu.bitcast(x, jnp.uint32)


def _bf(x):
    return pltpu.bitcast(x, BF)


def _pack16(y):
    g = y.shape[0] // 16
    y = y.reshape(g, 2, 8, y.shape[1])
    return pltpu.pack_elementwise(
        [y[:, 0].reshape(8 * g, -1), y[:, 1].reshape(8 * g, -1)], packed_dtype=BF)


def _nt_dot(a, b):
    return jax.lax.dot_general(a, b, (((1,), (1,)), ((), ())), preferred_element_type=F32)


def _dot(a, b):
    return jnp.dot(a, b, preferred_element_type=F32)


def kernel(*refs):
    jax.lax.fori_loop(0, S // R, lambda t, c: (step(t, *refs), c)[1], 0)


def step(t, x_hbm, wa_hbm, woa_hbm, wb_hbm, wob_hbm, gw_hbm, o_hbm,
         o_ref, osems, x_ref, gw_ref, wa_ref, woa_ref, wb_ref, wob_ref, sems,
         qa_ref, ka_ref, vta_ref, ot_ref, oa_ref, s_ref, p_ref,
         wbt_ref, wobp_ref, tmp_ref, qb_ref, kb_ref, vb_ref, ob_ref):
    not_first = t > 0
    row0 = pl.multiple_of(t * R, R)
    prow0 = pl.multiple_of(t * (R // 2), R // 2)

    phase = pl.when(t >= 0)

    def sec(ref, i):
        return ref.at[:, pl.ds(i * D, D)]

    copies = [pltpu.make_async_copy(sec(wb_hbm, i), wb_ref.at[i], sems.at[i]) for i in range(3)]
    copies += [pltpu.make_async_copy(sec(wa_hbm, i), wa_ref.at[i], sems.at[3 + i]) for i in range(3)]
    copies += [pltpu.make_async_copy(wob_hbm, wob_ref, sems.at[6]),
               pltpu.make_async_copy(woa_hbm, woa_ref, sems.at[7])]
    x_first = pltpu.make_async_copy(x_hbm.at[pl.ds(0, R)], x_ref.at[pl.ds(0, R)], sems.at[8])
    x_rest = pltpu.make_async_copy(x_hbm.at[pl.ds(R, S - R)], x_ref.at[pl.ds(R, S - R)], sems.at[9])
    gw_copy = pltpu.make_async_copy(gw_hbm, gw_ref, sems.at[10])

    @pl.when(t == 0)
    def _():
        copies[0].start()
        x_first.start()
        gw_copy.start()
        ka_ref[:, 0:WA // 2, :] = jnp.zeros((NT, WA // 2, 128), U32)
        for j in range(WA // 128):
            vta_ref[j] = jnp.zeros((D // 2, 128), U32)
        for u in range(NU):
            z = (WA + QC) // 2 if u % 2 == 0 else 0
            p_ref[:, u, z:z + QC // 2, :] = jnp.zeros((2, QC // 2, 128), U32)
        kb_ref[:, 0:HB, :] = jnp.zeros((NLT, HB, 128), F32)
        vb_ref[:, 0:HB, :] = jnp.zeros((NLT, HB, 128), F32)

    @pl.when(t == 1)
    def _():
        x_rest.wait()

    def permute_rows(dst_ref):
        for c in range(NLT):
            for d in range(DH):
                dst_ref[c, d * H:(d + 1) * H, :] = tmp_ref[c, pl.ds(d, H, stride=DH), :].astype(BF)

    def prep_b(i):
        copies[i].wait()
        for j in ((1,), (2, 3), (4, 5, 6, 7))[i]:
            copies[j].start()
        for c in range(NLT):
            for n in range(NLT):
                w = wb_ref[i, c * 128:(c + 1) * 128, n * 128:(n + 1) * 128]
                tmp_ref[c, n * 128:(n + 1) * 128, :] = w.astype(F32).T
        permute_rows(wbt_ref.at[i])
        if i == 0:
            x_first.wait()
            gw_copy.wait()

    def proj_b(i):
        dst = (qb_ref, kb_ref, vb_ref)[i]
        x = x_ref[pl.ds(row0, R), :]
        for n in range(NLT):
            y = None
            for c in range(NLT):
                z = _nt_dot(x[:, c * 128:(c + 1) * 128], wbt_ref[i, c, n * 128:(n + 1) * 128, :])
                y = z if y is None else y + z
            if i == 0:
                dst[n] = y * QSCALE
            else:
                dst[n, pl.ds(row0 + HB, R), :] = y

    @pl.when(t == 0)
    def _():
        for i in range(3):
            prep_b(i)
            proj_b(i)
        x_rest.start()
        for cp in copies[3:6]:
            cp.wait()

    @pl.when(t > 0)
    def _():
        for i in range(3):
            proj_b(i)

    rowb = jax.lax.broadcasted_iota(jnp.int32, (RB, 128), 0)

    never = t < 0
    chain = [None, None]

    def attn_b(ci):
        r = ci * RB
        q = [qb_ref[c, r:r + RB, :] for c in range(NLT)]
        if chain[ci % LINK] is not None:
            q[0] = jnp.where(never, chain[ci % LINK], q[0])
            q[NLT - 1] = jnp.where(never, chain[ci % LINK], q[NLT - 1])
        sc = []
        for j in range(8):
            acc = None
            for c in range(NLT):
                y = q[c] * kb_ref[c, pl.ds(row0 + (r + HB - 2 * j), RB), :]
                acc = y if acc is None else acc + y
            acc = acc + pltpu.roll(acc, 64, 1)
            acc = acc + pltpu.roll(acc, 32, 1)
            if r < 2 * j:
                acc = jnp.where(not_first | (rowb >= 2 * j - r), acc, NEG)
            sc.append(acc)
        m = sc[0]
        for y in sc[1:]:
            m = jnp.maximum(m, y)
        e = [jnp.exp2(y - m) for y in sc]
        l = e[0]
        for y in e[1:]:
            l = l + y
        inv = 1.0 / l
        for c in range(NLT):
            acc = None
            for j in range(8):
                y = e[j] * vb_ref[c, pl.ds(row0 + (r + HB - 2 * j), RB), :]
                acc = y if acc is None else acc + y
            ob_ref[r:r + RB, c * 128:(c + 1) * 128] = (acc * inv).astype(BF)
        chain[ci % LINK] = acc

    @phase
    def _():
        x = x_ref[pl.ds(row0, R), :]

        def put_tile(ref, rows, c, y):
            y = _u32(y.astype(BF))
            ref[_TILES.index((c, c, 0)), rows, :] = y
            for i, (ta, tb, split) in enumerate(_TILES):
                if ta != tb and tb == c:
                    lane = jax.lax.broadcasted_iota(jnp.int32, y.shape, 1)
                    ref[i, rows, :] = jnp.where(lane >= split, ref[_TILES.index((ta, ta, 0)), rows, :], y)

        for n in range(3 * NLT):
            sec_i, c = divmod(n, NLT)
            y = _dot(x, wa_ref[sec_i, :, c * 128:(c + 1) * 128])
            if sec_i == 0:
                put_tile(qa_ref, pl.ds(0, R // 2), c, y * QSCALE)
            elif sec_i == 1:
                put_tile(ka_ref, pl.ds(prow0 + WA // 2, R // 2), c, y)
            else:
                va = _bf(_pack16(y).astype(U32))
                for j in range(R // 128):
                    vta_ref[t * (R // 128) + WA // 128 + j, c * 64:(c + 1) * 64, :] = (
                        _u32(va[j * 128:(j + 1) * 128, :].T))
            for ci in range(n * NB1 // (3 * NLT), (n + 1) * NB1 // (3 * NLT)):
                attn_b(ci)

    lane128 = jax.lax.broadcasted_iota(jnp.int32, (QC, 128), 1)
    row64 = jax.lax.broadcasted_iota(jnp.int32, (QC, 128), 0)
    lower = row64 <= (lane128 & (QC - 1))
    lane32 = jax.lax.broadcasted_iota(jnp.int32, (QC // 2, 128), 1)
    row48 = jax.lax.broadcasted_iota(jnp.int32, (48, 128), 0)
    lane48 = jax.lax.broadcasted_iota(jnp.int32, (48, 128), 1)
    left = lane48 < 64

    def masked_q(p, i):
        tix, off = _PAIR[p]
        qt = qa_ref[tix, i * QC // 2:(i + 1) * QC // 2, :]
        rel = (lane32 - off) & 127
        ones = jnp.uint32(0xFFFFFFFF)
        m0 = jnp.where(rel < DH, ones, jnp.uint32(0))
        m1 = jnp.where((rel >= DH) & (rel < 2 * DH), ones, jnp.uint32(0))
        return _bf(jnp.concatenate([qt & m0, qt & m1], axis=0))

    def qk_a(sl, u, p, i):
        kk = _bf(ka_ref[_PAIR[p][0], pl.ds(prow0 + i * QC // 2, (WA + QC) // 2), :])
        s_ref[sl, u] = _nt_dot(kk, masked_q(p, i))

    def sm_a(sl, u, i):
        def chunk(c):
            v = s_ref[sl, u, c * QC:(c + 1) * QC, :]
            if c < WA // QC - i:
                v = jnp.where(not_first, v, NEG)
            return v

        def put_p(c, v):
            o = (QC * (i % 2) + c * QC) // 2
            p_ref[sl, u, o:o + QC // 2, :] = _pack16(v).astype(U32)

        mrg = jnp.where(lower, s_ref[sl, u, WA:WA + QC, :], chunk(0))
        mid = [chunk(c) for c in range(1, 4)]
        m = jnp.max(mrg, axis=0, keepdims=True)
        for v in mid:
            m = jnp.maximum(m, jnp.max(v, axis=0, keepdims=True))
        pg = jnp.exp2(mrg - m)
        put_p(0, jnp.where(lower, 0.0, pg))
        put_p(4, jnp.where(lower, pg, 0.0))
        for c, v in enumerate(mid):
            put_p(c + 1, jnp.exp2(v - m))

    word = jax.lax.broadcasted_iota(jnp.int32, (8, 128), 0)
    ones_w = jnp.uint32(0x3F803F80)

    def pv_a(sl, u, p, i):
        w0 = 20 * p - 4 * (p % 2)
        c0 = t * (R // 128) + i // 2
        acc = None
        for j in range(3):
            v = vta_ref[c0 + j, w0:w0 + 24, :]
            if p % 2:
                v = jnp.concatenate([jnp.where(word < 4, ones_w, v[0:8]), v[8:24]], axis=0)
            else:
                v = jnp.concatenate([v[0:16], jnp.where(word >= 4, ones_w, v[16:24])], axis=0)
            y = _dot(_bf(v), _bf(p_ref[sl, u, j * 64:(j + 1) * 64, :]))
            acc = y if acc is None else acc + y
        if p % 2:
            return acc[8:48] * jnp.tile(1.0 / acc[0:8], (5, 1))
        return acc[0:40] * jnp.tile(1.0 / acc[40:48], (5, 1))

    row40 = jax.lax.broadcasted_iota(jnp.int32, (40, 128), 0)
    left = jax.lax.broadcasted_iota(jnp.int32, (40, 128), 1) < 64

    def put(p, mm, r_e, r_o):
        h0 = row40 < DH
        tt = jnp.where(left, jnp.where(h0, r_e, pltpu.roll(r_e, 64, 1)),
                       jnp.where(h0, pltpu.roll(r_o, 64, 1), r_o))
        ot_ref[40 * p:40 * p + 40, mm * 128:(mm + 1) * 128] = tt
        for c in range(NLT):
            if 40 * p < (c + 1) * 128 <= 40 * p + 40:
                oa_ref[mm * 128:(mm + 1) * 128, c * 128:(c + 1) * 128] = (
                    ot_ref[c * 128:(c + 1) * 128, mm * 128:(mm + 1) * 128].astype(BF).T)

    @phase
    def _():
        chain[:] = [None] * len(chain)
        batches = [(p, h) for p in range(NPAIR) for h in range(NBAT)]
        for n in range(len(batches) + 2):
            if n % BSTR == 0 and NB1 + n // BSTR < R // RB:
                attn_b(NB1 + n // BSTR)
            res = {}
            for u in range(NU):
                if n < len(batches):
                    p, h = batches[n]
                    qk_a(n % 2, u, p, NU * h + u)
                if 1 <= n <= len(batches):
                    p, h = batches[n - 1]
                    sm_a((n - 1) % 2, u, NU * h + u)
                if n >= 2:
                    p, h = batches[n - 2]
                    res[u] = pv_a((n - 2) % 2, u, p, NU * h + u)
                    if u % 2:
                        put(p, (NU * h + u) // 2, res[u - 1], res[u])

    @pl.when(t == 0)
    def _():
        copies[6].wait()
        copies[7].wait()
        for c in range(NLT):
            tmp_ref[c] = wob_ref[:, c * 128:(c + 1) * 128].astype(F32)
        permute_rows(wobp_ref)

    x = x_ref[pl.ds(row0, R), :]
    gl = jnp.sum(x.astype(F32) * gw_ref[...].astype(F32), axis=1, keepdims=True)
    g = jax.nn.sigmoid(gl)
    slot = t % 2
    parts = ((0, 384), (384, 256))

    def out_copy(tt, sl, k):
        c0, cn = parts[k]
        return pltpu.make_async_copy(o_ref.at[sl, :, pl.ds(c0, cn)],
                                     o_hbm.at[pl.ds(tt * R, R), pl.ds(c0, cn)], osems.at[sl, k])

    @pl.when(t >= 2)
    def _():
        for k in range(2):
            out_copy(t - 2, slot, k).wait()

    for c in range(NLT):
        a = _dot(oa_ref[...], woa_ref[:, c * 128:(c + 1) * 128])
        b = _dot(ob_ref[...], wobp_ref[c])
        o_ref[slot, :, c * 128:(c + 1) * 128] = (g * a + (1.0 - g) * b).astype(o_ref.dtype)
        if c == 2:
            out_copy(t, slot, 0).start()
    out_copy(t, slot, 1).start()

    @pl.when(t == S // R - 1)
    def _():
        for k in range(2):
            out_copy(t - 1, 1 - slot, k).wait()
            out_copy(t, slot, k).wait()


@jax.jit
def pallas_gated_mix__sliding_block__sliding_local_dilated__prompt_kernel(
    A_x: jax.Array,
    A_wqkv: jax.Array,
    A_wo: jax.Array,
    B_x: jax.Array,
    B_wqkv: jax.Array,
    B_wo: jax.Array,
    gate_w: jax.Array,
):
    del B_x
    x = A_x.reshape(S, D)
    gw = gate_w.reshape(1, D)
    hbm = pl.BlockSpec(memory_space=pl.ANY)
    out = pl.pallas_call(
        kernel,
        in_specs=[hbm] * 6,
        out_specs=hbm,
        out_shape=jax.ShapeDtypeStruct((S, D), BF),
        scratch_shapes=[
            pltpu.VMEM((2, R, D), BF),
            pltpu.SemaphoreType.DMA((2, 2)),
            pltpu.VMEM((S, D), BF),
            pltpu.VMEM((1, D), BF),
            pltpu.VMEM((3, D, D), BF),
            pltpu.VMEM((D, D), BF),
            pltpu.VMEM((3, D, D), BF),
            pltpu.VMEM((D, D), BF),
            pltpu.SemaphoreType.DMA((11,)),
            pltpu.VMEM((NT, R // 2, 128), U32),
            pltpu.VMEM((NT, (WA + S) // 2, 128), U32),
            pltpu.VMEM(((WA + S) // 128, D // 2, 128), U32),
            pltpu.VMEM((D, R), F32),
            pltpu.VMEM((R, D), BF),
            pltpu.VMEM((2, NU, WA + QC, 128), F32),
            pltpu.VMEM((2, NU, 192, 128), U32),
            pltpu.VMEM((3, NLT, D, 128), BF),
            pltpu.VMEM((NLT, D, 128), BF),
            pltpu.VMEM((NLT, D, 128), F32),
            pltpu.VMEM((NLT, R, 128), F32),
            pltpu.VMEM((NLT, HB + S, 128), F32),
            pltpu.VMEM((NLT, HB + S, 128), F32),
            pltpu.VMEM((R, D), BF),
        ],
        compiler_params=pltpu.CompilerParams(
            vmem_limit_bytes=100 * 1024 * 1024,
        ),
        name="gated_mix_attn",
    )(x, A_wqkv, A_wo, B_wqkv, B_wo, gw)
    return out.reshape(1, S, D)
```
